```python
import jax
import jax.numpy as jnp

def _softmax(x, axis=-1):
    return jax.nn.softmax(x, axis=axis)

def _gelu(x):
    return jax.nn.gelu(x, approximate=True)

def _silu(x):
    return jax.nn.silu(x)

def _sigmoid(x):
    return jax.nn.sigmoid(x)

def _layernorm(x, axis=-1, eps=1e-05):
    m = jnp.mean(x, axis=axis, keepdims=True)
    v = jnp.var(x, axis=axis, keepdims=True)
    return (x - m) / jnp.sqrt(v + eps)

def _scatter_add(tgt, idx, src, axis=0):
    return tgt.at[idx].add(src)

def _segment_sum(src, seg, n):
    return jax.ops.segment_sum(src, seg, n)

class _Rng:

    def __init__(self, key):
        self._k = key

    def _next(self):
        self._k, sub = jax.random.split(self._k)
        return sub

    def normal(self, shape):
        return jax.random.normal(self._next(), shape, dtype=jnp.bfloat16)

    def randint(self, lo, hi, shape):
        return jax.random.randint(self._next(), shape, lo, hi, dtype=jnp.int32)

    def uniform(self, shape, lo=0.0, hi=1.0):
        return jax.random.uniform(self._next(), shape, jnp.bfloat16, lo, hi)

    def permutation(self, n):
        return jax.random.permutation(self._next(), n)
kernel_name = 'adaLN_cond__mha_block_cached__moe_arch_mod__prompt'

def setup_inputs():
    _rng = _Rng(jax.random.key(int.from_bytes(__import__("os").urandom(4), "little")))
    _w = lambda a: (lambda t: t.astype(jnp.bfloat16) if jnp.issubdtype(t.dtype, jnp.floating) else t)(jnp.asarray(a))

    def _A_setup():
        B, Sq, D = (1, 2048, 1024)
        H, Sk, Dh = (32, 2048, 128)
        return {'x': _w((lambda *s: _rng.normal(s) * 0.05)(B, Sq, D)), 'k_cache': _w((lambda *s: _rng.normal(s) * 0.05)(B, H, Sk, Dh)), 'v_cache': _w((lambda *s: _rng.normal(s) * 0.05)(B, H, Sk, Dh)), 'wq': _w((lambda *s: _rng.normal(s) * 0.05)(D, H * Dh) * D ** (-0.5)), 'wo': _w((lambda *s: _rng.normal(s) * 0.05)(H * Dh, D) * (H * Dh) ** (-0.5))}
    _A_in = _A_setup()

    def _B_setup():
        B, S, D, F, C = (1, 2048, 1024, 3584, 2)
        return {'x': _w((lambda *s: _rng.normal(s) * 0.05)(B, S, D)), 'w_r': _w((lambda *s: _rng.normal(s) * 0.05)(D)), 'w_gate': _w((lambda *s: _rng.normal(s) * 0.05)(D, F)), 'w_up': _w((lambda *s: _rng.normal(s) * 0.05)(D, F)), 'w_down': _w((lambda *s: _rng.normal(s) * 0.05)(F, D))}
    _B_in = _B_setup()
    return {'A_x': _A_in['x'], 'A_k_cache': _A_in['k_cache'], 'A_v_cache': _A_in['v_cache'], 'A_wq': _A_in['wq'], 'A_wo': _A_in['wo'], 'B_x': _B_in['x'], 'B_w_r': _B_in['w_r'], 'B_w_gate': _B_in['w_gate'], 'B_w_up': _B_in['w_up'], 'B_w_down': _B_in['w_down'], 'c': _w((lambda *s: _rng.normal(s) * 0.05)(1, 1024)), 'w_mod': _w((lambda *s: _rng.normal(s) * 0.05)(1024, 6 * 1024) * 1024 ** (-0.5))}

def reference(A_x, A_k_cache, A_v_cache, A_wq, A_wo, B_x, B_w_r, B_w_gate, B_w_up, B_w_down, c, w_mod):

    def _A_ref(x, k_cache, v_cache, wq, wo):
        B, Sq, D = x.shape
        H, Dh = (32, 128)
        q = (lambda x, *d: x.transpose(*d))((x @ wq).reshape(B, Sq, H, Dh), 0, 2, 1, 3)
        scores = jnp.einsum('bhqd,bhkd->bhqk', q, k_cache) * Dh ** (-0.5)
        p = _softmax(scores, axis=-1)
        o = jnp.einsum('bhqk,bhkd->bhqd', p, v_cache)
        return (lambda x, *d: x.transpose(*d))(o, 0, 2, 1, 3).reshape(B, Sq, H * Dh) @ wo

    def _B_ref(x, w_r, w_gate, w_up, w_down):
        B, S, D = x.shape
        C = 2
        r = x @ w_r
        idx = jnp.argsort(-r, axis=-1)[:, :C]
        idx_e = jnp.repeat(idx.reshape(B, C, 1), D, axis=2)
        x_sel = jnp.take_along_axis(x, idx_e, axis=1)
        g = _silu(x_sel @ w_gate)
        u = x_sel @ w_up
        y = g * u @ w_down
        r_sel = _sigmoid(jnp.take_along_axis(r, idx, axis=1))
        y = y * r_sel.reshape(B, C, 1)
        b_off = (jnp.arange(B) * S).reshape(B, 1)
        flat_idx = (idx + b_off).reshape(B * C)
        zero = (x * 0.0).reshape(B * S, D)
        upd = _scatter_add(zero, flat_idx, y.reshape(B * C, D), axis=0)
        return x + upd.reshape(B, S, D)
    x = A_x
    mod = (_silu(c) @ w_mod).reshape(c.shape[0], 6, 1, -1)
    sa, ca, ga, sb, cb, gb = (mod[:, 0].copy(), mod[:, 1].copy(), mod[:, 2].copy(), mod[:, 3].copy(), mod[:, 4].copy(), mod[:, 5].copy())
    h = _layernorm(x, axis=-1) * (1 + ca) + sa
    x = x + ga * _A_ref(h, A_k_cache, A_v_cache, A_wq, A_wo)
    h = _layernorm(x, axis=-1) * (1 + cb) + sb
    x = x + gb * _B_ref(h, B_w_r, B_w_gate, B_w_up, B_w_down)
    return x
```

```python
import jax
import jax.numpy as jnp
from jax import lax
import jax.experimental.pallas as pl
import jax.experimental.pallas.tpu as pltpu

S = 2048
D = 1024
H = 32
DH = 128
F = 3584
EPS = 1e-5
HH = H // 2

TQ = 256
KR = 512
P_ROWS = 256
P_HEADS = 4
QU_ROWS = 512
QU_PER_IT = (H - P_HEADS) * (S // QU_ROWS) // HH
B_ROWS = S // HH
E_ROWS = 256
PACE = 24
GRP = 16

Q_SCALE = float(DH) ** -0.5 * 1.4426950408889634

f32 = jnp.float32
bf16 = jnp.bfloat16


def _r(x):
    return x.astype(bf16).astype(f32)


def _recip(x):
    r0 = pl.reciprocal(x, approx=True)
    return r0 * (2.0 - x * r0)


def _pace(v):
    t = v[0:8, 0:128]
    for _ in range(PACE):
        t = jnp.minimum(t, jnp.max(t, axis=1, keepdims=True))
    top = t if v.shape[1] == 128 else jnp.concatenate([t, v[0:8, 128:]], axis=1)
    return jnp.concatenate([top, v[8:, :]], axis=0)


def _attention(q_ref, k_ref, v_ref, o_ref):
    n = S // TQ

    def scores(c):
        q = q_ref[c * TQ:(c + 1) * TQ, :]
        return lax.dot_general(q, k_ref[...], (((1,), (1,)), ((), ())),
                               preferred_element_type=f32)

    def finish(c, s):
        m = jnp.max(s, axis=1, keepdims=True)
        o = None
        lp = None
        for r in range(S // KR):
            p = jnp.exp2(s[:, r * KR:(r + 1) * KR] - m)
            ps = [p[:, j * 128:(j + 1) * 128] for j in range(KR // 128)]
            t = ps[0]
            for x in ps[1:]:
                t = t + x
            lp = t if lp is None else lp + t
            ps[-1] = jnp.minimum(ps[-1], t)
            p = jnp.concatenate(ps, axis=1)
            d = jnp.dot(p.astype(bf16), v_ref[r * KR:(r + 1) * KR, :],
                        preferred_element_type=f32)
            o = d if o is None else o + d
        l = jnp.sum(lp, axis=1, keepdims=True)
        o_ref[c * TQ:(c + 1) * TQ, :] = (o * _recip(l)).astype(bf16)

    s = scores(0)
    for c in range(n):
        s_next = scores(c + 1) if c + 1 < n else None
        finish(c, s)
        s = s_next


def _kernel(x_hbm, k_hbm, v_hbm, wq_hbm, wo_hbm, wr_hbm, wg_hbm, wu_hbm, wd_hbm, c_hbm,
            wm_hbm, out_hbm,
            x_v, h_v, x2_v, out_v, q_v, olo_v, ohi_v, part_v, wq_v, wo_v, wma_v, wg_v, wu_v,
            wd_v, k_v, v_v, c_v, wr_v, mod_v, top_v, fix_v,
            sem_small, sem_wma, sem_x, sem_wq, sem_kv, sem_bg, sem_out, sem_fix):
    n_p = S // P_ROWS
    n_e = S // E_ROWS
    pq = P_HEADS * DH

    def cp_c():
        return pltpu.make_async_copy(c_hbm, c_v, sem_small.at[0])

    def cp_wr():
        return pltpu.make_async_copy(wr_hbm, wr_v, sem_small.at[1])

    def cp_wma(j):
        return pltpu.make_async_copy(wm_hbm.at[:, pl.ds(j * 512, 512)],
                                     wma_v.at[:, pl.ds(j * 512, 512)], sem_wma.at[j])

    def cp_x(i):
        return pltpu.make_async_copy(x_hbm.at[0, pl.ds(i * P_ROWS, P_ROWS), :],
                                     x_v.at[pl.ds(i * P_ROWS, P_ROWS), :], sem_x.at[i])

    wq_cols = ((0, pq), (pq, 1024), (pq + 1024, H * DH - pq - 1024))

    def cp_wq(j):
        lo, n = wq_cols[j]
        return pltpu.make_async_copy(wq_hbm.at[:, pl.ds(lo, n)], wq_v.at[:, pl.ds(lo, n)],
                                     sem_wq.at[j])

    def cp_k(h, slot):
        return pltpu.make_async_copy(k_hbm.at[0, h], k_v.at[slot], sem_kv.at[slot])

    def cp_v(h, slot):
        return pltpu.make_async_copy(v_hbm.at[0, h], v_v.at[slot], sem_kv.at[2 + slot])

    def cp_rows(src, dst, i, n, sem):
        return pltpu.make_async_copy(src.at[pl.ds(i * n, n), :], dst.at[pl.ds(i * n, n), :], sem)

    def cp_wmb():
        return pltpu.make_async_copy(wm_hbm.at[:, pl.ds(2 * D, 4 * D)], wq_v, sem_wq.at[0])

    def cp_out(i):
        return pltpu.make_async_copy(out_v.at[pl.ds(i * E_ROWS, E_ROWS), :],
                                     out_hbm.at[0, pl.ds(i * E_ROWS, E_ROWS), :], sem_out)

    cp_c().start()
    for j in range(4):
        cp_wma(j).start()
    cp_x(0).start()
    cp_wq(0).start()
    for i in range(1, n_p):
        cp_x(i).start()
    cp_k(0, 0).start()
    cp_v(0, 0).start()
    cp_wq(1).start()
    cp_wq(2).start()
    cp_wr().start()

    cp_c().wait()
    cf = c_v[...].astype(f32)
    sc = jnp.broadcast_to(_r(cf * jax.nn.sigmoid(cf)), (GRP, D)).astype(bf16)
    for j in range(4):
        cp_wma(j).wait()
        mj = jnp.dot(sc, wma_v[:, j * 512:(j + 1) * 512], preferred_element_type=f32)
        mj = _r(mj[0:8, :])
        if j >= 2:
            mj = _r(1.0 + mj)
        mod_v[:, j * 512:(j + 1) * 512] = mj

    def ln1(i):
        rows = pl.ds(pl.multiple_of(i * P_ROWS, P_ROWS), P_ROWS)
        x = x_v[rows, :].astype(f32)
        mu = jnp.sum(x, axis=1, keepdims=True) * (1.0 / D)
        d = x - mu
        var = jnp.sum(d * d, axis=1, keepdims=True) * (1.0 / D)
        n = d * lax.rsqrt(var + EPS)
        h_v[rows, :] = (n * mod_v[0:1, D:2 * D] + mod_v[0:1, 0:D]).astype(bf16)

    cp_x(0).wait()
    ln1(0)
    cp_wq(0).wait()

    def p_body(i, carry):
        nxt = jnp.minimum(i + 1, n_p - 1)

        @pl.when(i + 1 < n_p)
        def _():
            cp_x(i + 1).wait()

        rows = pl.ds(pl.multiple_of(i * P_ROWS, P_ROWS), P_ROWS)
        q = jnp.dot(h_v[rows, :], wq_v[:, 0:pq], preferred_element_type=f32) * Q_SCALE
        ln1(nxt)
        for j in range(P_HEADS):
            q_v[j, rows, :] = q[:, j * DH:(j + 1) * DH].astype(bf16)
        return carry

    lax.fori_loop(0, n_p, p_body, 0)
    cp_wq(1).wait()

    def kv_step(h):
        slot = h % 2
        cp_k(h, slot).wait()
        cp_v(h, slot).wait()

        @pl.when(h + 1 < H)
        def _():
            cp_k(h + 1, 1 - slot).start()
            cp_v(h + 1, 1 - slot).start()

        return slot

    def a_body(it, carry):
        slot = kv_step(it)
        cp_rows(wo_hbm, wo_v, it, H * DH // HH, sem_bg.at[0]).start()
        cp_rows(wg_hbm, wg_v, it, D // HH, sem_bg.at[1]).start()
        cp_rows(wu_hbm, wu_v, it, D // HH, sem_bg.at[2]).start()
        cp_rows(wd_hbm, wd_v, it, F // HH, sem_bg.at[3]).start()

        @pl.when(it == 1)
        def _():
            cp_wq(2).wait()

        _attention(q_v.at[it], k_v.at[slot], v_v.at[slot], olo_v.at[it])
        for u in range(QU_PER_IT):
            g = it * QU_PER_IT + u
            hd = P_HEADS + g // (S // QU_ROWS)
            rows = pl.ds(pl.multiple_of((g % (S // QU_ROWS)) * QU_ROWS, QU_ROWS), QU_ROWS)
            cols = pl.ds(pl.multiple_of(hd * DH, DH), DH)
            q = jnp.dot(h_v[rows, :], wq_v[:, cols], preferred_element_type=f32)
            if u == 0:
                q = _pace(q)
            q_v[hd, rows, :] = (q * Q_SCALE).astype(bf16)
        return carry

    lax.fori_loop(0, HH, a_body, 0)

    pltpu.make_async_copy(wo_v, wo_v, sem_bg.at[0]).wait()
    cp_wmb().start()

    def b_body(it, carry):
        slot = kv_step(HH + it)
        _attention(q_v.at[HH + it], k_v.at[slot], v_v.at[slot], ohi_v.at[it])
        rows = pl.ds(pl.multiple_of(it * B_ROWS, B_ROWS), B_ROWS)
        lhs = jnp.concatenate([olo_v[j, rows, :] for j in range(HH)], axis=1)
        for u in range(4):
            part = jnp.dot(lhs, wo_v[0:HH * DH, u * 256:(u + 1) * 256], preferred_element_type=f32)
            if u == 0:
                part = _pace(part)
            part_v[rows, u * 256:(u + 1) * 256] = part
        return carry

    lax.fori_loop(0, HH, b_body, 0)

    cp_wmb().wait()
    cp_wr().wait()
    mb = _r(jnp.dot(sc, wq_v[...], preferred_element_type=f32)[0:8, :])
    mod_v[:, 2 * D:4 * D] = mb[:, 0:2 * D]
    mod_v[:, 4 * D:5 * D] = _r(1.0 + mb[:, 2 * D:3 * D])
    mod_v[:, 5 * D:6 * D] = mb[:, 3 * D:4 * D]
    mod_v[:, 6 * D:7 * D] = jnp.broadcast_to(wr_v[...].astype(f32).reshape(1, D), (8, D))
    int_min = jnp.iinfo(jnp.int32).min
    top_v[...] = jnp.full(top_v.shape, int_min, jnp.int32)

    def router(h2):
        return _r(jnp.sum(h2 * mod_v[0:1, 6 * D:7 * D], axis=1, keepdims=True))

    def finish_rows(c, valid):
        r0 = pl.multiple_of(c * E_ROWS, E_ROWS)
        rows = pl.ds(r0, E_ROWS)
        x2 = _r(x_v[rows, :].astype(f32) + mod_v[0:1, 2 * D:3 * D] * part_v[rows, :])
        mu = jnp.sum(x2, axis=1, keepdims=True) * (1.0 / D)
        dc = x2 - mu
        var = _r(jnp.sum(dc * dc, axis=1, keepdims=True) * (1.0 / D))
        den = _r(jnp.sqrt(_r(var + EPS)))
        n = _r(_r(x2 - _r(mu)) * _recip(den))
        h2 = _r(_r(n * mod_v[0:1, 4 * D:5 * D]) + mod_v[0:1, 3 * D:4 * D])
        x2_v[rows, :] = x2.astype(bf16)
        h_v[rows, :] = h2.astype(bf16)
        out_v[rows, :] = (x2 + _r(mod_v[0:1, 5 * D:6 * D] * h2)).astype(bf16)
        r = router(h2) + 0.0
        r = jnp.where(r != r, -jnp.inf, r)
        bits = pltpu.bitcast(jnp.broadcast_to(r, (E_ROWS, 128)), jnp.int32)
        bits = jnp.where(bits < 0, bits ^ 0x7FFF0000, bits)
        idx = r0 + lax.broadcasted_iota(jnp.int32, (E_ROWS, 128), 0)
        key = bits | (0xFFFF - idx)
        if valid is not None:
            key = jnp.where(valid, key, int_min)
        m1 = top_v[0]
        m2 = top_v[1]
        for g in range(E_ROWS // 8):
            kg = key[g * 8:(g + 1) * 8, :]
            m2 = jnp.maximum(m2, jnp.minimum(m1, kg))
            m1 = jnp.maximum(m1, kg)
        top_v[0] = m1
        top_v[1] = m2

    def e_body(c, carry):
        @pl.when(c >= 2)
        def _():
            cp_out(c - 2).start()

        rows = pl.ds(pl.multiple_of(c * E_ROWS, E_ROWS), E_ROWS)
        prev = part_v[rows, :]
        lhs = jnp.concatenate([ohi_v[j, rows, :] for j in range(HH)], axis=1)
        acc = prev + jnp.dot(lhs, wo_v[HH * DH:H * DH, :], preferred_element_type=f32)
        finish_rows(jnp.maximum(c - 1, 0), c > 0)
        part_v[rows, :] = acc
        return carry

    lax.fori_loop(0, n_e, e_body, 0)
    cp_out(n_e - 2).start()
    finish_rows(n_e - 1, None)
    cp_out(n_e - 1).start()

    m1 = top_v[0]
    m2 = top_v[1]
    t1 = jnp.max(m1, axis=0, keepdims=True)
    t2 = jnp.max(jnp.where(m1 == t1, m2, m1), axis=0, keepdims=True)
    i1 = 0xFFFF - (t1[0, 0] & 0xFFFF)
    i2 = 0xFFFF - (t2[0, 0] & 0xFFFF)
    g1 = pl.multiple_of((i1 // GRP) * GRP, GRP)
    g2 = pl.multiple_of((i2 // GRP) * GRP, GRP)

    pltpu.make_async_copy(wg_v, wg_v, sem_bg.at[1]).wait()
    pltpu.make_async_copy(wu_v, wu_v, sem_bg.at[2]).wait()
    pltpu.make_async_copy(wd_v, wd_v, sem_bg.at[3]).wait()

    xs = jnp.concatenate([h_v[pl.ds(g1, GRP), :], h_v[pl.ds(g2, GRP), :]], axis=0)
    y = None
    for j in range(F // 512):
        fc = slice(j * 512, (j + 1) * 512)
        g = _r(jnp.dot(xs, wg_v[:, fc], preferred_element_type=f32))
        u = _r(jnp.dot(xs, wu_v[:, fc], preferred_element_type=f32))
        a = (_r(g * jax.nn.sigmoid(g)) * u).astype(bf16)
        d = jnp.dot(a, wd_v[fc, :], preferred_element_type=f32)
        y = d if y is None else y + d
    h2 = xs.astype(f32)
    x2 = jnp.concatenate([x2_v[pl.ds(g1, GRP), :], x2_v[pl.ds(g2, GRP), :]], axis=0).astype(f32)
    upd = _r(_r(y) * _r(jax.nn.sigmoid(router(h2))))
    loc = lax.broadcasted_iota(jnp.int32, (2 * GRP, D), 0)
    row = jnp.where(loc < GRP, g1 + loc, g2 + loc - GRP)
    sel = jnp.logical_or(row == i1, row == i2)
    hb = _r(h2 + jnp.where(sel, upd, 0.0))
    fix_v[...] = (x2 + _r(mod_v[0:1, 5 * D:6 * D] * hb)).astype(bf16)

    pltpu.make_async_copy(out_v, out_v, sem_out).wait()
    fix1 = pltpu.make_async_copy(fix_v.at[pl.ds(0, GRP), :], out_hbm.at[0, pl.ds(g1, GRP), :],
                                 sem_fix.at[0])
    fix2 = pltpu.make_async_copy(fix_v.at[pl.ds(GRP, GRP), :], out_hbm.at[0, pl.ds(g2, GRP), :],
                                 sem_fix.at[1])
    fix1.start()

    @pl.when(g2 != g1)
    def _():
        fix2.start()
        fix2.wait()

    fix1.wait()


@jax.jit
def pallas_adaLN_cond__mha_block_cached__moe_arch_mod__prompt_kernel(
    A_x: jax.Array,
    A_k_cache: jax.Array,
    A_v_cache: jax.Array,
    A_wq: jax.Array,
    A_wo: jax.Array,
    B_x: jax.Array,
    B_w_r: jax.Array,
    B_w_gate: jax.Array,
    B_w_up: jax.Array,
    B_w_down: jax.Array,
    c: jax.Array,
    w_mod: jax.Array,
):
    del B_x
    vm = pltpu.VMEM
    dma = pltpu.SemaphoreType.DMA
    scratch = [
        vm((S, D), bf16),
        vm((S, D), bf16),
        vm((S, D), bf16),
        vm((S, D), bf16),
        vm((H, S, DH), bf16),
        vm((HH, S, DH), bf16),
        vm((HH, S, DH), bf16),
        vm((S, D), f32),
        vm((D, H * DH), bf16),
        vm((H * DH, D), bf16),
        vm((D, 2 * D), bf16),
        vm((D, F), bf16),
        vm((D, F), bf16),
        vm((F, D), bf16),
        vm((2, S, DH), bf16),
        vm((2, S, DH), bf16),
        vm((1, D), bf16),
        vm((D,), bf16),
        vm((8, 7 * D), f32),
        vm((2, 8, 128), jnp.int32),
        vm((2 * GRP, D), bf16),
        dma((2,)), dma((4,)), dma((S // P_ROWS,)), dma((3,)), dma((4,)), dma((4,)),
        dma(()), dma((2,)),
    ]
    return pl.pallas_call(
        _kernel,
        in_specs=[pl.BlockSpec(memory_space=pl.ANY)] * 11,
        out_specs=pl.BlockSpec(memory_space=pl.ANY),
        out_shape=jax.ShapeDtypeStruct(A_x.shape, A_x.dtype),
        scratch_shapes=scratch,
        compiler_params=pltpu.CompilerParams(vmem_limit_bytes=124 * 1024 * 1024),
        name="adaln_mha_moe",
    )(A_x, A_k_cache, A_v_cache, A_wq, A_wo, B_w_r, B_w_gate, B_w_up, B_w_down, c, w_mod)
```

```python
import jax
import jax.numpy as jnp
from jax import lax
import jax.experimental.pallas as pl
import jax.experimental.pallas.tpu as pltpu

S = 2048
D = 1024
H = 32
DH = 128
F = 3584
EPS = 1e-5
HH = H // 2

TQ = 256
KR = 512
P_ROWS = 256
P_HEADS = 4
QU_ROWS = 512
QU_PER_IT = (H - P_HEADS) * (S // QU_ROWS) // HH
B_ROWS = S // HH
E_ROWS = 128
PACE = 24
GRP = 16
FC = 512
P_LO, P_HI = 0.25, 0.97
E_LO0, E_LO1, E_HI, E_KEY = 0.15, 0.2, 0.88, 0.08

Q_SCALE = float(DH) ** -0.5 * 1.4426950408889634

f32 = jnp.float32
bf16 = jnp.bfloat16
u32 = jnp.uint32


def _r(x):
    return x.astype(bf16).astype(f32)


def _recip(x):
    r0 = pl.reciprocal(x, approx=True)
    return r0 * (2.0 - x * r0)


def _pace(v):
    t = v[0:8, 0:128]
    for _ in range(PACE):
        t = jnp.minimum(t, jnp.max(t, axis=1, keepdims=True))
    top = t if v.shape[1] == 128 else jnp.concatenate([t, v[0:8, 128:]], axis=1)
    return jnp.concatenate([top, v[8:, :]], axis=0)


def _tiles(v):
    u = pltpu.bitcast(v, u32)
    return [[u[a * 8:(a + 1) * 8, b * 128:(b + 1) * 128] for b in range(u.shape[1] // 128)]
            for a in range(u.shape[0] // 8)]


def _col_dots(k_tiles, rhs, n_tiles, never, deps):
    n_r = len(k_tiles) // 4
    n_i = k_tiles[0].shape[0] // GRP
    total = n_tiles * n_r * n_i
    at = {}
    for n, (pos, d) in enumerate(deps):
        at.setdefault((min(int(pos * total), total - 1), n % 4), []).append(d)
    outs = []
    for j in range(n_tiles):
        tl = list(k_tiles)
        for k in range(len(k_tiles)):
            base = (j * n_r + k // 4) * n_i
            if not any((base + i, k % 4) in at for i in range(n_i)):
                continue
            tu = pltpu.bitcast(tl[k], u32)
            parts = []
            for i in range(n_i):
                t = tu[i * 8:(i + 1) * 8, :]
                for d in at.get((base + i, k % 4), ()):
                    t = jnp.where(never, d, t)
                parts.append(t)
            tl[k] = pltpu.bitcast(jnp.concatenate(parts, axis=0), bf16)
        outs.append(jnp.dot(jnp.concatenate(tl, axis=1), rhs(j), preferred_element_type=f32))
    return outs


def _never(i):
    return jnp.full((8, 128), i, jnp.int32) > (1 << 20)


def _attention(q_ref, k_ref, v_ref, o_ref):
    n = S // TQ

    def scores(c):
        q = q_ref[c * TQ:(c + 1) * TQ, :]
        return lax.dot_general(q, k_ref[...], (((1,), (1,)), ((), ())),
                               preferred_element_type=f32)

    def finish(c, s):
        m = jnp.max(s, axis=1, keepdims=True)
        o = None
        lp = None
        for r in range(S // KR):
            p = jnp.exp2(s[:, r * KR:(r + 1) * KR] - m)
            ps = [p[:, j * 128:(j + 1) * 128] for j in range(KR // 128)]
            t = ps[0]
            for x in ps[1:]:
                t = t + x
            lp = t if lp is None else lp + t
            ps[-1] = jnp.minimum(ps[-1], t)
            p = jnp.concatenate(ps, axis=1)
            d = jnp.dot(p.astype(bf16), v_ref[r * KR:(r + 1) * KR, :],
                        preferred_element_type=f32)
            o = d if o is None else o + d
        l = jnp.sum(lp, axis=1, keepdims=True)
        o_ref[c * TQ:(c + 1) * TQ, :] = (o * _recip(l)).astype(bf16)

    s = scores(0)
    for c in range(n):
        s_next = scores(c + 1) if c + 1 < n else None
        finish(c, s)
        s = s_next


SEM_C, SEM_WR, SEM_WMA, SEM_X, SEM_WQ, SEM_KV, SEM_BG, SEM_OUT, SEM_FIX, SEM_WMB, N_SEM = (
    0, 1, 2, 6, 14, 17, 21, 25, 26, 28, 30)
SA, CA1, GA, SB, CB1, GB, WR = range(7)


def _kernel(x_hbm, k_hbm, v_hbm, wq_hbm, wo_hbm, wr_hbm, wg_hbm, wu_hbm, wd_hbm, c_hbm,
            wm_hbm, out_hbm,
            x_v, h_v, x2_v, out_v, q_v, olo_v, ohi_v, part_v, acc_v, wq_v, wo_v, wma_v, wg_v,
            wu_v, wd_v, k_v, v_v, c_v, wr_v, sc_v, mod_v, top_v, fix_v, sems):
    n_p = S // P_ROWS
    n_e = S // (2 * E_ROWS)
    pq = P_HEADS * DH

    def cp(src, dst, sem):
        return pltpu.make_async_copy(src, dst, sems.at[sem])

    def cp_c():
        return cp(c_hbm, c_v, SEM_C)

    def cp_wr():
        return cp(wr_hbm, wr_v, SEM_WR)

    def cp_wma(j):
        return cp(wm_hbm.at[:, pl.ds(j * 512, 512)], wma_v.at[:, pl.ds(j * 512, 512)], SEM_WMA + j)

    def cp_x(i):
        return cp(x_hbm.at[0, pl.ds(i * P_ROWS, P_ROWS), :], x_v.at[pl.ds(i * P_ROWS, P_ROWS), :],
                  SEM_X + i)

    wq_cols = ((0, pq), (pq, 1024), (pq + 1024, H * DH - pq - 1024))

    def cp_wq(j):
        lo, n = wq_cols[j]
        return cp(wq_hbm.at[:, pl.ds(lo, n)], wq_v.at[:, pl.ds(lo, n)], SEM_WQ + j)

    def cp_k(h, slot):
        return cp(k_hbm.at[0, h], k_v.at[slot], SEM_KV + slot)

    def cp_v(h, slot):
        return cp(v_hbm.at[0, h], v_v.at[slot], SEM_KV + 2 + slot)

    def cp_rows(src, dst, i, n, sem):
        return cp(src.at[pl.ds(i * n, n), :], dst.at[pl.ds(i * n, n), :], sem)

    def cp_wmb(j):
        return cp(wm_hbm.at[:, pl.ds((2 + 2 * j) * D, 2 * D)], wq_v.at[:, pl.ds(2 * j * D, 2 * D)],
                  SEM_WMB + j)

    def cp_out(i):
        return cp(out_v.at[pl.ds(i * E_ROWS, E_ROWS), :],
                  out_hbm.at[0, pl.ds(i * E_ROWS, E_ROWS), :], SEM_OUT)

    def mrow(k, n):
        m = mod_v[:, k * D:(k + 1) * D]
        return jnp.concatenate([m] * (n // 8), axis=0)

    cp_c().start()
    for j in range(4):
        cp_wma(j).start()
    cp_x(0).start()
    cp_wq(0).start()
    for i in range(1, n_p):
        cp_x(i).start()
    cp_k(0, 0).start()
    cp_v(0, 0).start()
    cp_wq(1).start()
    cp_wq(2).start()
    cp_wr().start()

    cp_c().wait()
    cf = c_v[...].astype(f32)
    sc_v[...] = jnp.broadcast_to(cf * jax.nn.sigmoid(cf), (GRP, D)).astype(bf16)

    def wma_body(j, carry):
        cp_wma(j).wait()
        cols = pl.ds(pl.multiple_of(j * 512, 512), 512)
        mj = jnp.dot(sc_v[...], wma_v[:, cols], preferred_element_type=f32)
        mod_v[:, cols] = _r(_r(mj[0:8, :]) + jnp.where(j >= 2, 1.0, 0.0))
        return carry

    lax.fori_loop(0, 4, wma_body, 0)

    def ln1(i):
        rows = pl.ds(pl.multiple_of(i * P_ROWS, P_ROWS), P_ROWS)
        x = x_v[rows, :].astype(f32)
        mu = jnp.sum(x, axis=1, keepdims=True) * (1.0 / D)
        d = x - mu
        var = jnp.sum(d * d, axis=1, keepdims=True) * (1.0 / D)
        n = d * lax.rsqrt(var + EPS)
        h = (n * mrow(CA1, P_ROWS) + mrow(SA, P_ROWS)).astype(bf16)
        h_v[rows, :] = h
        return h

    cp_x(0).wait()
    ln1(0)
    cp_wq(0).wait()

    def p_body(i, carry):
        @pl.when(i + 1 < n_p)
        def _():
            cp_x(i + 1).wait()

        rows = pl.ds(pl.multiple_of(i * P_ROWS, P_ROWS), P_ROWS)
        lhs = [h_v[rows, k * 128:(k + 1) * 128] for k in range(D // 128)]
        tl = [t for row in _tiles(ln1(jnp.minimum(i + 1, n_p - 1))) for t in row]
        deps = [(P_LO + (P_HI - P_LO) * n / len(tl), t) for n, t in enumerate(tl)]
        qs = _col_dots(lhs, lambda j: wq_v[:, j * DH:(j + 1) * DH], P_HEADS, _never(i), deps)
        for j in range(P_HEADS):
            q_v[j, rows, :] = (qs[j] * Q_SCALE).astype(bf16)
        return carry

    lax.fori_loop(0, n_p, p_body, 0)
    cp_wq(1).wait()

    def kv_wait(h):
        slot = h % 2
        cp_k(h, slot).wait()
        cp_v(h, slot).wait()
        return slot

    def kv_prefetch(h, slot):
        @pl.when(h + 1 < H)
        def _():
            cp_k(h + 1, 1 - slot).start()
            cp_v(h + 1, 1 - slot).start()

    def a_body(it, carry):
        @pl.when(it == 1)
        def _():
            cp_wq(2).wait()

        slot = kv_wait(it)
        kv_prefetch(it, slot)
        cp_rows(wo_hbm, wo_v, it, H * DH // HH, SEM_BG).start()
        cp_rows(wg_hbm, wg_v, it, D // HH, SEM_BG + 1).start()
        cp_rows(wu_hbm, wu_v, it, D // HH, SEM_BG + 2).start()
        cp_rows(wd_hbm, wd_v, it, F // HH, SEM_BG + 3).start()

        @pl.when(it == HH - 4)
        def _():
            cp_wmb(0).start()

        _attention(q_v.at[it], k_v.at[slot], v_v.at[slot], olo_v.at[it])
        for u in range(QU_PER_IT):
            g = it * QU_PER_IT + u
            hd = P_HEADS + g // (S // QU_ROWS)
            rows = pl.ds(pl.multiple_of((g % (S // QU_ROWS)) * QU_ROWS, QU_ROWS), QU_ROWS)
            cols = pl.ds(pl.multiple_of(hd * DH, DH), DH)
            q = jnp.dot(h_v[rows, :], wq_v[:, cols], preferred_element_type=f32)
            if u == 0:
                q = _pace(q)
            q_v[hd, rows, :] = (q * Q_SCALE).astype(bf16)
        return carry

    lax.fori_loop(0, HH, a_body, 0)

    cp(wo_v, wo_v, SEM_BG).wait()
    cp_wmb(0).wait()
    cp_wmb(1).start()

    def b_body(it, carry):
        @pl.when(it == HH // 2)
        def _():
            cp_wmb(1).wait()

        slot = kv_wait(HH + it)
        kv_prefetch(HH + it, slot)
        _attention(q_v.at[HH + it], k_v.at[slot], v_v.at[slot], ohi_v.at[it])
        rows = pl.ds(pl.multiple_of(it * B_ROWS, B_ROWS), B_ROWS)
        lhs = jnp.concatenate([olo_v[j, rows, :] for j in range(HH)], axis=1)
        one = jnp.where(it // 4 == CB1 - GA, 1.0, 0.0)
        mb = None
        for u in range(4):
            part = jnp.dot(lhs, wo_v[0:HH * DH, u * 256:(u + 1) * 256], preferred_element_type=f32)
            if u == 0:
                part = _pace(part)
            part_v[rows, u * 256:(u + 1) * 256] = part
            c0 = pl.multiple_of(it * 256 + (u // 2) * 128, 128)
            ks = slice((u % 2) * 512, (u % 2 + 1) * 512)
            d = jnp.dot(sc_v[:, ks], wq_v[ks, pl.ds(c0, 128)], preferred_element_type=f32)[0:8, :]
            if u % 2 == 0:
                mb = d
            else:
                mod_v[:, pl.ds(pl.multiple_of(GA * D + c0, 128), 128)] = _r(_r(mb + d) + one)
        return carry

    lax.fori_loop(0, HH, b_body, 0)

    cp_wr().wait()
    cp(wg_v, wg_v, SEM_BG + 1).wait()
    cp(wu_v, wu_v, SEM_BG + 2).wait()
    cp(wd_v, wd_v, SEM_BG + 3).wait()
    mod_v[:, WR * D:(WR + 1) * D] = jnp.broadcast_to(wr_v[...].astype(f32).reshape(1, D), (8, D))
    int_min = jnp.iinfo(jnp.int32).min
    top_v[...] = jnp.full(top_v.shape, int_min, jnp.int32)
    acc_v[...] = jnp.zeros(acc_v.shape, f32)

    def router_parts(h2):
        pr = h2 * mrow(WR, h2.shape[0])
        run = [pr[:, 0:128]]
        for b in range(1, D // 128):
            run.append(run[-1] + pr[:, b * 128:(b + 1) * 128])
        return run

    def finish_rows(r0, attn, valid, m1, m2, lo, hi):
        rows = pl.ds(r0, E_ROWS)
        x2 = _r(x_v[rows, :].astype(f32) + mrow(GA, E_ROWS) * attn)
        mu = jnp.sum(x2, axis=1, keepdims=True) * (1.0 / D)
        dc = x2 - mu
        var = _r(jnp.sum(dc * dc, axis=1, keepdims=True) * (1.0 / D))
        den = _r(jnp.sqrt(_r(var + EPS)))
        n = _r(_r(x2 - _r(mu)) * _recip(den))
        h2 = _r(_r(n * mrow(CB1, E_ROWS)) + mrow(SB, E_ROWS))
        x2_v[rows, :] = x2.astype(bf16)
        h_v[rows, :] = h2.astype(bf16)
        ob = (x2 + _r(mrow(GB, E_ROWS) * h2)).astype(bf16)
        out_v[rows, :] = ob
        run = router_parts(h2)
        r = _r(jnp.sum(run[-1], axis=1, keepdims=True)) + 0.0
        r = jnp.where(r != r, -jnp.inf, r)
        bits = pltpu.bitcast(jnp.broadcast_to(r, (E_ROWS, 128)), jnp.int32)
        bits = jnp.where(bits < 0, bits ^ 0x7FFF0000, bits)
        idx = r0 + lax.broadcasted_iota(jnp.int32, (E_ROWS, 128), 0)
        key = bits | (0xFFFF - idx)
        if valid is not None:
            key = jnp.where(valid, key, int_min)
        deps = []
        ot = _tiles(ob)
        n_t = len(ot) * len(ot[0])
        for p in range(len(ot)):
            for b in range(len(ot[0])):
                pos = lo + (hi - lo) * (p * len(ot[0]) + b) / n_t
                deps.append((pos, ot[p][b]))
                for g in (2 * p, 2 * p + 1):
                    deps.append((pos, pltpu.bitcast(run[b][g * 8:(g + 1) * 8, :], u32)))
            for g in (2 * p, 2 * p + 1):
                kg = key[g * 8:(g + 1) * 8, :]
                m2 = jnp.maximum(m2, jnp.minimum(m1, kg))
                m1 = jnp.maximum(m1, kg)
            deps.append((pos + E_KEY, pltpu.bitcast(m2, u32)))
        return m1, m2, deps

    def out_proj(r0, never, deps):
        rows = pl.ds(r0, E_ROWS)
        lhs = [ohi_v[j, rows, :] for j in range(HH)]
        ds = _col_dots(lhs, lambda j: wo_v[HH * DH:H * DH, j * 128:(j + 1) * 128], D // 128,
                       never, deps)
        return part_v[rows, :] + jnp.concatenate(ds, axis=1)

    def e_body(c, carry):
        @pl.when(c >= 2)
        def _():
            cp_out(2 * c - 3).start()

        @pl.when(c >= 1)
        def _():
            cp_out(2 * c - 2).start()

        never = _never(c)
        ra = pl.multiple_of(2 * c * E_ROWS, E_ROWS)
        rb = pl.multiple_of(ra + E_ROWS, E_ROWS)
        rp = pl.multiple_of(jnp.maximum(ra - E_ROWS, 0), E_ROWS)
        m1, m2, deps = finish_rows(rp, acc_v[...], c > 0, top_v[0], top_v[1], E_LO0, E_HI)
        attn = out_proj(ra, never, deps)
        m1, m2, deps = finish_rows(ra, attn, None, m1, m2, E_LO1, E_HI)
        acc_v[...] = out_proj(rb, never, deps)
        top_v[0] = m1
        top_v[1] = m2
        return carry

    lax.fori_loop(0, n_e, e_body, 0)
    cp_out(2 * n_e - 3).start()
    cp_out(2 * n_e - 2).start()
    m1, m2, _ = finish_rows(S - E_ROWS, acc_v[...], None, top_v[0], top_v[1], 0.0, 1.0)
    cp_out(2 * n_e - 1).start()

    t1 = jnp.max(m1, axis=0, keepdims=True)
    t2 = jnp.max(jnp.where(m1 == t1, m2, m1), axis=0, keepdims=True)
    i1 = 0xFFFF - (t1[0, 0] & 0xFFFF)
    i2 = 0xFFFF - (t2[0, 0] & 0xFFFF)
    g1 = pl.multiple_of((i1 // GRP) * GRP, GRP)
    g2 = pl.multiple_of((i2 // GRP) * GRP, GRP)

    xs = jnp.concatenate([h_v[pl.ds(g1, GRP), :], h_v[pl.ds(g2, GRP), :]], axis=0)

    def act(j):
        fc = slice(j * FC, (j + 1) * FC)
        g = _r(jnp.dot(xs, wg_v[:, fc], preferred_element_type=f32))
        u = _r(jnp.dot(xs, wu_v[:, fc], preferred_element_type=f32))
        return (_r(g * jax.nn.sigmoid(g)) * u).astype(bf16)

    y = None
    a = act(0)
    for j in range(F // FC):
        a_next = act(j + 1) if (j + 1) * FC < F else None
        d = jnp.dot(a, wd_v[j * FC:(j + 1) * FC, :], preferred_element_type=f32)
        y = d if y is None else y + d
        a = a_next
    h2 = xs.astype(f32)
    x2 = jnp.concatenate([x2_v[pl.ds(g1, GRP), :], x2_v[pl.ds(g2, GRP), :]], axis=0).astype(f32)
    r = _r(jnp.sum(router_parts(h2)[-1], axis=1, keepdims=True))
    upd = _r(_r(y) * _r(jax.nn.sigmoid(r)))
    loc = lax.broadcasted_iota(jnp.int32, (2 * GRP, D), 0)
    row = jnp.where(loc < GRP, g1 + loc, g2 + loc - GRP)
    sel = jnp.logical_or(row == i1, row == i2)
    hb = _r(h2 + jnp.where(sel, upd, 0.0))
    fix_v[...] = (x2 + _r(mrow(GB, 2 * GRP) * hb)).astype(bf16)

    cp(out_v, out_v, SEM_OUT).wait()
    fix1 = cp(fix_v.at[pl.ds(0, GRP), :], out_hbm.at[0, pl.ds(g1, GRP), :], SEM_FIX)
    fix2 = cp(fix_v.at[pl.ds(GRP, GRP), :], out_hbm.at[0, pl.ds(g2, GRP), :], SEM_FIX + 1)
    fix1.start()

    @pl.when(g2 != g1)
    def _():
        fix2.start()
        fix2.wait()

    fix1.wait()


@jax.jit
def pallas_adaLN_cond__mha_block_cached__moe_arch_mod__prompt_kernel(
    A_x: jax.Array,
    A_k_cache: jax.Array,
    A_v_cache: jax.Array,
    A_wq: jax.Array,
    A_wo: jax.Array,
    B_x: jax.Array,
    B_w_r: jax.Array,
    B_w_gate: jax.Array,
    B_w_up: jax.Array,
    B_w_down: jax.Array,
    c: jax.Array,
    w_mod: jax.Array,
):
    del B_x
    vm = pltpu.VMEM
    scratch = [
        vm((S, D), bf16),
        vm((S, D), bf16),
        vm((S, D), bf16),
        vm((S, D), bf16),
        vm((H, S, DH), bf16),
        vm((HH, S, DH), bf16),
        vm((HH, S, DH), bf16),
        vm((S, D), f32),
        vm((E_ROWS, D), f32),
        vm((D, H * DH), bf16),
        vm((H * DH, D), bf16),
        vm((D, 2 * D), bf16),
        vm((D, F), bf16),
        vm((D, F), bf16),
        vm((F, D), bf16),
        vm((2, S, DH), bf16),
        vm((2, S, DH), bf16),
        vm((1, D), bf16),
        vm((D,), bf16),
        vm((GRP, D), bf16),
        vm((8, 7 * D), f32),
        vm((2, 8, 128), jnp.int32),
        vm((2 * GRP, D), bf16),
        pltpu.SemaphoreType.DMA((N_SEM,)),
    ]
    return pl.pallas_call(
        _kernel,
        in_specs=[pl.BlockSpec(memory_space=pl.ANY)] * 11,
        out_specs=pl.BlockSpec(memory_space=pl.ANY),
        out_shape=jax.ShapeDtypeStruct(A_x.shape, A_x.dtype),
        scratch_shapes=scratch,
        compiler_params=pltpu.CompilerParams(vmem_limit_bytes=124 * 1024 * 1024,
                                             disable_bounds_checks=True),
        name="adaln_mha_moe",
    )(A_x, A_k_cache, A_v_cache, A_wq, A_wo, B_w_r, B_w_gate, B_w_up, B_w_down, c, w_mod)
```

```python
import jax
import jax.numpy as jnp
from jax import lax
import jax.experimental.pallas as pl
import jax.experimental.pallas.tpu as pltpu

S = 2048
D = 1024
H = 32
DH = 128
F = 3584
EPS = 1e-5
HH = H // 2

TQ = 256
KR = 512
P_ROWS = 256
P_HEADS = 4
QU_ROWS = 512
QU_PER_IT = (H - P_HEADS) * (S // QU_ROWS) // HH
B_ROWS = S // HH
E_ROWS = 128
PACE = 24
GRP = 16
FC = 512
P_LO, P_HI = 0.25, 0.97
E_LO0, E_LO1, E_HI, E_KEY = 0.15, 0.25, 0.97, 0.1

Q_SCALE = float(DH) ** -0.5 * 1.4426950408889634

f32 = jnp.float32
bf16 = jnp.bfloat16
u32 = jnp.uint32


def _r(x):
    return x.astype(bf16).astype(f32)


def _recip(x):
    r0 = pl.reciprocal(x, approx=True)
    return r0 * (2.0 - x * r0)


def _pace(v):
    t = v[0:8, 0:128]
    for _ in range(PACE):
        t = jnp.minimum(t, jnp.max(t, axis=1, keepdims=True))
    top = t if v.shape[1] == 128 else jnp.concatenate([t, v[0:8, 128:]], axis=1)
    return jnp.concatenate([top, v[8:, :]], axis=0)


def _tiles(v):
    u = pltpu.bitcast(v, u32)
    return [[u[a * 8:(a + 1) * 8, b * 128:(b + 1) * 128] for b in range(u.shape[1] // 128)]
            for a in range(u.shape[0] // 8)]


def _col_dots(k_tiles, rhs, n_tiles, never, deps):
    n_r = len(k_tiles) // 4
    n_i = k_tiles[0].shape[0] // GRP
    total = n_tiles * n_r * n_i
    at = {}
    for n, (pos, d) in enumerate(deps):
        at.setdefault((min(int(pos * total), total - 1), n % 4), []).append(d)
    outs = []
    for j in range(n_tiles):
        tl = list(k_tiles)
        for k in range(len(k_tiles)):
            base = (j * n_r + k // 4) * n_i
            if not any((base + i, k % 4) in at for i in range(n_i)):
                continue
            tu = pltpu.bitcast(tl[k], u32)
            parts = []
            for i in range(n_i):
                t = tu[i * 8:(i + 1) * 8, :]
                for d in at.get((base + i, k % 4), ()):
                    t = jnp.where(never, d, t)
                parts.append(t)
            tl[k] = pltpu.bitcast(jnp.concatenate(parts, axis=0), bf16)
        outs.append(jnp.dot(jnp.concatenate(tl, axis=1), rhs(j), preferred_element_type=f32))
    return outs


def _never(i):
    return jnp.full((8, 128), i, jnp.int32) > (1 << 20)


def _attention(q_ref, k_ref, v_ref, o_ref):
    n = S // TQ

    def scores(c):
        q = q_ref[c * TQ:(c + 1) * TQ, :]
        return lax.dot_general(q, k_ref[...], (((1,), (1,)), ((), ())),
                               preferred_element_type=f32)

    def finish(c, s):
        m = jnp.max(s, axis=1, keepdims=True)
        o = None
        lp = None
        for r in range(S // KR):
            p = jnp.exp2(s[:, r * KR:(r + 1) * KR] - m)
            ps = [p[:, j * 128:(j + 1) * 128] for j in range(KR // 128)]
            t = ps[0]
            for x in ps[1:]:
                t = t + x
            lp = t if lp is None else lp + t
            ps[-1] = jnp.minimum(ps[-1], t)
            p = jnp.concatenate(ps, axis=1)
            d = jnp.dot(p.astype(bf16), v_ref[r * KR:(r + 1) * KR, :],
                        preferred_element_type=f32)
            o = d if o is None else o + d
        l = jnp.sum(lp, axis=1, keepdims=True)
        o_ref[c * TQ:(c + 1) * TQ, :] = (o * _recip(l)).astype(bf16)

    s = scores(0)
    for c in range(n):
        s_next = scores(c + 1) if c + 1 < n else None
        finish(c, s)
        s = s_next


SEM_C, SEM_WR, SEM_WMA, SEM_X, SEM_WQ, SEM_KV, SEM_BG, SEM_OUT, SEM_FIX, SEM_WMB, N_SEM = (
    0, 1, 2, 6, 14, 17, 21, 25, 26, 28, 30)
SA, CA1, GA, SB, CB1, GB, WR = range(7)


def _kernel(x_hbm, k_hbm, v_hbm, wq_hbm, wo_hbm, wr_hbm, wg_hbm, wu_hbm, wd_hbm, c_hbm,
            wm_hbm, out_hbm,
            x_v, h_v, x2_v, out_v, q_v, olo_v, ohi_v, part_v, acc_v, wq_v, wo_v, wma_v, wg_v,
            wu_v, wd_v, k_v, v_v, c_v, wr_v, sc_v, mod_v, top_v, rp_v, fix_v, sems):
    n_p = S // P_ROWS
    n_e = S // (2 * E_ROWS)
    pq = P_HEADS * DH

    def cp(src, dst, sem):
        return pltpu.make_async_copy(src, dst, sems.at[sem])

    def cp_c():
        return cp(c_hbm, c_v, SEM_C)

    def cp_wr():
        return cp(wr_hbm, wr_v, SEM_WR)

    def cp_wma(j):
        return cp(wm_hbm.at[:, pl.ds(j * 512, 512)], wma_v.at[:, pl.ds(j * 512, 512)], SEM_WMA + j)

    def cp_x(i):
        return cp(x_hbm.at[0, pl.ds(i * P_ROWS, P_ROWS), :], x_v.at[pl.ds(i * P_ROWS, P_ROWS), :],
                  SEM_X + i)

    wq_cols = ((0, pq), (pq, 1024), (pq + 1024, H * DH - pq - 1024))

    def cp_wq(j):
        lo, n = wq_cols[j]
        return cp(wq_hbm.at[:, pl.ds(lo, n)], wq_v.at[:, pl.ds(lo, n)], SEM_WQ + j)

    def cp_k(h, slot):
        return cp(k_hbm.at[0, h], k_v.at[slot], SEM_KV + slot)

    def cp_v(h, slot):
        return cp(v_hbm.at[0, h], v_v.at[slot], SEM_KV + 2 + slot)

    def cp_rows(src, dst, i, n, sem):
        return cp(src.at[pl.ds(i * n, n), :], dst.at[pl.ds(i * n, n), :], sem)

    def cp_wmb(j):
        return cp(wm_hbm.at[:, pl.ds((2 + 2 * j) * D, 2 * D)], wq_v.at[:, pl.ds(2 * j * D, 2 * D)],
                  SEM_WMB + j)

    def cp_out(i):
        return cp(out_v.at[pl.ds(i * E_ROWS, E_ROWS), :],
                  out_hbm.at[0, pl.ds(i * E_ROWS, E_ROWS), :], SEM_OUT)

    def mrow(k, n):
        m = mod_v[:, k * D:(k + 1) * D]
        return jnp.concatenate([m] * (n // 8), axis=0)

    cp_c().start()
    for j in range(4):
        cp_wma(j).start()
    cp_x(0).start()
    cp_wq(0).start()
    for i in range(1, n_p):
        cp_x(i).start()
    cp_k(0, 0).start()
    cp_v(0, 0).start()
    cp_wq(1).start()
    cp_wq(2).start()
    cp_wr().start()

    cp_c().wait()
    cf = c_v[...].astype(f32)
    sc_v[...] = jnp.broadcast_to(cf * jax.nn.sigmoid(cf), (GRP, D)).astype(bf16)

    def wma_body(j, carry):
        cp_wma(j).wait()
        cols = pl.ds(pl.multiple_of(j * 512, 512), 512)
        mj = jnp.dot(sc_v[...], wma_v[:, cols], preferred_element_type=f32)
        mod_v[:, cols] = _r(_r(mj[0:8, :]) + jnp.where(j >= 2, 1.0, 0.0))
        return carry

    lax.fori_loop(0, 4, wma_body, 0)

    def ln1(i):
        rows = pl.ds(pl.multiple_of(i * P_ROWS, P_ROWS), P_ROWS)
        x = x_v[rows, :].astype(f32)
        mu = jnp.sum(x, axis=1, keepdims=True) * (1.0 / D)
        d = x - mu
        var = jnp.sum(d * d, axis=1, keepdims=True) * (1.0 / D)
        n = d * lax.rsqrt(var + EPS)
        h = (n * mrow(CA1, P_ROWS) + mrow(SA, P_ROWS)).astype(bf16)
        h_v[rows, :] = h
        return h

    cp_x(0).wait()
    ln1(0)
    cp_wq(0).wait()

    def p_body(i, carry):
        @pl.when(i + 1 < n_p)
        def _():
            cp_x(i + 1).wait()

        rows = pl.ds(pl.multiple_of(i * P_ROWS, P_ROWS), P_ROWS)
        lhs = [h_v[rows, k * 128:(k + 1) * 128] for k in range(D // 128)]
        tl = [t for row in _tiles(ln1(jnp.minimum(i + 1, n_p - 1))) for t in row]
        deps = [(P_LO + (P_HI - P_LO) * n / len(tl), t) for n, t in enumerate(tl)]
        qs = _col_dots(lhs, lambda j: wq_v[:, j * DH:(j + 1) * DH], P_HEADS, _never(i), deps)
        for j in range(P_HEADS):
            q_v[j, rows, :] = (qs[j] * Q_SCALE).astype(bf16)
        return carry

    lax.fori_loop(0, n_p, p_body, 0)
    cp_wq(1).wait()

    def kv_wait(h):
        slot = h % 2
        cp_k(h, slot).wait()
        cp_v(h, slot).wait()
        return slot

    def kv_prefetch(h, slot):
        @pl.when(h + 1 < H)
        def _():
            cp_k(h + 1, 1 - slot).start()
            cp_v(h + 1, 1 - slot).start()

    def a_body(it, carry):
        @pl.when(it == 1)
        def _():
            cp_wq(2).wait()

        slot = kv_wait(it)
        kv_prefetch(it, slot)
        cp_rows(wo_hbm, wo_v, it, H * DH // HH, SEM_BG).start()
        cp_rows(wg_hbm, wg_v, it, D // HH, SEM_BG + 1).start()
        cp_rows(wu_hbm, wu_v, it, D // HH, SEM_BG + 2).start()
        cp_rows(wd_hbm, wd_v, it, F // HH, SEM_BG + 3).start()

        @pl.when(it == HH - 4)
        def _():
            cp_wmb(0).start()

        _attention(q_v.at[it], k_v.at[slot], v_v.at[slot], olo_v.at[it])
        for u in range(QU_PER_IT):
            g = it * QU_PER_IT + u
            hd = P_HEADS + g // (S // QU_ROWS)
            rows = pl.ds(pl.multiple_of((g % (S // QU_ROWS)) * QU_ROWS, QU_ROWS), QU_ROWS)
            cols = pl.ds(pl.multiple_of(hd * DH, DH), DH)
            q = jnp.dot(h_v[rows, :], wq_v[:, cols], preferred_element_type=f32)
            if u == 0:
                q = _pace(q)
            q_v[hd, rows, :] = (q * Q_SCALE).astype(bf16)
        return carry

    lax.fori_loop(0, HH, a_body, 0)

    cp(wo_v, wo_v, SEM_BG).wait()
    cp_wmb(0).wait()
    cp_wmb(1).start()

    def b_body(it, carry):
        @pl.when(it == HH // 2)
        def _():
            cp_wmb(1).wait()

        slot = kv_wait(HH + it)
        kv_prefetch(HH + it, slot)
        _attention(q_v.at[HH + it], k_v.at[slot], v_v.at[slot], ohi_v.at[it])
        rows = pl.ds(pl.multiple_of(it * B_ROWS, B_ROWS), B_ROWS)
        lhs = jnp.concatenate([olo_v[j, rows, :] for j in range(HH)], axis=1)
        one = jnp.where(it // 4 == CB1 - GA, 1.0, 0.0)
        mb = None
        for u in range(4):
            part = jnp.dot(lhs, wo_v[0:HH * DH, u * 256:(u + 1) * 256], preferred_element_type=f32)
            if u == 0:
                part = _pace(part)
            part_v[rows, u * 256:(u + 1) * 256] = part
            c0 = pl.multiple_of(it * 256 + (u // 2) * 128, 128)
            ks = slice((u % 2) * 512, (u % 2 + 1) * 512)
            d = jnp.dot(sc_v[:, ks], wq_v[ks, pl.ds(c0, 128)], preferred_element_type=f32)[0:8, :]
            if u % 2 == 0:
                mb = d
            else:
                mod_v[:, pl.ds(pl.multiple_of(GA * D + c0, 128), 128)] = _r(_r(mb + d) + one)
        return carry

    lax.fori_loop(0, HH, b_body, 0)

    cp_wr().wait()
    cp(wg_v, wg_v, SEM_BG + 1).wait()
    cp(wu_v, wu_v, SEM_BG + 2).wait()
    cp(wd_v, wd_v, SEM_BG + 3).wait()
    mod_v[:, WR * D:(WR + 1) * D] = jnp.broadcast_to(wr_v[...].astype(f32).reshape(1, D), (8, D))
    int_min = jnp.iinfo(jnp.int32).min
    top_v[...] = jnp.full(top_v.shape, int_min, jnp.int32)
    acc_v[...] = jnp.zeros(acc_v.shape, f32)
    rp_v[...] = jnp.zeros(rp_v.shape, f32)

    def router_parts(h2):
        pr = h2 * mrow(WR, h2.shape[0])
        run = [pr[:, 0:128]]
        for b in range(1, D // 128):
            run.append(run[-1] + pr[:, b * 128:(b + 1) * 128])
        return run

    def finish_rows(r0, attn, lo, hi):
        rows = pl.ds(r0, E_ROWS)
        x2 = _r(x_v[rows, :].astype(f32) + mrow(GA, E_ROWS) * attn)
        mu = jnp.sum(x2, axis=1, keepdims=True) * (1.0 / D)
        dc = x2 - mu
        var = _r(jnp.sum(dc * dc, axis=1, keepdims=True) * (1.0 / D))
        den = _r(jnp.sqrt(_r(var + EPS)))
        n = _r(_r(x2 - _r(mu)) * _recip(den))
        h2 = _r(_r(n * mrow(CB1, E_ROWS)) + mrow(SB, E_ROWS))
        x2_v[rows, :] = x2.astype(bf16)
        h_v[rows, :] = h2.astype(bf16)
        ob = (x2 + _r(mrow(GB, E_ROWS) * h2)).astype(bf16)
        out_v[rows, :] = ob
        run = router_parts(h2)
        deps = []
        ot = _tiles(ob)
        n_t = len(ot) * len(ot[0])
        for p in range(len(ot)):
            for b in range(len(ot[0])):
                pos = lo + (hi - lo) * (p * len(ot[0]) + b) / n_t
                deps.append((pos, ot[p][b]))
                for g in (2 * p, 2 * p + 1):
                    deps.append((pos, pltpu.bitcast(run[b][g * 8:(g + 1) * 8, :], u32)))
        return run[-1], deps

    def score_rows(r0, rp, valid, m1, m2):
        r = _r(jnp.sum(rp, axis=1, keepdims=True)) + 0.0
        r = jnp.where(r != r, -jnp.inf, r)
        bits = pltpu.bitcast(jnp.broadcast_to(r, (E_ROWS, 128)), jnp.int32)
        bits = jnp.where(bits < 0, bits ^ 0x7FFF0000, bits)
        idx = r0 + lax.broadcasted_iota(jnp.int32, (E_ROWS, 128), 0)
        key = bits | (0xFFFF - idx)
        if valid is not None:
            key = jnp.where(valid, key, int_min)
        for g in range(E_ROWS // 8):
            kg = key[g * 8:(g + 1) * 8, :]
            m2 = jnp.maximum(m2, jnp.minimum(m1, kg))
            m1 = jnp.maximum(m1, kg)
        return m1, m2

    def out_proj(r0, never, deps):
        rows = pl.ds(r0, E_ROWS)
        lhs = [ohi_v[j, rows, :] for j in range(HH)]
        ds = _col_dots(lhs, lambda j: wo_v[HH * DH:H * DH, j * 128:(j + 1) * 128], D // 128,
                       never, deps)
        return part_v[rows, :] + jnp.concatenate(ds, axis=1)

    def e_body(c, carry):
        @pl.when(c >= 2)
        def _():
            cp_out(2 * c - 3).start()

        @pl.when(c >= 1)
        def _():
            cp_out(2 * c - 2).start()

        never = _never(c)
        ra = pl.multiple_of(2 * c * E_ROWS, E_ROWS)
        rb = pl.multiple_of(ra + E_ROWS, E_ROWS)
        rp = pl.multiple_of(jnp.maximum(ra - E_ROWS, 0), E_ROWS)
        m1, m2 = score_rows(ra - 3 * E_ROWS, rp_v[0], c >= 2, top_v[0], top_v[1])
        m1, m2 = score_rows(ra - 2 * E_ROWS, rp_v[1], c >= 1, m1, m2)
        top_v[0] = m1
        top_v[1] = m2
        rp_v[0], deps = finish_rows(rp, acc_v[...], E_LO0, E_HI)
        if E_KEY is not None:
            deps.append((E_KEY, pltpu.bitcast(m2, u32)))
        attn = out_proj(ra, never, deps)
        rp_v[1], deps = finish_rows(ra, attn, E_LO1, E_HI)
        acc_v[...] = out_proj(rb, never, deps)
        return carry

    lax.fori_loop(0, n_e, e_body, 0)
    cp_out(2 * n_e - 3).start()
    cp_out(2 * n_e - 2).start()
    m1, m2 = score_rows(S - 3 * E_ROWS, rp_v[0], None, top_v[0], top_v[1])
    m1, m2 = score_rows(S - 2 * E_ROWS, rp_v[1], None, m1, m2)
    rp_last, _ = finish_rows(S - E_ROWS, acc_v[...], 0.0, 1.0)
    m1, m2 = score_rows(S - E_ROWS, rp_last, None, m1, m2)
    cp_out(2 * n_e - 1).start()

    t1 = jnp.max(m1, axis=0, keepdims=True)
    t2 = jnp.max(jnp.where(m1 == t1, m2, m1), axis=0, keepdims=True)
    i1 = 0xFFFF - (t1[0, 0] & 0xFFFF)
    i2 = 0xFFFF - (t2[0, 0] & 0xFFFF)
    g1 = pl.multiple_of((i1 // GRP) * GRP, GRP)
    g2 = pl.multiple_of((i2 // GRP) * GRP, GRP)

    xs = jnp.concatenate([h_v[pl.ds(g1, GRP), :], h_v[pl.ds(g2, GRP), :]], axis=0)

    def act(j):
        fc = slice(j * FC, (j + 1) * FC)
        g = _r(jnp.dot(xs, wg_v[:, fc], preferred_element_type=f32))
        u = _r(jnp.dot(xs, wu_v[:, fc], preferred_element_type=f32))
        return (_r(g * jax.nn.sigmoid(g)) * u).astype(bf16)

    y = None
    a = act(0)
    for j in range(F // FC):
        a_next = act(j + 1) if (j + 1) * FC < F else None
        d = jnp.dot(a, wd_v[j * FC:(j + 1) * FC, :], preferred_element_type=f32)
        y = d if y is None else y + d
        a = a_next
    h2 = xs.astype(f32)
    x2 = jnp.concatenate([x2_v[pl.ds(g1, GRP), :], x2_v[pl.ds(g2, GRP), :]], axis=0).astype(f32)
    r = _r(jnp.sum(router_parts(h2)[-1], axis=1, keepdims=True))
    upd = _r(_r(y) * _r(jax.nn.sigmoid(r)))
    loc = lax.broadcasted_iota(jnp.int32, (2 * GRP, D), 0)
    row = jnp.where(loc < GRP, g1 + loc, g2 + loc - GRP)
    sel = jnp.logical_or(row == i1, row == i2)
    hb = _r(h2 + jnp.where(sel, upd, 0.0))
    fix_v[...] = (x2 + _r(mrow(GB, 2 * GRP) * hb)).astype(bf16)

    cp(out_v, out_v, SEM_OUT).wait()
    fix1 = cp(fix_v.at[pl.ds(0, GRP), :], out_hbm.at[0, pl.ds(g1, GRP), :], SEM_FIX)
    fix2 = cp(fix_v.at[pl.ds(GRP, GRP), :], out_hbm.at[0, pl.ds(g2, GRP), :], SEM_FIX + 1)
    fix1.start()

    @pl.when(g2 != g1)
    def _():
        fix2.start()
        fix2.wait()

    fix1.wait()


@jax.jit
def pallas_adaLN_cond__mha_block_cached__moe_arch_mod__prompt_kernel(
    A_x: jax.Array,
    A_k_cache: jax.Array,
    A_v_cache: jax.Array,
    A_wq: jax.Array,
    A_wo: jax.Array,
    B_x: jax.Array,
    B_w_r: jax.Array,
    B_w_gate: jax.Array,
    B_w_up: jax.Array,
    B_w_down: jax.Array,
    c: jax.Array,
    w_mod: jax.Array,
):
    del B_x
    vm = pltpu.VMEM
    scratch = [
        vm((S, D), bf16),
        vm((S, D), bf16),
        vm((S, D), bf16),
        vm((S, D), bf16),
        vm((H, S, DH), bf16),
        vm((HH, S, DH), bf16),
        vm((HH, S, DH), bf16),
        vm((S, D), f32),
        vm((E_ROWS, D), f32),
        vm((D, H * DH), bf16),
        vm((H * DH, D), bf16),
        vm((D, 2 * D), bf16),
        vm((D, F), bf16),
        vm((D, F), bf16),
        vm((F, D), bf16),
        vm((2, S, DH), bf16),
        vm((2, S, DH), bf16),
        vm((1, D), bf16),
        vm((D,), bf16),
        vm((GRP, D), bf16),
        vm((8, 7 * D), f32),
        vm((2, 8, 128), jnp.int32),
        vm((2, E_ROWS, 128), f32),
        vm((2 * GRP, D), bf16),
        pltpu.SemaphoreType.DMA((N_SEM,)),
    ]
    return pl.pallas_call(
        _kernel,
        in_specs=[pl.BlockSpec(memory_space=pl.ANY)] * 11,
        out_specs=pl.BlockSpec(memory_space=pl.ANY),
        out_shape=jax.ShapeDtypeStruct(A_x.shape, A_x.dtype),
        scratch_shapes=scratch,
        compiler_params=pltpu.CompilerParams(vmem_limit_bytes=124 * 1024 * 1024,
                                             disable_bounds_checks=True),
        name="adaln_mha_moe",
    )(A_x, A_k_cache, A_v_cache, A_wq, A_wo, B_w_r, B_w_gate, B_w_up, B_w_down, c, w_mod)
```

```python
import jax
import jax.numpy as jnp
from jax import lax
import jax.experimental.pallas as pl
import jax.experimental.pallas.tpu as pltpu

S = 2048
D = 1024
H = 32
DH = 128
F = 3584
EPS = 1e-5
HH = H // 2

TQ = 256
KR = 512
P_ROWS = 256
P_HEADS = 4
QU_ROWS = 512
QU_PER_IT = (H - P_HEADS) * (S // QU_ROWS) // HH
B_ROWS = S // HH
E_ROWS = 128
PACE = 24
GRP = 16
FC = 512
PAD = 128
P_LO, P_HI = 0.25, 0.97
E_LO0, E_LO1, E_HI, E_KEY = 0.15, 0.25, 0.97, 0.1

Q_SCALE = float(DH) ** -0.5 * 1.4426950408889634

f32 = jnp.float32
bf16 = jnp.bfloat16
u32 = jnp.uint32


def _r(x):
    return x.astype(bf16).astype(f32)


def _recip(x):
    r0 = pl.reciprocal(x, approx=True)
    return r0 * (2.0 - x * r0)


def _pace(v):
    t = v[0:8, 0:128]
    for _ in range(PACE):
        t = jnp.minimum(t, jnp.max(t, axis=1, keepdims=True))
    top = t if v.shape[1] == 128 else jnp.concatenate([t, v[0:8, 128:]], axis=1)
    return jnp.concatenate([top, v[8:, :]], axis=0)


def _tiles(v):
    u = pltpu.bitcast(v, u32)
    return [[u[a * 8:(a + 1) * 8, b * 128:(b + 1) * 128] for b in range(u.shape[1] // 128)]
            for a in range(u.shape[0] // 8)]


def _col_dots(k_tiles, rhs, n_tiles, never, deps):
    n_r = len(k_tiles) // 4
    n_i = k_tiles[0].shape[0] // GRP
    total = n_tiles * n_r * n_i
    at = {}
    for n, (pos, d) in enumerate(deps):
        at.setdefault((min(int(pos * total), total - 1), n % 4), []).append(d)
    outs = []
    for j in range(n_tiles):
        tl = list(k_tiles)
        for k in range(len(k_tiles)):
            base = (j * n_r + k // 4) * n_i
            if not any((base + i, k % 4) in at for i in range(n_i)):
                continue
            tu = pltpu.bitcast(tl[k], u32)
            parts = []
            for i in range(n_i):
                t = tu[i * 8:(i + 1) * 8, :]
                for d in at.get((base + i, k % 4), ()):
                    t = jnp.where(never, d, t)
                parts.append(t)
            tl[k] = pltpu.bitcast(jnp.concatenate(parts, axis=0), bf16)
        outs.append(jnp.dot(jnp.concatenate(tl, axis=1), rhs(j), preferred_element_type=f32))
    return outs


def _never(i):
    return jnp.full((8, 128), i, jnp.int32) > (1 << 20)


def _attention(q_ref, k_ref, v_ref, o_ref):
    n = S // TQ

    def scores(c):
        q = q_ref[c * TQ:(c + 1) * TQ, :]
        return lax.dot_general(q, k_ref[...], (((1,), (1,)), ((), ())),
                               preferred_element_type=f32)

    def finish(c, s):
        m = jnp.max(s, axis=1, keepdims=True)
        o = None
        lp = None
        for r in range(S // KR):
            p = jnp.exp2(s[:, r * KR:(r + 1) * KR] - m)
            ps = [p[:, j * 128:(j + 1) * 128] for j in range(KR // 128)]
            t = ps[0]
            for x in ps[1:]:
                t = t + x
            lp = t if lp is None else lp + t
            ps[-1] = jnp.minimum(ps[-1], t)
            p = jnp.concatenate(ps, axis=1)
            d = jnp.dot(p.astype(bf16), v_ref[r * KR:(r + 1) * KR, :],
                        preferred_element_type=f32)
            o = d if o is None else o + d
        l = jnp.sum(lp, axis=1, keepdims=True)
        o_ref[c * TQ:(c + 1) * TQ, :] = (o * _recip(l)).astype(bf16)

    s = scores(0)
    for c in range(n):
        s_next = scores(c + 1) if c + 1 < n else None
        finish(c, s)
        s = s_next


SEM_C, SEM_WR, SEM_WMA, SEM_X, SEM_WQ, SEM_KV, SEM_BG, SEM_OUT, SEM_FIX, SEM_WMB, N_SEM = (
    0, 1, 2, 6, 14, 17, 25, 29, 30, 32, 34)
SA, CA1, GA, SB, CB1, GB, WR = range(7)


def _kernel(x_hbm, k_hbm, v_hbm, wq_hbm, wo_hbm, wr_hbm, wg_hbm, wu_hbm, wd_hbm, c_hbm,
            wm_hbm, out_hbm,
            x_v, h_v, x2_v, out_v, q_v, olo_v, ohi_v, part_v, acc_v, wq_v, wo_v, wma_v, wg_v,
            wu_v, wd_v, k_v, v_v, c_v, wr_v, sc_v, mod_v, top_v, rp_v, fix_v, sems):
    n_p = S // P_ROWS
    n_e = S // (2 * E_ROWS)
    pq = P_HEADS * DH

    def cp(src, dst, sem):
        return pltpu.make_async_copy(src, dst, sems.at[sem])

    def cp_c():
        return cp(c_hbm, c_v, SEM_C)

    def cp_wr():
        return cp(wr_hbm, wr_v, SEM_WR)

    def cp_wma(j):
        return cp(wm_hbm.at[:, pl.ds(j * 512, 512)], wma_v.at[:, pl.ds(j * 512, 512)], SEM_WMA + j)

    def cp_x(i):
        return cp(x_hbm.at[0, pl.ds(i * P_ROWS, P_ROWS), :], x_v.at[pl.ds(i * P_ROWS, P_ROWS), :],
                  SEM_X + i)

    wq_cols = ((0, pq), (pq, 1024), (pq + 1024, H * DH - pq - 1024))

    def cp_wq(j):
        lo, n = wq_cols[j]
        return cp(wq_hbm.at[:, pl.ds(lo, n)], wq_v.at[:, pl.ds(lo, n)], SEM_WQ + j)

    def cp_k(h):
        return cp(k_hbm.at[0, h], k_v.at[h & 3], SEM_KV + (h & 3))

    def cp_v(h):
        return cp(v_hbm.at[0, h], v_v.at[h & 3], SEM_KV + 4 + (h & 3))

    def cp_rows(src, dst, i, n, sem):
        return cp(src.at[pl.ds(i * n, n), :], dst.at[pl.ds(i * n, n), pl.ds(0, src.shape[1])], sem)

    def cp_wmb(j):
        return cp(wm_hbm.at[:, pl.ds((2 + 2 * j) * D, 2 * D)], wq_v.at[:, pl.ds(2 * j * D, 2 * D)],
                  SEM_WMB + j)

    def cp_out(i):
        return cp(out_v.at[pl.ds(i * E_ROWS, E_ROWS), :],
                  out_hbm.at[0, pl.ds(i * E_ROWS, E_ROWS), :], SEM_OUT)

    def mrow(k, n):
        m = mod_v[:, k * D:(k + 1) * D]
        return jnp.concatenate([m] * (n // 8), axis=0)

    cp_c().start()
    for j in range(4):
        cp_wma(j).start()
    cp_x(0).start()
    cp_wq(0).start()
    for i in range(1, n_p):
        cp_x(i).start()
    cp_k(0).start()
    cp_v(0).start()
    cp_wq(1).start()
    cp_k(1).start()
    cp_v(1).start()
    cp_wq(2).start()
    cp_wr().start()

    cp_c().wait()
    cf = c_v[...].astype(f32)
    sc_v[...] = jnp.broadcast_to(cf * jax.nn.sigmoid(cf), (GRP, D)).astype(bf16)

    def wma_body(j, carry):
        cp_wma(j).wait()
        cols = pl.ds(pl.multiple_of(j * 512, 512), 512)
        mj = jnp.dot(sc_v[...], wma_v[:, cols], preferred_element_type=f32)
        mod_v[:, cols] = _r(_r(mj[0:8, :]) + jnp.where(j >= 2, 1.0, 0.0))
        return carry

    lax.fori_loop(0, 4, wma_body, 0)

    def ln1(i):
        rows = pl.ds(pl.multiple_of(i * P_ROWS, P_ROWS), P_ROWS)
        x = x_v[rows, :].astype(f32)
        mu = jnp.sum(x, axis=1, keepdims=True) * (1.0 / D)
        d = x - mu
        var = jnp.sum(d * d, axis=1, keepdims=True) * (1.0 / D)
        n = d * lax.rsqrt(var + EPS)
        h = (n * mrow(CA1, P_ROWS) + mrow(SA, P_ROWS)).astype(bf16)
        h_v[rows, :] = h
        return h

    cp_x(0).wait()
    ln1(0)
    cp_wq(0).wait()

    def p_body(i, carry):
        @pl.when(i + 1 < n_p)
        def _():
            cp_x(i + 1).wait()

        rows = pl.ds(pl.multiple_of(i * P_ROWS, P_ROWS), P_ROWS)
        lhs = [h_v[rows, k * 128:(k + 1) * 128] for k in range(D // 128)]
        tl = [t for row in _tiles(ln1(jnp.minimum(i + 1, n_p - 1))) for t in row]
        deps = [(P_LO + (P_HI - P_LO) * n / len(tl), t) for n, t in enumerate(tl)]
        qs = _col_dots(lhs, lambda j: wq_v[:, j * DH:(j + 1) * DH], P_HEADS, _never(i), deps)
        for j in range(P_HEADS):
            q_v[j, rows, :] = (qs[j] * Q_SCALE).astype(bf16)
        return carry

    lax.fori_loop(0, n_p, p_body, 0)
    cp_wq(1).wait()

    def kv_wait(h):
        cp_k(h).wait()
        cp_v(h).wait()
        return h & 3

    def kv_prefetch(h):
        @pl.when(h + 2 < H)
        def _():
            cp_k(h + 2).start()
            cp_v(h + 2).start()

    def a_body(it, carry):
        @pl.when(it == 1)
        def _():
            cp_wq(2).wait()

        slot = kv_wait(it)

        def q_unit(u):
            g = it * QU_PER_IT + u
            hd = P_HEADS + (g >> 2)
            r0 = pl.multiple_of((g & 3) * QU_ROWS, QU_ROWS)
            cols = pl.ds(pl.multiple_of(hd * DH, DH), DH)
            q = jnp.dot(h_v[pl.ds(r0, QU_ROWS), :], wq_v[:, cols], preferred_element_type=f32)
            if u == 1:
                q = _pace(q)
            return hd, r0, (q * Q_SCALE).astype(bf16)

        late = [q_unit(0)]
        _attention(q_v.at[it], k_v.at[slot], v_v.at[slot], olo_v.at[it])
        for u in range(1, QU_PER_IT):
            hd, r0, q = q_unit(u)
            if u == 1:
                late.append((hd, r0, q[0:GRP, :]))
                q_v[hd, pl.ds(r0 + GRP, QU_ROWS - GRP), :] = q[GRP:, :]
            else:
                q_v[hd, pl.ds(r0, QU_ROWS), :] = q
            if u == QU_PER_IT - 2:
                for hd, r0, q in late:
                    q_v[hd, pl.ds(r0, q.shape[0]), :] = q

        kv_prefetch(it)
        for n, (src, dst) in enumerate(((wo_hbm, wo_v), (wg_hbm, wg_v), (wu_hbm, wu_v),
                                        (wd_hbm, wd_v))):
            @pl.when(it >> 2 == n)
            def _():
                cp_rows(src, dst, it & 3, src.shape[0] // 4, SEM_BG + n).start()

        @pl.when(it == HH - 4)
        def _():
            cp_wmb(0).start()

        return carry

    lax.fori_loop(0, HH, a_body, 0)

    cp(wo_hbm, wo_v.at[:, pl.ds(0, D)], SEM_BG).wait()
    cp_wmb(0).wait()
    cp_wmb(1).start()

    def b_body(it, carry):
        @pl.when(it == HH // 2)
        def _():
            cp_wmb(1).wait()

        slot = kv_wait(HH + it)
        rows = pl.ds(pl.multiple_of(it * B_ROWS, B_ROWS), B_ROWS)

        def o_unit(lo, hi, pace):
            lhs = jnp.concatenate([olo_v[j, rows, :] for j in range(HH)], axis=1)
            part = jnp.dot(lhs, wo_v[0:HH * DH, lo:hi], preferred_element_type=f32)
            part_v[rows, lo:hi] = _pace(part) if pace else part

        o_unit(0, 128, False)
        _attention(q_v.at[HH + it], k_v.at[slot], v_v.at[slot], ohi_v.at[it])
        one = jnp.where(it >> 2 == CB1 - GA, 1.0, 0.0)
        mb = None
        for u in range(4):
            o_unit(max(u * 256, 128), (u + 1) * 256, u == 0)
            c0 = pl.multiple_of(it * 256 + (u // 2) * 128, 128)
            ks = slice((u % 2) * 512, (u % 2 + 1) * 512)
            d = jnp.dot(sc_v[:, ks], wq_v[ks, pl.ds(c0, 128)], preferred_element_type=f32)[0:8, :]
            if u % 2 == 0:
                mb = d
            else:
                mod_v[:, pl.ds(pl.multiple_of(GA * D + c0, 128), 128)] = _r(_r(mb + d) + one)
        kv_prefetch(HH + it)
        return carry

    lax.fori_loop(0, HH, b_body, 0)

    cp_wr().wait()
    cp(wg_v, wg_v, SEM_BG + 1).wait()
    cp(wu_v, wu_v, SEM_BG + 2).wait()
    cp(wd_hbm, wd_v.at[:, pl.ds(0, D)], SEM_BG + 3).wait()
    mod_v[:, WR * D:(WR + 1) * D] = jnp.broadcast_to(wr_v[...].astype(f32).reshape(1, D), (8, D))
    int_min = jnp.iinfo(jnp.int32).min
    top_v[...] = jnp.full(top_v.shape, int_min, jnp.int32)
    acc_v[...] = jnp.zeros(acc_v.shape, f32)
    rp_v[...] = jnp.zeros(rp_v.shape, f32)

    def router_parts(h2):
        pr = h2 * mrow(WR, h2.shape[0])
        run = [pr[:, 0:128]]
        for b in range(1, D // 128):
            run.append(run[-1] + pr[:, b * 128:(b + 1) * 128])
        return run

    def finish_rows(r0, attn, lo, hi):
        rows = pl.ds(r0, E_ROWS)
        x2 = _r(x_v[rows, :].astype(f32) + mrow(GA, E_ROWS) * attn)
        mu = jnp.sum(x2, axis=1, keepdims=True) * (1.0 / D)
        dc = x2 - mu
        var = _r(jnp.sum(dc * dc, axis=1, keepdims=True) * (1.0 / D))
        den = _r(jnp.sqrt(_r(var + EPS)))
        n = _r(_r(x2 - _r(mu)) * _recip(den))
        h2 = _r(_r(n * mrow(CB1, E_ROWS)) + mrow(SB, E_ROWS))
        x2_v[rows, :] = x2.astype(bf16)
        h_v[rows, :] = h2.astype(bf16)
        ob = (x2 + _r(mrow(GB, E_ROWS) * h2)).astype(bf16)
        out_v[rows, :] = ob
        run = router_parts(h2)
        deps = []
        ot = _tiles(ob)
        n_t = len(ot) * len(ot[0])
        for p in range(len(ot)):
            for b in range(len(ot[0])):
                pos = lo + (hi - lo) * (p * len(ot[0]) + b) / n_t
                deps.append((pos, ot[p][b]))
                for g in (2 * p, 2 * p + 1):
                    deps.append((pos, pltpu.bitcast(run[b][g * 8:(g + 1) * 8, :], u32)))
        return run[-1], deps

    def score_rows(r0, rp, valid, m1, m2):
        r = _r(jnp.sum(rp, axis=1, keepdims=True)) + 0.0
        r = jnp.where(r != r, -jnp.inf, r)
        bits = pltpu.bitcast(jnp.broadcast_to(r, (E_ROWS, 128)), jnp.int32)
        bits = jnp.where(bits < 0, bits ^ 0x7FFF0000, bits)
        idx = r0 + lax.broadcasted_iota(jnp.int32, (E_ROWS, 128), 0)
        key = bits | (0xFFFF - idx)
        if valid is not None:
            key = jnp.where(valid, key, int_min)
        for g in range(E_ROWS // 8):
            kg = key[g * 8:(g + 1) * 8, :]
            m2 = jnp.maximum(m2, jnp.minimum(m1, kg))
            m1 = jnp.maximum(m1, kg)
        return m1, m2

    def out_proj(r0, never, deps):
        rows = pl.ds(r0, E_ROWS)
        lhs = [ohi_v[j, rows, :] for j in range(HH)]
        ds = _col_dots(lhs, lambda j: wo_v[HH * DH:H * DH, j * 128:(j + 1) * 128], D // 128,
                       never, deps)
        return part_v[rows, :] + jnp.concatenate(ds, axis=1)

    def e_body(c, carry):
        @pl.when(c >= 2)
        def _():
            cp_out(2 * c - 3).start()

        @pl.when(c >= 1)
        def _():
            cp_out(2 * c - 2).start()

        never = _never(c)
        ra = pl.multiple_of(2 * c * E_ROWS, E_ROWS)
        rb = pl.multiple_of(ra + E_ROWS, E_ROWS)
        rp = pl.multiple_of(jnp.maximum(ra - E_ROWS, 0), E_ROWS)
        m1, m2 = score_rows(ra - 3 * E_ROWS, rp_v[0], c >= 2, top_v[0], top_v[1])
        m1, m2 = score_rows(ra - 2 * E_ROWS, rp_v[1], c >= 1, m1, m2)
        top_v[0] = m1
        top_v[1] = m2
        rp_v[0], deps = finish_rows(rp, acc_v[...], E_LO0, E_HI)
        if E_KEY is not None:
            deps.append((E_KEY, pltpu.bitcast(m2, u32)))
        attn = out_proj(ra, never, deps)
        rp_v[1], deps = finish_rows(ra, attn, E_LO1, E_HI)
        acc_v[...] = out_proj(rb, never, deps)
        return carry

    lax.fori_loop(0, n_e, e_body, 0)
    cp_out(2 * n_e - 3).start()
    cp_out(2 * n_e - 2).start()
    m1, m2 = score_rows(S - 3 * E_ROWS, rp_v[0], None, top_v[0], top_v[1])
    m1, m2 = score_rows(S - 2 * E_ROWS, rp_v[1], None, m1, m2)
    rp_last, _ = finish_rows(S - E_ROWS, acc_v[...], 0.0, 1.0)
    m1, m2 = score_rows(S - E_ROWS, rp_last, None, m1, m2)
    cp_out(2 * n_e - 1).start()

    t1 = jnp.max(m1, axis=0, keepdims=True)
    t2 = jnp.max(jnp.where(m1 == t1, m2, m1), axis=0, keepdims=True)
    i1 = 0xFFFF - (t1[0, 0] & 0xFFFF)
    i2 = 0xFFFF - (t2[0, 0] & 0xFFFF)
    g1 = pl.multiple_of((i1 // GRP) * GRP, GRP)
    g2 = pl.multiple_of((i2 // GRP) * GRP, GRP)

    xs = jnp.concatenate([h_v[pl.ds(g1, GRP), :], h_v[pl.ds(g2, GRP), :]], axis=0)

    def act(j):
        fc = slice(j * FC, (j + 1) * FC)
        g = _r(jnp.dot(xs, wg_v[:, fc], preferred_element_type=f32))
        u = _r(jnp.dot(xs, wu_v[:, fc], preferred_element_type=f32))
        return (_r(g * jax.nn.sigmoid(g)) * u).astype(bf16)

    y = None
    a = act(0)
    for j in range(F // FC):
        a_next = act(j + 1) if (j + 1) * FC < F else None
        d = jnp.dot(a, wd_v[j * FC:(j + 1) * FC, 0:D], preferred_element_type=f32)
        y = d if y is None else y + d
        a = a_next
    h2 = xs.astype(f32)
    x2 = jnp.concatenate([x2_v[pl.ds(g1, GRP), :], x2_v[pl.ds(g2, GRP), :]], axis=0).astype(f32)
    r = _r(jnp.sum(router_parts(h2)[-1], axis=1, keepdims=True))
    upd = _r(_r(y) * _r(jax.nn.sigmoid(r)))
    loc = lax.broadcasted_iota(jnp.int32, (2 * GRP, D), 0)
    row = jnp.where(loc < GRP, g1 + loc, g2 + loc - GRP)
    sel = jnp.logical_or(row == i1, row == i2)
    hb = _r(h2 + jnp.where(sel, upd, 0.0))
    fix_v[...] = (x2 + _r(mrow(GB, 2 * GRP) * hb)).astype(bf16)

    cp(out_v, out_v, SEM_OUT).wait()
    fix1 = cp(fix_v.at[pl.ds(0, GRP), :], out_hbm.at[0, pl.ds(g1, GRP), :], SEM_FIX)
    fix2 = cp(fix_v.at[pl.ds(GRP, GRP), :], out_hbm.at[0, pl.ds(g2, GRP), :], SEM_FIX + 1)
    fix1.start()

    @pl.when(g2 != g1)
    def _():
        fix2.start()
        fix2.wait()

    fix1.wait()


@jax.jit
def pallas_adaLN_cond__mha_block_cached__moe_arch_mod__prompt_kernel(
    A_x: jax.Array,
    A_k_cache: jax.Array,
    A_v_cache: jax.Array,
    A_wq: jax.Array,
    A_wo: jax.Array,
    B_x: jax.Array,
    B_w_r: jax.Array,
    B_w_gate: jax.Array,
    B_w_up: jax.Array,
    B_w_down: jax.Array,
    c: jax.Array,
    w_mod: jax.Array,
):
    del B_x
    vm = pltpu.VMEM
    scratch = [
        vm((S, D), bf16),
        vm((S, D), bf16),
        vm((S, D), bf16),
        vm((S, D), bf16),
        vm((H, S, DH), bf16),
        vm((HH, S, DH), bf16),
        vm((HH, S, DH), bf16),
        vm((S, D), f32),
        vm((E_ROWS, D), f32),
        vm((D, H * DH + PAD), bf16),
        vm((H * DH, D + PAD), bf16),
        vm((D, 2 * D + PAD), bf16),
        vm((D, F), bf16),
        vm((D, F), bf16),
        vm((F, D + PAD), bf16),
        vm((4, S, DH), bf16),
        vm((4, S, DH), bf16),
        vm((1, D), bf16),
        vm((D,), bf16),
        vm((GRP, D), bf16),
        vm((8, 7 * D), f32),
        vm((2, 8, 128), jnp.int32),
        vm((2, E_ROWS, 128), f32),
        vm((2 * GRP, D), bf16),
        pltpu.SemaphoreType.DMA((N_SEM,)),
    ]
    return pl.pallas_call(
        _kernel,
        in_specs=[pl.BlockSpec(memory_space=pl.ANY)] * 11,
        out_specs=pl.BlockSpec(memory_space=pl.ANY),
        out_shape=jax.ShapeDtypeStruct(A_x.shape, A_x.dtype),
        scratch_shapes=scratch,
        compiler_params=pltpu.CompilerParams(vmem_limit_bytes=124 * 1024 * 1024,
                                             disable_bounds_checks=True),
        name="adaln_mha_moe",
    )(A_x, A_k_cache, A_v_cache, A_wq, A_wo, B_w_r, B_w_gate, B_w_up, B_w_down, c, w_mod)
```

```python
import jax
import jax.numpy as jnp
from jax import lax
import jax.experimental.pallas as pl
import jax.experimental.pallas.tpu as pltpu

S = 2048
D = 1024
H = 32
DH = 128
F = 3584
EPS = 1e-5
HH = H // 2

TQ = 256
KR = 512
P_ROWS = 256
P_HEADS = 4
QU_ROWS = 512
QU_PER_IT = (H - P_HEADS) * (S // QU_ROWS) // HH
B_ROWS = S // HH
E_ROWS = 64
E_SUB = 4
PACE = 24
GRP = 16
FC = 512
PAD = 128
P_LO, P_HI = 0.25, 0.97
E_LO0, E_LO1, E_HI, E_KEY = 0.3, 0.3, 0.97, 0.2

Q_SCALE = float(DH) ** -0.5 * 1.4426950408889634

f32 = jnp.float32
bf16 = jnp.bfloat16
u32 = jnp.uint32


def _r(x):
    return x.astype(bf16).astype(f32)


def _recip(x):
    r0 = pl.reciprocal(x, approx=True)
    return r0 * (2.0 - x * r0)


def _pace(v):
    t = v[0:8, 0:128]
    for _ in range(PACE):
        t = jnp.minimum(t, jnp.max(t, axis=1, keepdims=True))
    top = t if v.shape[1] == 128 else jnp.concatenate([t, v[0:8, 128:]], axis=1)
    return jnp.concatenate([top, v[8:, :]], axis=0)


def _tiles(v):
    u = pltpu.bitcast(v, u32)
    return [[u[a * 8:(a + 1) * 8, b * 128:(b + 1) * 128] for b in range(u.shape[1] // 128)]
            for a in range(u.shape[0] // 8)]


def _col_dots(k_tiles, rhs, n_tiles, never, deps):
    n_r = len(k_tiles) // 4
    n_i = k_tiles[0].shape[0] // GRP
    total = n_tiles * n_r * n_i
    at = {}
    for n, (pos, d) in enumerate(deps):
        at.setdefault((min(int(pos * total), total - 1), n % 4), []).append(d)
    outs = []
    for j in range(n_tiles):
        tl = list(k_tiles)
        for k in range(len(k_tiles)):
            base = (j * n_r + k // 4) * n_i
            if not any((base + i, k % 4) in at for i in range(n_i)):
                continue
            tu = pltpu.bitcast(tl[k], u32)
            parts = []
            for i in range(n_i):
                t = tu[i * 8:(i + 1) * 8, :]
                for d in at.get((base + i, k % 4), ()):
                    t = jnp.where(never, d, t)
                parts.append(t)
            tl[k] = pltpu.bitcast(jnp.concatenate(parts, axis=0), bf16)
        outs.append(jnp.dot(jnp.concatenate(tl, axis=1), rhs(j), preferred_element_type=f32))
    return outs


def _never(i):
    return jnp.full((8, 128), i, jnp.int32) > (1 << 20)


def _attention(q_ref, k_ref, v_ref, o_ref):
    n = S // TQ

    def scores(c):
        q = q_ref[c * TQ:(c + 1) * TQ, :]
        return lax.dot_general(q, k_ref[...], (((1,), (1,)), ((), ())),
                               preferred_element_type=f32)

    def finish(c, s):
        m = jnp.max(s, axis=1, keepdims=True)
        o = None
        lp = None
        for r in range(S // KR):
            p = jnp.exp2(s[:, r * KR:(r + 1) * KR] - m)
            ps = [p[:, j * 128:(j + 1) * 128] for j in range(KR // 128)]
            t = ps[0]
            for x in ps[1:]:
                t = t + x
            lp = t if lp is None else lp + t
            ps[-1] = jnp.minimum(ps[-1], t)
            p = jnp.concatenate(ps, axis=1)
            d = jnp.dot(p.astype(bf16), v_ref[r * KR:(r + 1) * KR, :],
                        preferred_element_type=f32)
            o = d if o is None else o + d
        l = jnp.sum(lp, axis=1, keepdims=True)
        o_ref[c * TQ:(c + 1) * TQ, :] = (o * _recip(l)).astype(bf16)

    s = scores(0)
    for c in range(n):
        s_next = scores(c + 1) if c + 1 < n else None
        finish(c, s)
        s = s_next


SEM_C, SEM_WR, SEM_WMA, SEM_X, SEM_WQ, SEM_KV, SEM_BG, SEM_OUT, SEM_FIX, SEM_WMB, N_SEM = (
    0, 1, 2, 6, 14, 17, 25, 29, 30, 32, 34)
SA, CA1, GA, SB, CB1, GB, WR = range(7)


def _kernel(x_hbm, k_hbm, v_hbm, wq_hbm, wo_hbm, wr_hbm, wg_hbm, wu_hbm, wd_hbm, c_hbm,
            wm_hbm, out_hbm,
            x_v, h_v, x2_v, out_v, q_v, olo_v, ohi_v, part_v, acc_v, wqp_v, wq_v, wo_v, wma_v,
            wg_v, wu_v, wd_v, k_v, v_v, c_v, wr_v, sc_v, mod_v, top_v, rp_v, fix_v, sems):
    n_p = S // P_ROWS
    n_e = S // (E_SUB * E_ROWS)
    pq = P_HEADS * DH

    def cp(src, dst, sem):
        return pltpu.make_async_copy(src, dst, sems.at[sem])

    def cp_c():
        return cp(c_hbm, c_v, SEM_C)

    def cp_wr():
        return cp(wr_hbm, wr_v, SEM_WR)

    def cp_wma(j):
        return cp(wm_hbm.at[:, pl.ds(j * 512, 512)], wma_v.at[:, pl.ds(j * 512, 512)], SEM_WMA + j)

    def cp_x(i):
        return cp(x_hbm.at[0, pl.ds(i * P_ROWS, P_ROWS), :], x_v.at[pl.ds(i * P_ROWS, P_ROWS), :],
                  SEM_X + i)

    def cp_wqp():
        return cp(wq_hbm.at[:, pl.ds(0, pq)], wqp_v.at[:, pl.ds(0, pq)], SEM_WQ)

    def cp_tile(src, col, j, sem):
        return cp(src.at[:, pl.ds(pl.multiple_of(col * DH, DH), DH)], wq_v.at[j], sem)

    def tiles_wait(lo, hi, sem):
        cp(wq_v.at[pl.ds(lo, hi - lo)], wq_v.at[pl.ds(lo, hi - lo)], sem).wait()

    def cp_k(h):
        return cp(k_hbm.at[0, h], k_v.at[h & 3], SEM_KV + (h & 3))

    def cp_v(h):
        return cp(v_hbm.at[0, h], v_v.at[h & 3], SEM_KV + 4 + (h & 3))

    def cp_rows(src, dst, i, n, sem):
        return cp(src.at[pl.ds(i * n, n), :], dst.at[pl.ds(i * n, n), pl.ds(0, src.shape[1])], sem)

    def wmb_start(g, half):
        for k in range(4):
            cp_tile(wm_hbm, 2 * D // DH + 4 * g + k, 4 * g + k, SEM_WMB + half).start()

    def cp_out(i, n):
        return cp(out_v.at[pl.ds(i * E_ROWS, n * E_ROWS), :],
                  out_hbm.at[0, pl.ds(i * E_ROWS, n * E_ROWS), :], SEM_OUT)

    def mrow(k, n):
        m = mod_v[:, k * D:(k + 1) * D]
        return jnp.concatenate([m] * (n // 8), axis=0)

    cp_c().start()
    cp_wr().start()
    for j in range(4):
        cp_wma(j).start()
    cp_x(0).start()
    cp_wqp().start()
    for i in range(1, n_p):
        cp_x(i).start()
    cp_k(0).start()
    cp_v(0).start()

    cp_c().wait()
    cp_wr().wait()
    mod_v[:, WR * D:(WR + 1) * D] = jnp.broadcast_to(wr_v[...].astype(f32).reshape(1, D), (8, D))
    int_min = jnp.iinfo(jnp.int32).min
    top_v[...] = jnp.full(top_v.shape, int_min, jnp.int32)
    acc_v[...] = jnp.zeros(acc_v.shape, f32)
    rp_v[...] = jnp.zeros(rp_v.shape, f32)
    cf = c_v[...].astype(f32)
    sc_v[...] = jnp.broadcast_to(cf * jax.nn.sigmoid(cf), (GRP, D)).astype(bf16)

    def wma_body(j, carry):
        cp_wma(j).wait()
        cols = pl.ds(pl.multiple_of(j * 512, 512), 512)
        mj = jnp.dot(sc_v[...], wma_v[:, cols], preferred_element_type=f32)
        mod_v[:, cols] = _r(_r(mj[0:8, :]) + jnp.where(j >= 2, 1.0, 0.0))
        return carry

    lax.fori_loop(0, 4, wma_body, 0)

    def ln1(i):
        rows = pl.ds(pl.multiple_of(i * P_ROWS, P_ROWS), P_ROWS)
        x = x_v[rows, :].astype(f32)
        mu = jnp.sum(x, axis=1, keepdims=True) * (1.0 / D)
        d = x - mu
        var = jnp.sum(d * d, axis=1, keepdims=True) * (1.0 / D)
        n = d * lax.rsqrt(var + EPS)
        h = (n * mrow(CA1, P_ROWS) + mrow(SA, P_ROWS)).astype(bf16)
        h_v[rows, :] = h
        return h

    cp_x(0).wait()
    ln1(0)
    cp_wqp().wait()

    def p_body(i, carry):
        @pl.when(i + 1 < n_p)
        def _():
            cp_x(i + 1).wait()

        rows = pl.ds(pl.multiple_of(i * P_ROWS, P_ROWS), P_ROWS)
        lhs = [h_v[rows, k * 128:(k + 1) * 128] for k in range(D // 128)]
        tl = [t for row in _tiles(ln1(jnp.minimum(i + 1, n_p - 1))) for t in row]
        deps = [(P_LO + (P_HI - P_LO) * n / len(tl), t) for n, t in enumerate(tl)]
        qs = _col_dots(lhs, lambda j: wqp_v[:, j * DH:(j + 1) * DH], P_HEADS, _never(i), deps)
        for j in range(P_HEADS):
            q_v[j, rows, :] = (qs[j] * Q_SCALE).astype(bf16)

        @pl.when(i + 1 < n_p)
        def _():
            for k in range(4):
                hd = P_HEADS + 4 * i + k
                cp_tile(wq_hbm, hd, hd, SEM_WQ + jnp.where(i < 2, 1, 2)).start()

        return carry

    lax.fori_loop(0, n_p, p_body, 0)
    cp_k(1).start()
    cp_v(1).start()
    tiles_wait(P_HEADS, P_HEADS + 8, SEM_WQ + 1)

    def kv_wait(h):
        cp_k(h).wait()
        cp_v(h).wait()
        return h & 3

    def kv_prefetch(h):
        @pl.when(h + 2 < H)
        def _():
            cp_k(h + 2).start()
            cp_v(h + 2).start()

    def a_body(it, carry):
        @pl.when(it == 1)
        def _():
            tiles_wait(P_HEADS + 8, H, SEM_WQ + 2)

        slot = kv_wait(it)

        def q_unit(u):
            g = it * QU_PER_IT + u
            hd = P_HEADS + (g >> 2)
            r0 = pl.multiple_of((g & 3) * QU_ROWS, QU_ROWS)
            q = jnp.dot(h_v[pl.ds(r0, QU_ROWS), :], wq_v[hd], preferred_element_type=f32)
            if u == 1:
                q = _pace(q)
            return hd, r0, (q * Q_SCALE).astype(bf16)

        late = [q_unit(0)]
        _attention(q_v.at[it], k_v.at[slot], v_v.at[slot], olo_v.at[it])
        for u in range(1, QU_PER_IT):
            hd, r0, q = q_unit(u)
            if u == 1:
                late.append((hd, r0, q[0:GRP, :]))
                q_v[hd, pl.ds(r0 + GRP, QU_ROWS - GRP), :] = q[GRP:, :]
            else:
                q_v[hd, pl.ds(r0, QU_ROWS), :] = q
            if u == QU_PER_IT - 2:
                for hd, r0, q in late:
                    q_v[hd, pl.ds(r0, q.shape[0]), :] = q

        kv_prefetch(it)
        for n, (src, dst) in enumerate(((wo_hbm, wo_v), (wg_hbm, wg_v), (wu_hbm, wu_v),
                                        (wd_hbm, wd_v))):
            @pl.when(it >> 2 == n)
            def _():
                cp_rows(src, dst, it & 3, src.shape[0] // 4, SEM_BG + n).start()

        @pl.when(it >> 2 == 2)
        def _():
            wmb_start(it & 3, 0)

        return carry

    lax.fori_loop(0, HH, a_body, 0)

    cp(wo_hbm, wo_v.at[:, pl.ds(0, D)], SEM_BG).wait()
    tiles_wait(0, HH, SEM_WMB)

    def b_body(it, carry):
        @pl.when(it == HH // 2)
        def _():
            tiles_wait(HH, H, SEM_WMB + 1)

        slot = kv_wait(HH + it)
        rows = pl.ds(pl.multiple_of(it * B_ROWS, B_ROWS), B_ROWS)

        def o_unit(lo, hi, pace):
            lhs = jnp.concatenate([olo_v[j, rows, :] for j in range(HH)], axis=1)
            part = jnp.dot(lhs, wo_v[0:HH * DH, lo:hi], preferred_element_type=f32)
            part_v[rows, lo:hi] = _pace(part) if pace else part

        o_unit(0, 128, False)
        _attention(q_v.at[HH + it], k_v.at[slot], v_v.at[slot], ohi_v.at[it])
        one = jnp.where(it >> 2 == CB1 - GA, 1.0, 0.0)
        mb = None
        for u in range(4):
            o_unit(max(u * 256, 128), (u + 1) * 256, u == 0)
            tile = 2 * it + u // 2
            ks = slice((u % 2) * 512, (u % 2 + 1) * 512)
            d = jnp.dot(sc_v[:, ks], wq_v[tile, ks, :], preferred_element_type=f32)[0:8, :]
            if u % 2 == 0:
                mb = d
            else:
                cols = pl.ds(pl.multiple_of(GA * D + tile * 128, 128), 128)
                mod_v[:, cols] = _r(_r(mb + d) + one)
        kv_prefetch(HH + it)

        @pl.when(it < 4)
        def _():
            wmb_start(4 + it, 1)

        return carry

    lax.fori_loop(0, HH, b_body, 0)

    cp(wg_v, wg_v, SEM_BG + 1).wait()
    cp(wu_v, wu_v, SEM_BG + 2).wait()
    cp(wd_hbm, wd_v.at[:, pl.ds(0, D)], SEM_BG + 3).wait()

    def router_parts(h2):
        pr = h2 * mrow(WR, h2.shape[0])
        run = [pr[:, 0:128]]
        for b in range(1, D // 128):
            run.append(run[-1] + pr[:, b * 128:(b + 1) * 128])
        return run

    def finish_rows(r0, attn, lo, hi):
        rows = pl.ds(r0, E_ROWS)
        x2 = _r(x_v[rows, :].astype(f32) + mrow(GA, E_ROWS) * attn)
        mu = jnp.sum(x2, axis=1, keepdims=True) * (1.0 / D)
        dc = x2 - mu
        var = _r(jnp.sum(dc * dc, axis=1, keepdims=True) * (1.0 / D))
        den = _r(jnp.sqrt(_r(var + EPS)))
        n = _r(_r(x2 - _r(mu)) * _recip(den))
        h2 = _r(_r(n * mrow(CB1, E_ROWS)) + mrow(SB, E_ROWS))
        x2_v[rows, :] = x2.astype(bf16)
        h_v[rows, :] = h2.astype(bf16)
        ob = (x2 + _r(mrow(GB, E_ROWS) * h2)).astype(bf16)
        out_v[rows, :] = ob
        run = router_parts(h2)
        deps = []
        ot = _tiles(ob)
        n_t = len(ot) * len(ot[0])
        for p in range(len(ot)):
            for b in range(len(ot[0])):
                pos = lo + (hi - lo) * (p * len(ot[0]) + b) / n_t
                deps.append((pos, ot[p][b]))
                for g in (2 * p, 2 * p + 1):
                    deps.append((pos, pltpu.bitcast(run[b][g * 8:(g + 1) * 8, :], u32)))
        return run[-1], deps

    def score_rows(r0, rp, valid, m1, m2):
        r = _r(jnp.sum(rp, axis=1, keepdims=True)) + 0.0
        r = jnp.where(r != r, -jnp.inf, r)
        bits = pltpu.bitcast(jnp.broadcast_to(r, (E_ROWS, 128)), jnp.int32)
        bits = jnp.where(bits < 0, bits ^ 0x7FFF0000, bits)
        idx = r0 + lax.broadcasted_iota(jnp.int32, (E_ROWS, 128), 0)
        key = bits | (0xFFFF - idx)
        if valid is not None:
            key = jnp.where(valid, key, int_min)
        for g in range(E_ROWS // 8):
            kg = key[g * 8:(g + 1) * 8, :]
            m2 = jnp.maximum(m2, jnp.minimum(m1, kg))
            m1 = jnp.maximum(m1, kg)
        return m1, m2

    def out_proj(r0, never, deps):
        rows = pl.ds(r0, E_ROWS)
        lhs = [ohi_v[j, rows, :] for j in range(HH)]
        ds = _col_dots(lhs, lambda j: wo_v[HH * DH:H * DH, j * 128:(j + 1) * 128], D // 128,
                       never, deps)
        return part_v[rows, :] + jnp.concatenate(ds, axis=1)

    def e_body(c, carry):
        b0 = E_SUB * c

        @pl.when(c >= 2)
        def _():
            cp_out(b0 - E_SUB - 1, 1).start()

        @pl.when(c >= 1)
        def _():
            cp_out(b0 - E_SUB, E_SUB - 1).start()

        never = _never(c)
        m1, m2 = top_v[0], top_v[1]
        for t in range(E_SUB):
            m1, m2 = score_rows((b0 - E_SUB - 1 + t) * E_ROWS, rp_v[t],
                                c >= (2 if t == 0 else 1), m1, m2)
        top_v[0] = m1
        top_v[1] = m2
        attn = acc_v[...]
        for t in range(E_SUB):
            prev = jnp.maximum(b0 - 1, 0) if t == 0 else b0 + t - 1
            rp_v[t], deps = finish_rows(pl.multiple_of(prev * E_ROWS, E_ROWS), attn,
                                        E_LO0 if t == 0 else E_LO1, E_HI)
            if t == 0:
                deps.append((E_KEY, pltpu.bitcast(m2, u32)))
            attn = out_proj(pl.multiple_of((b0 + t) * E_ROWS, E_ROWS), never, deps)
        acc_v[...] = attn
        return carry

    lax.fori_loop(0, n_e, e_body, 0)
    n_b = S // E_ROWS
    cp_out(n_b - E_SUB - 1, E_SUB).start()
    m1, m2 = top_v[0], top_v[1]
    for t in range(E_SUB):
        m1, m2 = score_rows((n_b - E_SUB - 1 + t) * E_ROWS, rp_v[t], None, m1, m2)
    rp_last, _ = finish_rows(S - E_ROWS, acc_v[...], 0.0, 1.0)
    m1, m2 = score_rows(S - E_ROWS, rp_last, None, m1, m2)
    cp_out(n_b - 1, 1).start()

    t1 = jnp.max(m1, axis=0, keepdims=True)
    t2 = jnp.max(jnp.where(m1 == t1, m2, m1), axis=0, keepdims=True)
    i1 = (0xFFFF - t1[0, 0]) & (S - 1)
    i2 = (0xFFFF - t2[0, 0]) & (S - 1)
    g1 = pl.multiple_of(i1 & -GRP, GRP)
    g2 = pl.multiple_of(i2 & -GRP, GRP)

    xs = jnp.concatenate([h_v[pl.ds(g1, GRP), :], h_v[pl.ds(g2, GRP), :]], axis=0)

    def act(j):
        fc = slice(j * FC, (j + 1) * FC)
        g = _r(jnp.dot(xs, wg_v[:, fc], preferred_element_type=f32))
        u = _r(jnp.dot(xs, wu_v[:, fc], preferred_element_type=f32))
        return (_r(g * jax.nn.sigmoid(g)) * u).astype(bf16)

    y = None
    a = act(0)
    for j in range(F // FC):
        a_next = act(j + 1) if (j + 1) * FC < F else None
        d = jnp.dot(a, wd_v[j * FC:(j + 1) * FC, 0:D], preferred_element_type=f32)
        y = d if y is None else y + d
        a = a_next
    h2 = xs.astype(f32)
    x2 = jnp.concatenate([x2_v[pl.ds(g1, GRP), :], x2_v[pl.ds(g2, GRP), :]], axis=0).astype(f32)
    r = _r(jnp.sum(router_parts(h2)[-1], axis=1, keepdims=True))
    upd = _r(_r(y) * _r(jax.nn.sigmoid(r)))
    loc = lax.broadcasted_iota(jnp.int32, (2 * GRP, D), 0)
    row = jnp.where(loc < GRP, g1 + loc, g2 + loc - GRP)
    sel = jnp.logical_or(row == i1, row == i2)
    hb = _r(h2 + jnp.where(sel, upd, 0.0))
    fix_v[...] = (x2 + _r(mrow(GB, 2 * GRP) * hb)).astype(bf16)

    cp(out_v, out_v, SEM_OUT).wait()
    fix1 = cp(fix_v.at[pl.ds(0, GRP), :], out_hbm.at[0, pl.ds(g1, GRP), :], SEM_FIX)
    fix2 = cp(fix_v.at[pl.ds(GRP, GRP), :], out_hbm.at[0, pl.ds(g2, GRP), :], SEM_FIX + 1)
    fix1.start()

    @pl.when(g2 != g1)
    def _():
        fix2.start()
        fix2.wait()

    fix1.wait()


@jax.jit
def pallas_adaLN_cond__mha_block_cached__moe_arch_mod__prompt_kernel(
    A_x: jax.Array,
    A_k_cache: jax.Array,
    A_v_cache: jax.Array,
    A_wq: jax.Array,
    A_wo: jax.Array,
    B_x: jax.Array,
    B_w_r: jax.Array,
    B_w_gate: jax.Array,
    B_w_up: jax.Array,
    B_w_down: jax.Array,
    c: jax.Array,
    w_mod: jax.Array,
):
    del B_x
    vm = pltpu.VMEM
    scratch = [
        vm((S, D), bf16),
        vm((S, D), bf16),
        vm((S, D), bf16),
        vm((S, D), bf16),
        vm((H, S, DH), bf16),
        vm((HH, S, DH), bf16),
        vm((HH, S, DH), bf16),
        vm((S, D), f32),
        vm((E_ROWS, D), f32),
        vm((D, P_HEADS * DH + PAD), bf16),
        vm((H, D, DH), bf16),
        vm((H * DH, D + PAD), bf16),
        vm((D, 2 * D + PAD), bf16),
        vm((D, F), bf16),
        vm((D, F), bf16),
        vm((F, D + PAD), bf16),
        vm((4, S, DH), bf16),
        vm((4, S, DH), bf16),
        vm((1, D), bf16),
        vm((D,), bf16),
        vm((GRP, D), bf16),
        vm((8, 7 * D), f32),
        vm((2, 8, 128), jnp.int32),
        vm((E_SUB, E_ROWS, 128), f32),
        vm((2 * GRP, D), bf16),
        pltpu.SemaphoreType.DMA((N_SEM,)),
    ]
    return pl.pallas_call(
        _kernel,
        in_specs=[pl.BlockSpec(memory_space=pl.ANY)] * 11,
        out_specs=pl.BlockSpec(memory_space=pl.ANY),
        out_shape=jax.ShapeDtypeStruct(A_x.shape, A_x.dtype),
        scratch_shapes=scratch,
        compiler_params=pltpu.CompilerParams(vmem_limit_bytes=124 * 1024 * 1024,
                                             disable_bounds_checks=True),
        name="adaln_mha_moe",
    )(A_x, A_k_cache, A_v_cache, A_wq, A_wo, B_w_r, B_w_gate, B_w_up, B_w_down, c, w_mod)
```

```python
import jax
import jax.numpy as jnp
from jax import lax
import jax.experimental.pallas as pl
import jax.experimental.pallas.tpu as pltpu

S = 2048
D = 1024
H = 32
DH = 128
F = 3584
EPS = 1e-5
HH = H // 2

TQ = 256
KR = 512
P_ROWS = 256
P_HEADS = 4
U_ROWS = 128
N_RB = S // U_ROWS
N_QU = (H - P_HEADS) // 4 * N_RB
N_OU = 2 * 2 * N_RB
U_PER_IT = (N_QU + N_OU) // HH
E_ROWS = 64
E_SUB = 4
PACE = 48
GRP = 16
FC = 512
PAD = 128
P_LO, P_HI = 0.25, 0.97
E_LO0, E_LO1, E_HI, E_KEY = 0.3, 0.3, 0.97, 0.2

Q_SCALE = float(DH) ** -0.5 * 1.4426950408889634

f32 = jnp.float32
bf16 = jnp.bfloat16
u32 = jnp.uint32


def _r(x):
    return x.astype(bf16).astype(f32)


def _recip(x):
    r0 = pl.reciprocal(x, approx=True)
    return r0 * (2.0 - x * r0)


def _pace(t):
    for _ in range(PACE):
        t = jnp.minimum(t, jnp.max(t, axis=1, keepdims=True))
    return t


def _tiles(v):
    u = pltpu.bitcast(v, u32)
    return [[u[a * 8:(a + 1) * 8, b * 128:(b + 1) * 128] for b in range(u.shape[1] // 128)]
            for a in range(u.shape[0] // 8)]


def _col_dots(k_tiles, rhs, n_tiles, never, deps):
    n_r = len(k_tiles) // 4
    n_i = k_tiles[0].shape[0] // GRP
    total = n_tiles * n_r * n_i
    at = {}
    for n, (pos, d) in enumerate(deps):
        at.setdefault((min(int(pos * total), total - 1), n % 4), []).append(d)
    outs = []
    for j in range(n_tiles):
        tl = list(k_tiles)
        for k in range(len(k_tiles)):
            base = (j * n_r + k // 4) * n_i
            if not any((base + i, k % 4) in at for i in range(n_i)):
                continue
            tu = pltpu.bitcast(tl[k], u32)
            parts = []
            for i in range(n_i):
                t = tu[i * 8:(i + 1) * 8, :]
                for d in at.get((base + i, k % 4), ()):
                    t = jnp.where(never, d, t)
                parts.append(t)
            tl[k] = pltpu.bitcast(jnp.concatenate(parts, axis=0), bf16)
        outs.append(jnp.dot(jnp.concatenate(tl, axis=1), rhs(j), preferred_element_type=f32))
    return outs


def _never(i):
    return jnp.full((8, 128), i, jnp.int32) > (1 << 20)


def _attention(heads):
    items = [(refs, c) for refs in heads for c in range(S // TQ)]

    def scores(item):
        (q_ref, k_ref, _, _), c = item
        q = (q_ref[c * TQ:(c + 1) * TQ, :] * Q_SCALE).astype(bf16)
        return lax.dot_general(q, k_ref[...], (((1,), (1,)), ((), ())),
                               preferred_element_type=f32)

    def weigh(item, s):
        (_, _, v_ref, o_ref), c = item
        m = jnp.max(s, axis=1, keepdims=True)
        o = None
        lp = None
        for r in range(S // KR):
            p = jnp.exp2(s[:, r * KR:(r + 1) * KR] - m)
            ps = [p[:, j * 128:(j + 1) * 128] for j in range(KR // 128)]
            t = ps[0]
            for x in ps[1:]:
                t = t + x
            lp = t if lp is None else lp + t
            ps[-1] = jnp.minimum(ps[-1], t)
            p = jnp.concatenate(ps, axis=1)
            d = jnp.dot(p.astype(bf16), v_ref[r * KR:(r + 1) * KR, :],
                        preferred_element_type=f32)
            o = d if o is None else o + d
        l = jnp.sum(lp, axis=1, keepdims=True)
        o_ref[c * TQ:(c + 1) * TQ, :] = (o * _recip(l)).astype(bf16)

    s = scores(items[0])
    for n, item in enumerate(items):
        s_next = scores(items[n + 1]) if n + 1 < len(items) else None
        weigh(item, s)
        s = s_next


SEM_C, SEM_WR, SEM_WMA, SEM_X, SEM_WQ, SEM_KV, SEM_BG, SEM_OUT, SEM_FIX, SEM_WMB, SEM_O, N_SEM = (
    0, 1, 2, 6, 14, 17, 21, 25, 26, 28, 30, 32)
WO = H
SA, CA1, GA, SB, CB1, GB, WR = range(7)


def _kernel(x_hbm, k_hbm, v_hbm, wq_hbm, wo_hbm, wr_hbm, wg_hbm, wu_hbm, wd_hbm, c_hbm,
            wm_hbm, out_hbm,
            x_v, h2_v, out_v, l_v, f_v, acc_v, w_v, wg_v, wu_v, wd_v, k_v, v_v, o_v,
            c_v, wr_v, sc_v, mod_v, top_v, rp_v, fix_v, sems):
    n_p = S // P_ROWS
    n_e = S // (E_SUB * E_ROWS)
    pq = P_HEADS * DH

    def cp(src, dst, sem):
        return pltpu.make_async_copy(src, dst, sems.at[sem])

    def cp_c():
        return cp(c_hbm, c_v, SEM_C)

    def cp_wr():
        return cp(wr_hbm, wr_v, SEM_WR)

    def cp_wma(j):
        return cp(wm_hbm.at[:, pl.ds(j * 512, 512)],
                  h2_v.at[pl.ds((j >> 1) * D, D), pl.ds((j & 1) * 512, 512)], SEM_WMA + j)

    def cp_x(i):
        return cp(x_hbm.at[0, pl.ds(i * P_ROWS, P_ROWS), :], x_v.at[pl.ds(i * P_ROWS, P_ROWS), :],
                  SEM_X + i)

    def cp_wqp():
        return cp(wq_hbm.at[:, pl.ds(0, pq)], out_v.at[pl.ds(0, D), pl.ds(0, pq)], SEM_WQ)

    def cp_tile(src, row, col, j, sem):
        return cp(src.at[pl.ds(pl.multiple_of(row * D, D), D), pl.ds(pl.multiple_of(col * DH, DH), DH)],
                  w_v.at[j], sem)

    def tiles_wait(lo, n, sem):
        cp(w_v.at[pl.ds(lo, n)], w_v.at[pl.ds(lo, n)], sem).wait()

    def cp_k(it):
        return cp(k_hbm.at[0, pl.ds(2 * it, 2)], k_v.at[it & 1], SEM_KV + (it & 1))

    def cp_v(it):
        return cp(v_hbm.at[0, pl.ds(2 * it, 2)], v_v.at[it & 1], SEM_KV + 2 + (it & 1))

    def cp_rows(src, dst, i, n, sem):
        return cp(src.at[pl.ds(i * n, n), :], dst.at[pl.ds(i * n, n), pl.ds(0, src.shape[1])], sem)

    def wmb_start(it):
        for k in range(2):
            cp_tile(wm_hbm, 0, 2 * D // DH + 2 * it + k, 2 * (it & 1) + k,
                    SEM_WMB + (it & 1)).start()

    def cp_out(i, n):
        return cp(out_v.at[pl.ds(i * E_ROWS, n * E_ROWS), pl.ds(0, D)],
                  out_hbm.at[0, pl.ds(i * E_ROWS, n * E_ROWS), :], SEM_OUT)

    def mrow(k, n):
        m = mod_v[:, k * D:(k + 1) * D]
        return jnp.concatenate([m] * (n // 8), axis=0)

    cp_c().start()
    cp_wr().start()
    for j in range(4):
        cp_wma(j).start()
    cp_x(0).start()
    cp_wqp().start()
    for i in range(1, n_p):
        cp_x(i).start()
    cp_k(0).start()
    cp_v(0).start()
    wmb_start(0)

    cp_c().wait()
    cp_wr().wait()
    mod_v[:, WR * D:(WR + 1) * D] = jnp.broadcast_to(wr_v[...].astype(f32).reshape(1, D), (8, D))
    int_min = jnp.iinfo(jnp.int32).min
    top_v[...] = jnp.full(top_v.shape, int_min, jnp.int32)
    acc_v[...] = jnp.zeros(acc_v.shape, f32)
    rp_v[...] = jnp.zeros(rp_v.shape, f32)
    cf = c_v[...].astype(f32)
    sc_v[...] = jnp.broadcast_to(cf * jax.nn.sigmoid(cf), (GRP, D)).astype(bf16)

    def wma_body(j, carry):
        cp_wma(j).wait()
        cols = pl.ds(pl.multiple_of(j * 512, 512), 512)
        w = h2_v[pl.ds(pl.multiple_of((j >> 1) * D, D), D),
                 pl.ds(pl.multiple_of((j & 1) * 512, 512), 512)]
        mj = jnp.dot(sc_v[...], w, preferred_element_type=f32)
        mod_v[:, cols] = _r(_r(mj[0:8, :]) + jnp.where(j >= 2, 1.0, 0.0))
        return carry

    lax.fori_loop(0, 4, wma_body, 0)

    def ln1(i):
        rows = pl.ds(pl.multiple_of(i * P_ROWS, P_ROWS), P_ROWS)
        x = x_v[rows, :].astype(f32)
        mu = jnp.sum(x, axis=1, keepdims=True) * (1.0 / D)
        d = x - mu
        var = jnp.sum(d * d, axis=1, keepdims=True) * (1.0 / D)
        n = d * lax.rsqrt(var + EPS)
        h = (n * mrow(CA1, P_ROWS) + mrow(SA, P_ROWS)).astype(bf16)
        for k in range(D // 128):
            l_v[k, rows, :] = h[:, k * 128:(k + 1) * 128]
        return h

    cp_x(0).wait()
    ln1(0)
    cp_wqp().wait()

    def p_body(i, carry):
        @pl.when(i + 1 < n_p)
        def _():
            cp_x(i + 1).wait()

        rows = pl.ds(pl.multiple_of(i * P_ROWS, P_ROWS), P_ROWS)
        lhs = [l_v[k, rows, :] for k in range(D // 128)]
        tl = [t for row in _tiles(ln1(jnp.minimum(i + 1, n_p - 1))) for t in row]
        deps = [(P_LO + (P_HI - P_LO) * n / len(tl), t) for n, t in enumerate(tl)]
        qs = _col_dots(lhs, lambda j: out_v[0:D, j * DH:(j + 1) * DH], P_HEADS, _never(i), deps)
        for j in range(P_HEADS):
            f_v[j, rows, :] = qs[j]

        @pl.when(i + 1 < n_p)
        def _():
            for k in range(4):
                hd = P_HEADS + 4 * i + k
                cp_tile(wq_hbm, 0, hd, hd, SEM_WQ + jnp.where(i < 1, 1, 2)).start()

        return carry

    lax.fori_loop(0, n_p, p_body, 0)
    cp_k(1).start()
    cp_v(1).start()
    wmb_start(1)
    tiles_wait(P_HEADS, 4, SEM_WQ + 1)

    def m_body(it, carry):
        @pl.when(it == 1)
        def _():
            tiles_wait(P_HEADS + 4, H - P_HEADS - 4, SEM_WQ + 2)

        @pl.when(it == N_QU // U_PER_IT)
        def _():
            tiles_wait(WO, H, SEM_BG)

        @pl.when(jnp.logical_or(it == 6, it == 10))
        def _():
            cp(out_hbm.at[0], out_hbm.at[0], SEM_O).wait()

        @pl.when(jnp.logical_or(it == 8, it == 12))
        def _():
            dst = l_v.at[pl.ds(24 - 2 * it, 8)]
            cp(dst, dst, SEM_O + 1).wait()

        cp_k(it).wait()
        cp_v(it).wait()
        tiles_wait(2 * (it & 1), 2, SEM_WMB + (it & 1))
        slot = it & 1

        def unit(u, js):
            g = it * U_PER_IT + u
            is_q = g < N_QU
            blk4 = (g >> 4) * 4
            fb = blk4 + jnp.where(is_q, P_HEADS, -(H - P_HEADS))
            wb = blk4 + P_HEADS
            lb = jnp.where(is_q, 0, 8 - (fb & 8))
            r0 = pl.multiple_of((g & (N_RB - 1)) * U_ROWS, U_ROWS)
            lhs = jnp.concatenate([l_v[lb + k, pl.ds(r0, U_ROWS), :] for k in range(8)], axis=1)
            return [(fb + j, r0, jnp.dot(lhs, w_v[wb + j], preferred_element_type=f32))
                    for j in js]

        def put(tiles):
            for j, r0, v in tiles:
                f_v[j, pl.ds(r0, v.shape[0]), :] = v

        late = unit(0, [0])
        _attention([(f_v.at[2 * it + e], k_v.at[slot, e], v_v.at[slot, e],
                     o_v.at[(2 * it + e) & (HH - 1)]) for e in range(2)])
        one = jnp.where(it >> 2 == CB1 - GA, 1.0, 0.0)
        mb = None
        for u in range(U_PER_IT):
            tiles = unit(u, range(1 if u == 0 else 0, 4))
            if u == 0:
                j, r0, v = tiles[0]
                late.append((j, r0, _pace(v[0:8, :])))
                tiles[0] = (j, r0 + 8, v[8:, :])
            put(tiles)
            if u == U_PER_IT - 2:
                put(late)
            if u < 4:
                e = u // 2
                ks = slice(u % 2 * 512, (u % 2 + 1) * 512)
                d = jnp.dot(sc_v[:, ks], w_v[2 * slot + e, ks, :],
                            preferred_element_type=f32)[0:8, :]
                if u % 2 == 0:
                    mb = d
                else:
                    cols = pl.ds(pl.multiple_of(GA * D + (2 * it + e) * 128, 128), 128)
                    mod_v[:, cols] = _r(_r(mb + d) + one)

        @pl.when(it + 2 < HH)
        def _():
            cp_k(it + 2).start()
            cp_v(it + 2).start()
            wmb_start(it + 2)

        @pl.when(jnp.logical_or(it == 4, it == 8))
        def _():
            for k in range(8):
                cp(o_v.at[2 * it - 8 + k], out_hbm.at[0, :, pl.ds(k * DH, DH)], SEM_O).start()

        @pl.when(jnp.logical_or(it == 6, it == 10))
        def _():
            for k in range(8):
                cp(out_hbm.at[0, :, pl.ds(k * DH, DH)], l_v.at[20 - 2 * it + k], SEM_O + 1).start()

        @pl.when(it < 8)
        def _():
            for k in range(4):
                t = 4 * it + k
                cp_tile(wo_hbm, t >> 3, t & 7, WO + t, SEM_BG).start()

        for n, (src, dst) in enumerate(((wg_hbm, wg_v), (wu_hbm, wu_v), (wd_hbm, wd_v))):
            @pl.when(it >> 1 == n + 4)
            def _():
                cp_rows(src, dst, it & 1, src.shape[0] // 2, SEM_BG + 1 + n).start()

        return carry

    lax.fori_loop(0, HH, m_body, 0)

    cp(wg_v, wg_v, SEM_BG + 1).wait()
    cp(wu_v, wu_v, SEM_BG + 2).wait()
    cp(wd_hbm, wd_v.at[:, pl.ds(0, D)], SEM_BG + 3).wait()

    def router_parts(h2):
        pr = h2 * mrow(WR, h2.shape[0])
        run = [pr[:, 0:128]]
        for b in range(1, D // 128):
            run.append(run[-1] + pr[:, b * 128:(b + 1) * 128])
        return run

    def finish_rows(r0, attn, lo, hi):
        rows = pl.ds(r0, E_ROWS)
        x2 = _r(x_v[rows, :].astype(f32) + mrow(GA, E_ROWS) * attn)
        mu = jnp.sum(x2, axis=1, keepdims=True) * (1.0 / D)
        dc = x2 - mu
        var = _r(jnp.sum(dc * dc, axis=1, keepdims=True) * (1.0 / D))
        den = _r(jnp.sqrt(_r(var + EPS)))
        n = _r(_r(x2 - _r(mu)) * _recip(den))
        h2 = _r(_r(n * mrow(CB1, E_ROWS)) + mrow(SB, E_ROWS))
        x_v[rows, :] = x2.astype(bf16)
        h2_v[rows, 0:D] = h2.astype(bf16)
        ob = (x2 + _r(mrow(GB, E_ROWS) * h2)).astype(bf16)
        out_v[rows, 0:D] = ob
        run = router_parts(h2)
        deps = []
        ot = _tiles(ob)
        n_t = len(ot) * len(ot[0])
        for p in range(len(ot)):
            for b in range(len(ot[0])):
                pos = lo + (hi - lo) * (p * len(ot[0]) + b) / n_t
                deps.append((pos, ot[p][b]))
                for g in (2 * p, 2 * p + 1):
                    deps.append((pos, pltpu.bitcast(run[b][g * 8:(g + 1) * 8, :], u32)))
        return run[-1], deps

    def score_rows(r0, rp, valid, m1, m2):
        r = _r(jnp.sum(rp, axis=1, keepdims=True)) + 0.0
        r = jnp.where(r != r, -jnp.inf, r)
        bits = pltpu.bitcast(jnp.broadcast_to(r, (E_ROWS, 128)), jnp.int32)
        bits = jnp.where(bits < 0, bits ^ 0x7FFF0000, bits)
        idx = r0 + lax.broadcasted_iota(jnp.int32, (E_ROWS, 128), 0)
        key = bits | (0xFFFF - idx)
        if valid is not None:
            key = jnp.where(valid, key, int_min)
        for g in range(E_ROWS // 8):
            kg = key[g * 8:(g + 1) * 8, :]
            m2 = jnp.maximum(m2, jnp.minimum(m1, kg))
            m1 = jnp.maximum(m1, kg)
        return m1, m2

    def out_proj(r0, never, deps):
        rows = pl.ds(r0, E_ROWS)
        lhs = [o_v[j, rows, :] for j in range(HH)]
        ds = _col_dots(lhs, lambda j: jnp.concatenate([w_v[WO + 16 + j], w_v[WO + 24 + j]], axis=0),
                       D // 128, never, deps)
        return jnp.concatenate([f_v[j, rows, :] + f_v[8 + j, rows, :] + ds[j]
                                for j in range(D // 128)], axis=1)

    def e_body(c, carry):
        b0 = E_SUB * c

        @pl.when(c >= 2)
        def _():
            cp_out(b0 - E_SUB - 1, 1).start()

        @pl.when(c >= 1)
        def _():
            cp_out(b0 - E_SUB, E_SUB - 1).start()

        never = _never(c)
        m1, m2 = top_v[0], top_v[1]
        for t in range(E_SUB):
            m1, m2 = score_rows((b0 - E_SUB - 1 + t) * E_ROWS, rp_v[t],
                                c >= (2 if t == 0 else 1), m1, m2)
        top_v[0] = m1
        top_v[1] = m2
        attn = acc_v[...]
        for t in range(E_SUB):
            prev = jnp.maximum(b0 - 1, 0) if t == 0 else b0 + t - 1
            rp_v[t], deps = finish_rows(pl.multiple_of(prev * E_ROWS, E_ROWS), attn,
                                        E_LO0 if t == 0 else E_LO1, E_HI)
            if t == 0:
                deps.append((E_KEY, pltpu.bitcast(m2, u32)))
            attn = out_proj(pl.multiple_of((b0 + t) * E_ROWS, E_ROWS), never, deps)
        acc_v[...] = attn
        return carry

    lax.fori_loop(0, n_e, e_body, 0)
    n_b = S // E_ROWS
    cp_out(n_b - E_SUB - 1, E_SUB).start()
    m1, m2 = top_v[0], top_v[1]
    for t in range(E_SUB):
        m1, m2 = score_rows((n_b - E_SUB - 1 + t) * E_ROWS, rp_v[t], None, m1, m2)
    rp_last, _ = finish_rows(S - E_ROWS, acc_v[...], 0.0, 1.0)
    m1, m2 = score_rows(S - E_ROWS, rp_last, None, m1, m2)
    cp_out(n_b - 1, 1).start()

    t1 = jnp.max(m1, axis=0, keepdims=True)
    t2 = jnp.max(jnp.where(m1 == t1, m2, m1), axis=0, keepdims=True)
    i1 = (0xFFFF - t1[0, 0]) & (S - 1)
    i2 = (0xFFFF - t2[0, 0]) & (S - 1)
    g1 = pl.multiple_of(i1 & -GRP, GRP)
    g2 = pl.multiple_of(i2 & -GRP, GRP)

    xs = jnp.concatenate([h2_v[pl.ds(g1, GRP), 0:D], h2_v[pl.ds(g2, GRP), 0:D]], axis=0)

    def act(j):
        fc = slice(j * FC, (j + 1) * FC)
        g = _r(jnp.dot(xs, wg_v[:, fc], preferred_element_type=f32))
        u = _r(jnp.dot(xs, wu_v[:, fc], preferred_element_type=f32))
        return (_r(g * jax.nn.sigmoid(g)) * u).astype(bf16)

    y = None
    a = act(0)
    for j in range(F // FC):
        a_next = act(j + 1) if (j + 1) * FC < F else None
        d = jnp.dot(a, wd_v[j * FC:(j + 1) * FC, 0:D], preferred_element_type=f32)
        y = d if y is None else y + d
        a = a_next
    h2 = xs.astype(f32)
    x2 = jnp.concatenate([x_v[pl.ds(g1, GRP), :], x_v[pl.ds(g2, GRP), :]], axis=0).astype(f32)
    r = _r(jnp.sum(router_parts(h2)[-1], axis=1, keepdims=True))
    upd = _r(_r(y) * _r(jax.nn.sigmoid(r)))
    loc = lax.broadcasted_iota(jnp.int32, (2 * GRP, D), 0)
    row = jnp.where(loc < GRP, g1 + loc, g2 + loc - GRP)
    sel = jnp.logical_or(row == i1, row == i2)
    hb = _r(h2 + jnp.where(sel, upd, 0.0))
    fix_v[...] = (x2 + _r(mrow(GB, 2 * GRP) * hb)).astype(bf16)

    cp(out_v.at[:, pl.ds(0, D)], out_hbm.at[0], SEM_OUT).wait()
    fix1 = cp(fix_v.at[pl.ds(0, GRP), :], out_hbm.at[0, pl.ds(g1, GRP), :], SEM_FIX)
    fix2 = cp(fix_v.at[pl.ds(GRP, GRP), :], out_hbm.at[0, pl.ds(g2, GRP), :], SEM_FIX + 1)
    fix1.start()

    @pl.when(g2 != g1)
    def _():
        fix2.start()
        fix2.wait()

    fix1.wait()


@jax.jit
def pallas_adaLN_cond__mha_block_cached__moe_arch_mod__prompt_kernel(
    A_x: jax.Array,
    A_k_cache: jax.Array,
    A_v_cache: jax.Array,
    A_wq: jax.Array,
    A_wo: jax.Array,
    B_x: jax.Array,
    B_w_r: jax.Array,
    B_w_gate: jax.Array,
    B_w_up: jax.Array,
    B_w_down: jax.Array,
    c: jax.Array,
    w_mod: jax.Array,
):
    del B_x
    vm = pltpu.VMEM
    scratch = [
        vm((S, D), bf16),
        vm((S, D + PAD), bf16),
        vm((S, D + PAD), bf16),
        vm((HH, S, DH), bf16),
        vm((H, S, DH), f32),
        vm((E_ROWS, D), f32),
        vm((2 * H, D, DH), bf16),
        vm((D, F), bf16),
        vm((D, F), bf16),
        vm((F, D + PAD), bf16),
        vm((2, 2, S, DH), bf16),
        vm((2, 2, S, DH), bf16),
        vm((HH, S, DH), bf16),
        vm((1, D), bf16),
        vm((D,), bf16),
        vm((GRP, D), bf16),
        vm((8, 7 * D), f32),
        vm((2, 8, 128), jnp.int32),
        vm((E_SUB, E_ROWS, 128), f32),
        vm((2 * GRP, D), bf16),
        pltpu.SemaphoreType.DMA((N_SEM,)),
    ]
    return pl.pallas_call(
        _kernel,
        in_specs=[pl.BlockSpec(memory_space=pl.ANY)] * 11,
        out_specs=pl.BlockSpec(memory_space=pl.ANY),
        out_shape=jax.ShapeDtypeStruct(A_x.shape, A_x.dtype),
        scratch_shapes=scratch,
        compiler_params=pltpu.CompilerParams(vmem_limit_bytes=124 * 1024 * 1024,
                                             disable_bounds_checks=True),
        name="adaln_mha_moe",
    )(A_x, A_k_cache, A_v_cache, A_wq, A_wo, B_w_r, B_w_gate, B_w_up, B_w_down, c, w_mod)
```

```python
import jax
import jax.numpy as jnp
from jax import lax
import jax.experimental.pallas as pl
import jax.experimental.pallas.tpu as pltpu

S = 2048
D = 1024
H = 32
DH = 128
F = 3584
EPS = 1e-5
HH = H // 2

TQ = 256
KR = 512
P_ROWS = 256
P_HEADS = 4
U_ROWS = 128
N_RB = S // U_ROWS
N_QU = (H - P_HEADS) // 4 * N_RB
N_OU = 2 * 2 * N_RB
U_PER_IT = (N_QU + N_OU) // HH
E_ROWS = 64
E_SUB = 4
PACE = 48
MV_STEP, MV_U0 = 2, 7
GRP = 16
FC = 512
PAD = 128
P_LO, P_HI = 0.25, 0.97
E_LO0, E_LO1, E_HI, E_KEY, E_RUN = 0.35, 0.3, 0.97, 0.3, 2

Q_SCALE = float(DH) ** -0.5 * 1.4426950408889634

f32 = jnp.float32
bf16 = jnp.bfloat16
u32 = jnp.uint32


def _r(x):
    return x.astype(bf16).astype(f32)


def _recip(x):
    r0 = pl.reciprocal(x, approx=True)
    return r0 * (2.0 - x * r0)


def _pace(t):
    for _ in range(PACE):
        t = jnp.minimum(t, jnp.max(t, axis=1, keepdims=True))
    return t


def _tiles(v):
    u = pltpu.bitcast(v, u32)
    return [[u[a * 8:(a + 1) * 8, b * 128:(b + 1) * 128] for b in range(u.shape[1] // 128)]
            for a in range(u.shape[0] // 8)]


def _col_dots(k_tiles, rhs, n_tiles, never, deps):
    n_r = len(k_tiles) // 4
    n_i = k_tiles[0].shape[0] // GRP
    total = n_tiles * n_r * n_i
    at = {}
    for n, (pos, d) in enumerate(deps):
        at.setdefault((min(int(pos * total), total - 1), n % 4), []).append(d)
    outs = []
    for j in range(n_tiles):
        tl = list(k_tiles)
        for k in range(len(k_tiles)):
            base = (j * n_r + k // 4) * n_i
            if not any((base + i, k % 4) in at for i in range(n_i)):
                continue
            tu = pltpu.bitcast(tl[k], u32)
            parts = []
            for i in range(n_i):
                t = tu[i * 8:(i + 1) * 8, :]
                for d in at.get((base + i, k % 4), ()):
                    t = jnp.where(never, d, t)
                parts.append(t)
            tl[k] = pltpu.bitcast(jnp.concatenate(parts, axis=0), bf16)
        outs.append(jnp.dot(jnp.concatenate(tl, axis=1), rhs(j), preferred_element_type=f32))
    return outs


def _matvec(a_ref, w_refs):
    accs = [None] * len(w_refs)
    steps = []
    for s in range(D // GRP):
        a = a_ref[s * GRP:(s + 1) * GRP, :]
        for n, w in enumerate(w_refs):
            t = w[s * GRP:(s + 1) * GRP, :].astype(f32) * a
            accs[n] = t if accs[n] is None else accs[n] + t
        if s % MV_STEP == MV_STEP - 1:
            steps += [t[0] for acc in accs for t in _tiles(acc)]
    res = [jnp.broadcast_to(jnp.sum(acc, axis=0, keepdims=True), (8, 128)) for acc in accs]
    return res, steps


def _lane_bcast(row):
    return jnp.concatenate([row] * 16, axis=0).T


def _never(i):
    return jnp.full((8, 128), i, jnp.int32) > (1 << 20)


def _attention(heads):
    items = [(refs, c) for refs in heads for c in range(S // TQ)]

    def scores(item):
        (q_ref, k_ref, _, _), c = item
        q = (q_ref[c * TQ:(c + 1) * TQ, :] * Q_SCALE).astype(bf16)
        return lax.dot_general(q, k_ref[...], (((1,), (1,)), ((), ())),
                               preferred_element_type=f32)

    def weigh(item, s):
        (_, _, v_ref, o_ref), c = item
        m = jnp.max(s, axis=1, keepdims=True)
        o = None
        lp = None
        for r in range(S // KR):
            p = jnp.exp2(s[:, r * KR:(r + 1) * KR] - m)
            ps = [p[:, j * 128:(j + 1) * 128] for j in range(KR // 128)]
            t = ps[0]
            for x in ps[1:]:
                t = t + x
            lp = t if lp is None else lp + t
            ps[-1] = jnp.minimum(ps[-1], t)
            p = jnp.concatenate(ps, axis=1)
            d = jnp.dot(p.astype(bf16), v_ref[r * KR:(r + 1) * KR, :],
                        preferred_element_type=f32)
            o = d if o is None else o + d
        l = jnp.sum(lp, axis=1, keepdims=True)
        o_ref[c * TQ:(c + 1) * TQ, :] = (o * _recip(l)).astype(bf16)

    s = scores(items[0])
    for n, item in enumerate(items):
        s_next = scores(items[n + 1]) if n + 1 < len(items) else None
        weigh(item, s)
        s = s_next


SEM_C, SEM_WR, SEM_WMA, SEM_X, SEM_WQ, SEM_KV, SEM_BG, SEM_OUT, SEM_FIX, SEM_WMB, SEM_O, N_SEM = (
    0, 1, 2, 6, 14, 17, 21, 25, 26, 28, 30, 32)
WO = H
SA, CA1, GA, SB, CB1, GB, WR = range(7)


def _kernel(x_hbm, k_hbm, v_hbm, wq_hbm, wo_hbm, wr_hbm, wg_hbm, wu_hbm, wd_hbm, c_hbm,
            wm_hbm, out_hbm,
            x_v, h2_v, out_v, l_v, f_v, acc_v, w_v, wg_v, wu_v, wd_v, k_v, v_v, o_v,
            c_v, wr_v, sc_v, scb_v, mod_v, top_v, rp_v, fix_v, sems):
    n_p = S // P_ROWS
    n_e = S // (E_SUB * E_ROWS)
    pq = P_HEADS * DH

    def cp(src, dst, sem):
        return pltpu.make_async_copy(src, dst, sems.at[sem])

    def cp_c():
        return cp(c_hbm, c_v, SEM_C)

    def cp_wr():
        return cp(wr_hbm, wr_v, SEM_WR)

    def cp_wma(j):
        return cp(wm_hbm.at[:, pl.ds(j * 512, 512)],
                  h2_v.at[pl.ds((j >> 1) * D, D), pl.ds((j & 1) * 512, 512)], SEM_WMA + j)

    def cp_x(i):
        return cp(x_hbm.at[0, pl.ds(i * P_ROWS, P_ROWS), :], x_v.at[pl.ds(i * P_ROWS, P_ROWS), :],
                  SEM_X + i)

    def cp_wqp():
        return cp(wq_hbm.at[:, pl.ds(0, pq)], out_v.at[pl.ds(0, D), pl.ds(0, pq)], SEM_WQ)

    def cp_tile(src, row, col, j, sem):
        return cp(src.at[pl.ds(pl.multiple_of(row * D, D), D), pl.ds(pl.multiple_of(col * DH, DH), DH)],
                  w_v.at[j], sem)

    def tiles_wait(lo, n, sem):
        cp(w_v.at[pl.ds(lo, n)], w_v.at[pl.ds(lo, n)], sem).wait()

    def cp_k(it):
        return cp(k_hbm.at[0, pl.ds(2 * it, 2)], k_v.at[it & 1], SEM_KV + (it & 1))

    def cp_v(it):
        return cp(v_hbm.at[0, pl.ds(2 * it, 2)], v_v.at[it & 1], SEM_KV + 2 + (it & 1))

    def cp_rows(src, dst, i, n, sem):
        return cp(src.at[pl.ds(i * n, n), :], dst.at[pl.ds(i * n, n), pl.ds(0, src.shape[1])], sem)

    def wmb_start(it):
        for k in range(2):
            cp_tile(wm_hbm, 0, 2 * D // DH + 2 * it + k, 2 * (it & 1) + k,
                    SEM_WMB + (it & 1)).start()

    def cp_out(i, n):
        return cp(out_v.at[pl.ds(i * E_ROWS, n * E_ROWS), pl.ds(0, D)],
                  out_hbm.at[0, pl.ds(i * E_ROWS, n * E_ROWS), :], SEM_OUT)

    def mrow(k, n):
        m = mod_v[:, k * D:(k + 1) * D]
        return jnp.concatenate([m] * (n // 8), axis=0)

    cp_c().start()
    cp_wr().start()
    for j in range(4):
        cp_wma(j).start()
    cp_x(0).start()
    cp_wqp().start()
    for i in range(1, n_p):
        cp_x(i).start()
    cp_k(0).start()
    cp_v(0).start()
    wmb_start(0)

    cp_c().wait()
    cp_wr().wait()
    mod_v[:, WR * D:(WR + 1) * D] = jnp.broadcast_to(wr_v[...].astype(f32).reshape(1, D), (8, D))
    int_min = jnp.iinfo(jnp.int32).min
    top_v[...] = jnp.full(top_v.shape, int_min, jnp.int32)
    acc_v[...] = jnp.zeros(acc_v.shape, f32)
    rp_v[...] = jnp.zeros(rp_v.shape, f32)
    cf = c_v[...].astype(f32)
    sc = jnp.broadcast_to(_r(cf * jax.nn.sigmoid(cf)), (8, D))
    sc_v[...] = jnp.concatenate([sc, sc], axis=0).astype(bf16)
    scb_v[...] = _lane_bcast(sc)

    def wma_body(j, carry):
        cp_wma(j).wait()
        cols = pl.ds(pl.multiple_of(j * 512, 512), 512)
        w = h2_v[pl.ds(pl.multiple_of((j >> 1) * D, D), D),
                 pl.ds(pl.multiple_of((j & 1) * 512, 512), 512)]
        mj = jnp.dot(sc_v[...], w, preferred_element_type=f32)
        mod_v[:, cols] = _r(_r(mj[0:8, :]) + jnp.where(j >= 2, 1.0, 0.0))
        return carry

    lax.fori_loop(0, 4, wma_body, 0)

    def ln1(i):
        rows = pl.ds(pl.multiple_of(i * P_ROWS, P_ROWS), P_ROWS)
        x = x_v[rows, :].astype(f32)
        mu = jnp.sum(x, axis=1, keepdims=True) * (1.0 / D)
        d = x - mu
        var = jnp.sum(d * d, axis=1, keepdims=True) * (1.0 / D)
        n = d * lax.rsqrt(var + EPS)
        h = (n * mrow(CA1, P_ROWS) + mrow(SA, P_ROWS)).astype(bf16)
        for k in range(D // 128):
            l_v[k, rows, :] = h[:, k * 128:(k + 1) * 128]
        return h

    cp_x(0).wait()
    ln1(0)
    cp_wqp().wait()

    def p_body(i, carry):
        @pl.when(i + 1 < n_p)
        def _():
            cp_x(i + 1).wait()

        rows = pl.ds(pl.multiple_of(i * P_ROWS, P_ROWS), P_ROWS)
        lhs = [l_v[k, rows, :] for k in range(D // 128)]
        tl = [t for row in _tiles(ln1(jnp.minimum(i + 1, n_p - 1))) for t in row]
        deps = [(P_LO + (P_HI - P_LO) * n / len(tl), t) for n, t in enumerate(tl)]
        qs = _col_dots(lhs, lambda j: out_v[0:D, j * DH:(j + 1) * DH], P_HEADS, _never(i), deps)
        for j in range(P_HEADS):
            f_v[j, rows, :] = qs[j]

        @pl.when(i + 1 < n_p)
        def _():
            for k in range(4):
                hd = P_HEADS + 4 * i + k
                cp_tile(wq_hbm, 0, hd, hd, SEM_WQ + jnp.where(i < 1, 1, 2)).start()

        return carry

    lax.fori_loop(0, n_p, p_body, 0)
    cp_k(1).start()
    cp_v(1).start()
    wmb_start(1)
    tiles_wait(P_HEADS, 4, SEM_WQ + 1)

    def m_body(it, carry):
        @pl.when(it == 1)
        def _():
            tiles_wait(P_HEADS + 4, H - P_HEADS - 4, SEM_WQ + 2)

        @pl.when(it == N_QU // U_PER_IT)
        def _():
            tiles_wait(WO, H, SEM_BG)

        @pl.when(jnp.logical_or(it == 6, it == 10))
        def _():
            cp(out_hbm.at[0], out_hbm.at[0], SEM_O).wait()

        @pl.when(jnp.logical_or(it == 8, it == 12))
        def _():
            dst = l_v.at[pl.ds(24 - 2 * it, 8)]
            cp(dst, dst, SEM_O + 1).wait()

        cp_k(it).wait()
        cp_v(it).wait()
        tiles_wait(2 * (it & 1), 2, SEM_WMB + (it & 1))
        slot = it & 1

        def unit(u, js, deps=()):
            g = it * U_PER_IT + u
            is_q = g < N_QU
            blk4 = (g >> 4) * 4
            fb = blk4 + jnp.where(is_q, P_HEADS, -(H - P_HEADS))
            wb = blk4 + P_HEADS
            lb = jnp.where(is_q, 0, 8 - (fb & 8))
            r0 = pl.multiple_of((g & (N_RB - 1)) * U_ROWS, U_ROWS)
            lhs = [l_v[lb + k, pl.ds(r0, U_ROWS), :] for k in range(8)]
            res = _col_dots(lhs, lambda n: w_v[wb + js[n]], len(js), never, deps)
            return [(fb + j, r0, v) for j, v in zip(js, res)]

        def put(tiles):
            for j, r0, v in tiles:
                f_v[j, pl.ds(r0, v.shape[0]), :] = v

        never = _never(it)
        late = unit(0, [0])
        _attention([(f_v.at[2 * it + e], k_v.at[slot, e], v_v.at[slot, e],
                     o_v.at[(2 * it + e) & (HH - 1)]) for e in range(2)])
        mb, steps = _matvec(scb_v, [w_v.at[2 * slot + e] for e in range(2)])
        one = jnp.where(it >> 2 == CB1 - GA, 1.0, 0.0)
        for e in range(2):
            cols = pl.ds(pl.multiple_of(GA * D + (2 * it + e) * 128, 128), 128)
            mod_v[:, cols] = _r(_r(mb[e]) + one)
        span = (U_PER_IT - MV_U0) * 0.9 / len(steps)
        steps = [(MV_U0 + n * span, t) for n, t in enumerate(steps)]
        for u in range(U_PER_IT):
            tiles = unit(u, list(range(1 if u == 0 else 0, 4)),
                         [(pos - u, t) for pos, t in steps if u <= pos < u + 1])
            if u == 0:
                j, r0, v = tiles[0]
                late.append((j, r0, _pace(v[0:8, :])))
                tiles[0] = (j, r0 + 8, v[8:, :])
            put(tiles)
            if u == U_PER_IT - 2:
                put(late)

        @pl.when(it + 2 < HH)
        def _():
            cp_k(it + 2).start()
            cp_v(it + 2).start()
            wmb_start(it + 2)

        @pl.when(jnp.logical_or(it == 4, it == 8))
        def _():
            for k in range(8):
                cp(o_v.at[2 * it - 8 + k], out_hbm.at[0, :, pl.ds(k * DH, DH)], SEM_O).start()

        @pl.when(jnp.logical_or(it == 6, it == 10))
        def _():
            for k in range(8):
                cp(out_hbm.at[0, :, pl.ds(k * DH, DH)], l_v.at[20 - 2 * it + k], SEM_O + 1).start()

        @pl.when(it < 8)
        def _():
            for k in range(4):
                t = 4 * it + k
                cp_tile(wo_hbm, t >> 3, t & 7, WO + t, SEM_BG).start()

        for n, (src, dst) in enumerate(((wg_hbm, wg_v), (wu_hbm, wu_v), (wd_hbm, wd_v))):
            @pl.when(it >> 1 == n + 4)
            def _():
                cp_rows(src, dst, it & 1, src.shape[0] // 2, SEM_BG + 1 + n).start()

        return carry

    lax.fori_loop(0, HH, m_body, 0)

    cp(wg_v, wg_v, SEM_BG + 1).wait()
    cp(wu_v, wu_v, SEM_BG + 2).wait()
    cp(wd_hbm, wd_v.at[:, pl.ds(0, D)], SEM_BG + 3).wait()

    def router_parts(h2):
        pr = h2 * mrow(WR, h2.shape[0])
        run = [pr[:, 0:128]]
        for b in range(1, D // 128):
            run.append(run[-1] + pr[:, b * 128:(b + 1) * 128])
        return run

    def finish_rows(r0, attn, lo, hi):
        rows = pl.ds(r0, E_ROWS)
        x2 = _r(x_v[rows, :].astype(f32) + mrow(GA, E_ROWS) * attn)
        mu = jnp.sum(x2, axis=1, keepdims=True) * (1.0 / D)
        dc = x2 - mu
        var = _r(jnp.sum(dc * dc, axis=1, keepdims=True) * (1.0 / D))
        den = _r(jnp.sqrt(_r(var + EPS)))
        n = _r(_r(x2 - _r(mu)) * _recip(den))
        h2 = _r(_r(n * mrow(CB1, E_ROWS)) + mrow(SB, E_ROWS))
        x2b = x2.astype(bf16)
        for k in range(D // 128):
            l_v[k, rows, :] = x2b[:, k * 128:(k + 1) * 128]
        h2_v[rows, 0:D] = h2.astype(bf16)
        of = x2 + _r(mrow(GB, E_ROWS) * h2)
        out_v[rows, 0:D] = of.astype(bf16)
        run = router_parts(h2)
        deps = []
        ot = _tiles(of)
        n_t = len(ot) * len(ot[0])
        for g in range(len(ot)):
            for b in range(len(ot[0])):
                pos = lo + (hi - lo) * (g * len(ot[0]) + b) / n_t
                deps.append((pos, ot[g][b]))
                if b % E_RUN == E_RUN - 1:
                    deps.append((pos, pltpu.bitcast(run[b][g * 8:(g + 1) * 8, :], u32)))
        return run[-1], deps

    def score_rows(r0, rp, valid, m1, m2):
        r = _r(jnp.sum(rp, axis=1, keepdims=True)) + 0.0
        r = jnp.where(r != r, -jnp.inf, r)
        bits = pltpu.bitcast(jnp.broadcast_to(r, (E_ROWS, 128)), jnp.int32)
        bits = jnp.where(bits < 0, bits ^ 0x7FFF0000, bits)
        idx = r0 + lax.broadcasted_iota(jnp.int32, (E_ROWS, 128), 0)
        key = bits | (0xFFFF - idx)
        if valid is not None:
            key = jnp.where(valid, key, int_min)
        for g in range(E_ROWS // 8):
            kg = key[g * 8:(g + 1) * 8, :]
            m2 = jnp.maximum(m2, jnp.minimum(m1, kg))
            m1 = jnp.maximum(m1, kg)
        return m1, m2

    def out_proj(r0, never, deps):
        rows = pl.ds(r0, E_ROWS)
        lhs = [o_v[j, rows, :] for j in range(HH)]
        ds = _col_dots(lhs, lambda j: jnp.concatenate([w_v[WO + 16 + j], w_v[WO + 24 + j]], axis=0),
                       D // 128, never, deps)
        return jnp.concatenate([f_v[j, rows, :] + f_v[8 + j, rows, :] + ds[j]
                                for j in range(D // 128)], axis=1)

    def e_body(c, carry):
        b0 = E_SUB * c

        @pl.when(c >= 2)
        def _():
            cp_out(b0 - E_SUB - 1, 1).start()

        @pl.when(c >= 1)
        def _():
            cp_out(b0 - E_SUB, E_SUB - 1).start()

        never = _never(c)
        m1, m2 = top_v[0], top_v[1]
        for t in range(E_SUB):
            m1, m2 = score_rows((b0 - E_SUB - 1 + t) * E_ROWS, rp_v[t],
                                c >= (2 if t == 0 else 1), m1, m2)
        top_v[0] = m1
        top_v[1] = m2
        attn = acc_v[...]
        for t in range(E_SUB):
            prev = jnp.maximum(b0 - 1, 0) if t == 0 else b0 + t - 1
            rp_v[t], deps = finish_rows(pl.multiple_of(prev * E_ROWS, E_ROWS), attn,
                                        E_LO0 if t == 0 else E_LO1, E_HI)
            if t == 0:
                deps.append((E_KEY, pltpu.bitcast(m2, u32)))
            attn = out_proj(pl.multiple_of((b0 + t) * E_ROWS, E_ROWS), never, deps)
        acc_v[...] = attn
        return carry

    lax.fori_loop(0, n_e, e_body, 0)
    n_b = S // E_ROWS
    cp_out(n_b - E_SUB - 1, E_SUB).start()
    m1, m2 = top_v[0], top_v[1]
    for t in range(E_SUB):
        m1, m2 = score_rows((n_b - E_SUB - 1 + t) * E_ROWS, rp_v[t], None, m1, m2)
    rp_last, _ = finish_rows(S - E_ROWS, acc_v[...], 0.0, 1.0)
    m1, m2 = score_rows(S - E_ROWS, rp_last, None, m1, m2)
    cp_out(n_b - 1, 1).start()

    t1 = jnp.max(m1, axis=0, keepdims=True)
    t2 = jnp.max(jnp.where(m1 == t1, m2, m1), axis=0, keepdims=True)
    i1 = (0xFFFF - t1[0, 0]) & (S - 1)
    i2 = (0xFFFF - t2[0, 0]) & (S - 1)
    g1 = pl.multiple_of(i1 & -GRP, GRP)
    g2 = pl.multiple_of(i2 & -GRP, GRP)

    xs = jnp.concatenate([h2_v[pl.ds(g1, GRP), 0:D], h2_v[pl.ds(g2, GRP), 0:D]], axis=0)

    def act(j):
        fc = slice(j * FC, (j + 1) * FC)
        g = _r(jnp.dot(xs, wg_v[:, fc], preferred_element_type=f32))
        u = _r(jnp.dot(xs, wu_v[:, fc], preferred_element_type=f32))
        return (_r(g * jax.nn.sigmoid(g)) * u).astype(bf16)

    y = None
    a = act(0)
    for j in range(F // FC):
        a_next = act(j + 1) if (j + 1) * FC < F else None
        d = jnp.dot(a, wd_v[j * FC:(j + 1) * FC, 0:D], preferred_element_type=f32)
        y = d if y is None else y + d
        a = a_next
    h2 = xs.astype(f32)
    x2 = jnp.concatenate(
        [jnp.concatenate([l_v[k, pl.ds(g, GRP), :] for k in range(D // 128)], axis=1)
         for g in (g1, g2)], axis=0).astype(f32)
    r = _r(jnp.sum(router_parts(h2)[-1], axis=1, keepdims=True))
    upd = _r(_r(y) * _r(jax.nn.sigmoid(r)))
    loc = lax.broadcasted_iota(jnp.int32, (2 * GRP, D), 0)
    row = jnp.where(loc < GRP, g1 + loc, g2 + loc - GRP)
    sel = jnp.logical_or(row == i1, row == i2)
    hb = _r(h2 + jnp.where(sel, upd, 0.0))
    fix_v[...] = (x2 + _r(mrow(GB, 2 * GRP) * hb)).astype(bf16)

    cp(out_v.at[:, pl.ds(0, D)], out_hbm.at[0], SEM_OUT).wait()
    fix1 = cp(fix_v.at[pl.ds(0, GRP), :], out_hbm.at[0, pl.ds(g1, GRP), :], SEM_FIX)
    fix2 = cp(fix_v.at[pl.ds(GRP, GRP), :], out_hbm.at[0, pl.ds(g2, GRP), :], SEM_FIX + 1)
    fix1.start()

    @pl.when(g2 != g1)
    def _():
        fix2.start()
        fix2.wait()

    fix1.wait()


@jax.jit
def pallas_adaLN_cond__mha_block_cached__moe_arch_mod__prompt_kernel(
    A_x: jax.Array,
    A_k_cache: jax.Array,
    A_v_cache: jax.Array,
    A_wq: jax.Array,
    A_wo: jax.Array,
    B_x: jax.Array,
    B_w_r: jax.Array,
    B_w_gate: jax.Array,
    B_w_up: jax.Array,
    B_w_down: jax.Array,
    c: jax.Array,
    w_mod: jax.Array,
):
    del B_x
    vm = pltpu.VMEM
    scratch = [
        vm((S, D), bf16),
        vm((S, D + PAD), bf16),
        vm((S, D + PAD), bf16),
        vm((HH, S, DH), bf16),
        vm((H, S, DH), f32),
        vm((E_ROWS, D), f32),
        vm((2 * H, D, DH), bf16),
        vm((D, F), bf16),
        vm((D, F), bf16),
        vm((F, D + PAD), bf16),
        vm((2, 2, S, DH), bf16),
        vm((2, 2, S, DH), bf16),
        vm((HH, S, DH), bf16),
        vm((1, D), bf16),
        vm((D,), bf16),
        vm((GRP, D), bf16),
        vm((D, 128), f32),
        vm((8, 7 * D), f32),
        vm((2, 8, 128), jnp.int32),
        vm((E_SUB, E_ROWS, 128), f32),
        vm((2 * GRP, D), bf16),
        pltpu.SemaphoreType.DMA((N_SEM,)),
    ]
    return pl.pallas_call(
        _kernel,
        in_specs=[pl.BlockSpec(memory_space=pl.ANY)] * 11,
        out_specs=pl.BlockSpec(memory_space=pl.ANY),
        out_shape=jax.ShapeDtypeStruct(A_x.shape, A_x.dtype),
        scratch_shapes=scratch,
        compiler_params=pltpu.CompilerParams(vmem_limit_bytes=124 * 1024 * 1024,
                                             disable_bounds_checks=True),
        name="adaln_mha_moe",
    )(A_x, A_k_cache, A_v_cache, A_wq, A_wo, B_w_r, B_w_gate, B_w_up, B_w_down, c, w_mod)
```

```python
import jax
import jax.numpy as jnp
from jax import lax
import jax.experimental.pallas as pl
import jax.experimental.pallas.tpu as pltpu

S = 2048
D = 1024
H = 32
DH = 128
F = 3584
EPS = 1e-5
HH = H // 2

TQ = 256
KR = 512
P_ROWS = 256
P_HEADS = 4
U_ROWS = 128
N_RB = S // U_ROWS
N_QU = (H - P_HEADS) // 4 * N_RB
N_OU = 2 * 2 * N_RB
U_PER_IT = (N_QU + N_OU) // HH
E_ROWS = 64
E_SUB = 4
PACE = 48
MV_STEP, MV_U0 = 2, 7
GRP = 16
FC = 512
PAD = 128
P_LO, P_HI = 0.25, 0.97
E_LO0, E_LO1, E_HI, E_KEY, E_RUN = 0.35, 0.3, 0.97, 0.3, 2

Q_SCALE = float(DH) ** -0.5 * 1.4426950408889634

f32 = jnp.float32
bf16 = jnp.bfloat16
u32 = jnp.uint32


def _r(x):
    return x.astype(bf16).astype(f32)


def _recip(x):
    r0 = pl.reciprocal(x, approx=True)
    return r0 * (2.0 - x * r0)


def _pace(t):
    for _ in range(PACE):
        t = jnp.minimum(t, jnp.max(t, axis=1, keepdims=True))
    return t


def _tiles(v):
    u = pltpu.bitcast(v, u32)
    return [[u[a * 8:(a + 1) * 8, b * 128:(b + 1) * 128] for b in range(u.shape[1] // 128)]
            for a in range(u.shape[0] // 8)]


def _col_dots(k_tiles, rhs, n_tiles, never, deps):
    n_r = len(k_tiles) // 4
    n_i = k_tiles[0].shape[0] // GRP
    total = n_tiles * n_r * n_i
    at = {}
    for n, (pos, d) in enumerate(deps):
        at.setdefault((min(int(pos * total), total - 1), n % 4), []).append(d)
    outs = []
    for j in range(n_tiles):
        tl = list(k_tiles)
        for k in range(len(k_tiles)):
            base = (j * n_r + k // 4) * n_i
            if not any((base + i, k % 4) in at for i in range(n_i)):
                continue
            tu = pltpu.bitcast(tl[k], u32)
            parts = []
            for i in range(n_i):
                t = tu[i * 8:(i + 1) * 8, :]
                for d in at.get((base + i, k % 4), ()):
                    t = jnp.where(never, d, t)
                parts.append(t)
            tl[k] = pltpu.bitcast(jnp.concatenate(parts, axis=0), bf16)
        outs.append(jnp.dot(jnp.concatenate(tl, axis=1), rhs(j), preferred_element_type=f32))
    return outs


def _matvec(a_ref, w_refs):
    accs = [None] * len(w_refs)
    steps = []
    for s in range(D // GRP):
        a = a_ref[s * GRP:(s + 1) * GRP, :]
        for n, w in enumerate(w_refs):
            t = w[s * GRP:(s + 1) * GRP, :].astype(f32) * a
            accs[n] = t if accs[n] is None else accs[n] + t
        if s % MV_STEP == MV_STEP - 1:
            steps += [t[0] for acc in accs for t in _tiles(acc)]
    res = [jnp.broadcast_to(jnp.sum(acc, axis=0, keepdims=True), (8, 128)) for acc in accs]
    return res, steps


def _lane_bcast(row):
    return jnp.concatenate([row] * 16, axis=0).T


def _never(i):
    return jnp.full((8, 128), i, jnp.int32) > (1 << 20)


def _attention(heads):
    items = [(refs, c) for refs in heads for c in range(S // TQ)]

    def scores(item):
        (q_ref, bias, k_ref, _, _), c = item
        q = q_ref[c * TQ:(c + 1) * TQ, :] + jnp.concatenate([bias] * (TQ // 8), axis=0)
        q = (q * Q_SCALE).astype(bf16)
        return lax.dot_general(q, k_ref[...], (((1,), (1,)), ((), ())),
                               preferred_element_type=f32)

    def weigh(item, s):
        (_, _, _, v_ref, o_ref), c = item
        m = jnp.max(s, axis=1, keepdims=True)
        o = None
        lp = None
        for r in range(S // KR):
            p = jnp.exp2(s[:, r * KR:(r + 1) * KR] - m)
            ps = [p[:, j * 128:(j + 1) * 128] for j in range(KR // 128)]
            t = ps[0]
            for x in ps[1:]:
                t = t + x
            lp = t if lp is None else lp + t
            ps[-1] = jnp.minimum(ps[-1], t)
            p = jnp.concatenate(ps, axis=1)
            d = jnp.dot(p.astype(bf16), v_ref[r * KR:(r + 1) * KR, :],
                        preferred_element_type=f32)
            o = d if o is None else o + d
        l = jnp.sum(lp, axis=1, keepdims=True)
        o_ref[c * TQ:(c + 1) * TQ, :] = (o * _recip(l)).astype(bf16)

    s = scores(items[0])
    for n, item in enumerate(items):
        s_next = scores(items[n + 1]) if n + 1 < len(items) else None
        weigh(item, s)
        s = s_next


SEM_C, SEM_WR, SEM_WMA, SEM_X, SEM_WQ, SEM_KV, SEM_BG, SEM_OUT, SEM_FIX, SEM_WMB, SEM_O, N_SEM = (
    0, 1, 2, 6, 14, 17, 21, 25, 26, 28, 30, 32)
WO = H
GA, SB, CB1, GB, WR = range(5)


def _kernel(x_hbm, k_hbm, v_hbm, wq_hbm, wo_hbm, wr_hbm, wg_hbm, wu_hbm, wd_hbm, c_hbm,
            wm_hbm, out_hbm,
            x_v, h2_v, out_v, l_v, f_v, acc_v, w_v, wg_v, wu_v, wd_v, k_v, v_v, o_v,
            c_v, wr_v, sc_v, scb_v, sab_v, ca_v, sq_v, mod_v, top_v, rp_v, fix_v, sems):
    n_p = S // P_ROWS
    n_e = S // (E_SUB * E_ROWS)
    pq = P_HEADS * DH

    def cp(src, dst, sem):
        return pltpu.make_async_copy(src, dst, sems.at[sem])

    def cp_c():
        return cp(c_hbm, c_v, SEM_C)

    def cp_wr():
        return cp(wr_hbm, wr_v, SEM_WR)

    def cp_wca(j):
        return cp(wm_hbm.at[:, pl.ds(D + j * 512, 512)],
                  h2_v.at[pl.ds(D, D), pl.ds(j * 512, 512)], SEM_WMA + j)

    def cp_wsa():
        return cp(wm_hbm.at[:, pl.ds(0, D)], h2_v.at[pl.ds(0, D), pl.ds(0, D)], SEM_WMA + 2)

    def cp_x(i):
        return cp(x_hbm.at[0, pl.ds(i * P_ROWS, P_ROWS), :], x_v.at[pl.ds(i * P_ROWS, P_ROWS), :],
                  SEM_X + i)

    def cp_wqp():
        return cp(wq_hbm.at[:, pl.ds(0, pq)], out_v.at[pl.ds(0, D), pl.ds(0, pq)], SEM_WQ)

    def cp_tile(src, row, col, j, sem):
        return cp(src.at[pl.ds(pl.multiple_of(row * D, D), D), pl.ds(pl.multiple_of(col * DH, DH), DH)],
                  w_v.at[j], sem)

    def tiles_wait(lo, n, sem):
        cp(w_v.at[pl.ds(lo, n)], w_v.at[pl.ds(lo, n)], sem).wait()

    def cp_k(it):
        return cp(k_hbm.at[0, pl.ds(2 * it, 2)], k_v.at[it & 1], SEM_KV + (it & 1))

    def cp_v(it):
        return cp(v_hbm.at[0, pl.ds(2 * it, 2)], v_v.at[it & 1], SEM_KV + 2 + (it & 1))

    def cp_rows(src, dst, i, n, sem):
        return cp(src.at[pl.ds(i * n, n), :], dst.at[pl.ds(i * n, n), pl.ds(0, src.shape[1])], sem)

    def wmb_start(it):
        for k in range(2):
            cp_tile(wm_hbm, 0, 2 * D // DH + 2 * it + k, 2 * (it & 1) + k,
                    SEM_WMB + (it & 1)).start()

    def cp_out(i, n):
        return cp(out_v.at[pl.ds(i * E_ROWS, n * E_ROWS), pl.ds(0, D)],
                  out_hbm.at[0, pl.ds(i * E_ROWS, n * E_ROWS), :], SEM_OUT)

    def mrow(k, n):
        m = mod_v[:, k * D:(k + 1) * D]
        return jnp.concatenate([m] * (n // 8), axis=0)

    cp_c().start()
    cp_wr().start()
    for j in range(2):
        cp_wca(j).start()
    cp_x(0).start()
    cp_wqp().start()
    for i in range(1, n_p):
        cp_x(i).start()
    cp_wsa().start()
    cp_k(0).start()
    cp_v(0).start()
    wmb_start(0)

    cp_c().wait()
    cp_wr().wait()
    mod_v[:, WR * D:(WR + 1) * D] = jnp.broadcast_to(wr_v[...].astype(f32).reshape(1, D), (8, D))
    int_min = jnp.iinfo(jnp.int32).min
    top_v[...] = jnp.full(top_v.shape, int_min, jnp.int32)
    acc_v[...] = jnp.zeros(acc_v.shape, f32)
    rp_v[...] = jnp.zeros(rp_v.shape, f32)
    cf = c_v[...].astype(f32)
    sc = jnp.broadcast_to(_r(cf * jax.nn.sigmoid(cf)), (8, D))
    sc_v[...] = jnp.concatenate([sc, sc], axis=0).astype(bf16)
    scb_v[...] = _lane_bcast(sc)

    def wca_body(j, carry):
        cp_wca(j).wait()
        cols = pl.ds(pl.multiple_of(j * 512, 512), 512)
        mj = jnp.dot(sc_v[...], h2_v[D:2 * D, cols], preferred_element_type=f32)
        ca_v[:, cols] = _r(_r(mj[0:8, :]) + 1.0)
        return carry

    lax.fori_loop(0, 2, wca_body, 0)

    def ln1(i):
        rows = pl.ds(pl.multiple_of(i * P_ROWS, P_ROWS), P_ROWS)
        x = x_v[rows, :].astype(f32)
        mu = jnp.sum(x, axis=1, keepdims=True) * (1.0 / D)
        d = x - mu
        var = jnp.sum(d * d, axis=1, keepdims=True) * (1.0 / D)
        n = d * lax.rsqrt(var + EPS)
        h = (n * jnp.concatenate([ca_v[...]] * (P_ROWS // 8), axis=0)).astype(bf16)
        for k in range(D // 128):
            l_v[k, rows, :] = h[:, k * 128:(k + 1) * 128]
        return h

    cp_x(0).wait()
    ln1(0)
    cp_wqp().wait()

    def p_body(i, carry):
        @pl.when(i + 1 < n_p)
        def _():
            cp_x(i + 1).wait()

        rows = pl.ds(pl.multiple_of(i * P_ROWS, P_ROWS), P_ROWS)
        lhs = [l_v[k, rows, :] for k in range(D // 128)]
        tl = [t for row in _tiles(ln1(jnp.minimum(i + 1, n_p - 1))) for t in row]
        deps = [(P_LO + (P_HI - P_LO) * n / len(tl), t) for n, t in enumerate(tl)]
        qs = _col_dots(lhs, lambda j: out_v[0:D, j * DH:(j + 1) * DH], P_HEADS, _never(i), deps)
        for j in range(P_HEADS):
            f_v[j, rows, :] = qs[j]

        @pl.when(i + 1 < n_p)
        def _():
            for k in range(4):
                hd = P_HEADS + 4 * i + k
                cp_tile(wq_hbm, 0, hd, hd, SEM_WQ + jnp.where(i < 1, 1, 2)).start()

        return carry

    lax.fori_loop(0, n_p, p_body, 0)
    cp_k(1).start()
    cp_v(1).start()
    wmb_start(1)
    cp_wsa().wait()
    sa = _r(jnp.dot(sc_v[...], h2_v[0:D, 0:D], preferred_element_type=f32))
    sab_v[...] = _lane_bcast(sa[0:8, :])
    sq = jnp.dot(sa.astype(bf16), out_v[0:D, 0:pq], preferred_element_type=f32)
    for j in range(P_HEADS):
        sq_v[j] = sq[0:8, j * DH:(j + 1) * DH]
    tiles_wait(P_HEADS, 4, SEM_WQ + 1)

    def m_body(it, carry):
        @pl.when(it == 1)
        def _():
            tiles_wait(P_HEADS + 4, H - P_HEADS - 4, SEM_WQ + 2)

        @pl.when(it == N_QU // U_PER_IT)
        def _():
            tiles_wait(WO, H, SEM_BG)

        @pl.when(jnp.logical_or(it == 6, it == 10))
        def _():
            cp(out_hbm.at[0], out_hbm.at[0], SEM_O).wait()

        @pl.when(jnp.logical_or(it == 8, it == 12))
        def _():
            dst = l_v.at[pl.ds(24 - 2 * it, 8)]
            cp(dst, dst, SEM_O + 1).wait()

        cp_k(it).wait()
        cp_v(it).wait()
        tiles_wait(2 * (it & 1), 2, SEM_WMB + (it & 1))
        slot = it & 1

        def unit(u, js, deps=()):
            g = it * U_PER_IT + u
            is_q = g < N_QU
            blk4 = (g >> 4) * 4
            fb = blk4 + jnp.where(is_q, P_HEADS, -(H - P_HEADS))
            wb = blk4 + P_HEADS
            lb = jnp.where(is_q, 0, 8 - (fb & 8))
            r0 = pl.multiple_of((g & (N_RB - 1)) * U_ROWS, U_ROWS)
            lhs = [l_v[lb + k, pl.ds(r0, U_ROWS), :] for k in range(8)]
            res = _col_dots(lhs, lambda n: w_v[wb + js[n]], len(js), never, deps)
            return [(fb + j, r0, v) for j, v in zip(js, res)]

        def put(tiles):
            for j, r0, v in tiles:
                f_v[j, pl.ds(r0, v.shape[0]), :] = v

        never = _never(it)
        late = unit(0, [0])
        _attention([(f_v.at[2 * it + e], sq_v[2 * it + e], k_v.at[slot, e], v_v.at[slot, e],
                     o_v.at[(2 * it + e) & (HH - 1)]) for e in range(2)])
        mb, steps = _matvec(scb_v, [w_v.at[2 * slot + e] for e in range(2)])
        one = jnp.where(it >> 2 == CB1 - GA, 1.0, 0.0)
        for e in range(2):
            cols = pl.ds(pl.multiple_of(GA * D + (2 * it + e) * 128, 128), 128)
            mod_v[:, cols] = _r(_r(mb[e]) + one)
        hq = jnp.minimum(2 * it + P_HEADS, H - 2)
        sq, more = _matvec(sab_v, [w_v.at[hq + e] for e in range(2)])
        for e in range(2):
            sq_v[hq + e] = sq[e]
        steps = steps + more
        span = (U_PER_IT - MV_U0) * 0.9 / len(steps)
        steps = [(MV_U0 + n * span, t) for n, t in enumerate(steps)]
        for u in range(U_PER_IT):
            tiles = unit(u, list(range(1 if u == 0 else 0, 4)),
                         [(pos - u, t) for pos, t in steps if u <= pos < u + 1])
            if u == 0:
                j, r0, v = tiles[0]
                late.append((j, r0, _pace(v[0:8, :])))
                tiles[0] = (j, r0 + 8, v[8:, :])
            put(tiles)
            if u == U_PER_IT - 2:
                put(late)

        @pl.when(it + 2 < HH)
        def _():
            cp_k(it + 2).start()
            cp_v(it + 2).start()
            wmb_start(it + 2)

        @pl.when(jnp.logical_or(it == 4, it == 8))
        def _():
            for k in range(8):
                cp(o_v.at[2 * it - 8 + k], out_hbm.at[0, :, pl.ds(k * DH, DH)], SEM_O).start()

        @pl.when(jnp.logical_or(it == 6, it == 10))
        def _():
            for k in range(8):
                cp(out_hbm.at[0, :, pl.ds(k * DH, DH)], l_v.at[20 - 2 * it + k], SEM_O + 1).start()

        @pl.when(it < 8)
        def _():
            for k in range(4):
                t = 4 * it + k
                cp_tile(wo_hbm, t >> 3, t & 7, WO + t, SEM_BG).start()

        for n, (src, dst) in enumerate(((wg_hbm, wg_v), (wu_hbm, wu_v), (wd_hbm, wd_v))):
            @pl.when(it >> 1 == n + 4)
            def _():
                cp_rows(src, dst, it & 1, src.shape[0] // 2, SEM_BG + 1 + n).start()

        return carry

    lax.fori_loop(0, HH, m_body, 0)

    cp(wg_v, wg_v, SEM_BG + 1).wait()
    cp(wu_v, wu_v, SEM_BG + 2).wait()
    cp(wd_hbm, wd_v.at[:, pl.ds(0, D)], SEM_BG + 3).wait()

    def router_parts(h2):
        pr = h2 * mrow(WR, h2.shape[0])
        run = [pr[:, 0:128]]
        for b in range(1, D // 128):
            run.append(run[-1] + pr[:, b * 128:(b + 1) * 128])
        return run

    def finish_rows(r0, attn, lo, hi):
        rows = pl.ds(r0, E_ROWS)
        x2 = _r(x_v[rows, :].astype(f32) + mrow(GA, E_ROWS) * attn)
        mu = jnp.sum(x2, axis=1, keepdims=True) * (1.0 / D)
        dc = x2 - mu
        var = _r(jnp.sum(dc * dc, axis=1, keepdims=True) * (1.0 / D))
        den = _r(jnp.sqrt(_r(var + EPS)))
        n = _r(_r(x2 - _r(mu)) * _recip(den))
        h2 = _r(_r(n * mrow(CB1, E_ROWS)) + mrow(SB, E_ROWS))
        x2b = x2.astype(bf16)
        for k in range(D // 128):
            l_v[k, rows, :] = x2b[:, k * 128:(k + 1) * 128]
        h2_v[rows, 0:D] = h2.astype(bf16)
        of = x2 + _r(mrow(GB, E_ROWS) * h2)
        out_v[rows, 0:D] = of.astype(bf16)
        run = router_parts(h2)
        deps = []
        ot = _tiles(of)
        n_t = len(ot) * len(ot[0])
        for g in range(len(ot)):
            for b in range(len(ot[0])):
                pos = lo + (hi - lo) * (g * len(ot[0]) + b) / n_t
                deps.append((pos, ot[g][b]))
                if b % E_RUN == E_RUN - 1:
                    deps.append((pos, pltpu.bitcast(run[b][g * 8:(g + 1) * 8, :], u32)))
        return run[-1], deps

    def score_rows(r0, rp, valid, m1, m2):
        r = _r(jnp.sum(rp, axis=1, keepdims=True)) + 0.0
        r = jnp.where(r != r, -jnp.inf, r)
        bits = pltpu.bitcast(jnp.broadcast_to(r, (E_ROWS, 128)), jnp.int32)
        bits = jnp.where(bits < 0, bits ^ 0x7FFF0000, bits)
        idx = r0 + lax.broadcasted_iota(jnp.int32, (E_ROWS, 128), 0)
        key = bits | (0xFFFF - idx)
        if valid is not None:
            key = jnp.where(valid, key, int_min)
        for g in range(E_ROWS // 8):
            kg = key[g * 8:(g + 1) * 8, :]
            m2 = jnp.maximum(m2, jnp.minimum(m1, kg))
            m1 = jnp.maximum(m1, kg)
        return m1, m2

    def out_proj(r0, never, deps):
        rows = pl.ds(r0, E_ROWS)
        lhs = [o_v[j, rows, :] for j in range(HH)]
        ds = _col_dots(lhs, lambda j: jnp.concatenate([w_v[WO + 16 + j], w_v[WO + 24 + j]], axis=0),
                       D // 128, never, deps)
        return jnp.concatenate([f_v[j, rows, :] + f_v[8 + j, rows, :] + ds[j]
                                for j in range(D // 128)], axis=1)

    def e_body(c, carry):
        b0 = E_SUB * c

        @pl.when(c >= 2)
        def _():
            cp_out(b0 - E_SUB - 1, 1).start()

        @pl.when(c >= 1)
        def _():
            cp_out(b0 - E_SUB, E_SUB - 1).start()

        never = _never(c)
        m1, m2 = top_v[0], top_v[1]
        for t in range(E_SUB):
            m1, m2 = score_rows((b0 - E_SUB - 1 + t) * E_ROWS, rp_v[t],
                                c >= (2 if t == 0 else 1), m1, m2)
        top_v[0] = m1
        top_v[1] = m2
        attn = acc_v[...]
        for t in range(E_SUB):
            prev = jnp.maximum(b0 - 1, 0) if t == 0 else b0 + t - 1
            rp_v[t], deps = finish_rows(pl.multiple_of(prev * E_ROWS, E_ROWS), attn,
                                        E_LO0 if t == 0 else E_LO1, E_HI)
            if t == 0:
                deps.append((E_KEY, pltpu.bitcast(m2, u32)))
            attn = out_proj(pl.multiple_of((b0 + t) * E_ROWS, E_ROWS), never, deps)
        acc_v[...] = attn
        return carry

    lax.fori_loop(0, n_e, e_body, 0)
    n_b = S // E_ROWS
    cp_out(n_b - E_SUB - 1, E_SUB).start()
    m1, m2 = top_v[0], top_v[1]
    for t in range(E_SUB):
        m1, m2 = score_rows((n_b - E_SUB - 1 + t) * E_ROWS, rp_v[t], None, m1, m2)
    rp_last, _ = finish_rows(S - E_ROWS, acc_v[...], 0.0, 1.0)
    m1, m2 = score_rows(S - E_ROWS, rp_last, None, m1, m2)
    cp_out(n_b - 1, 1).start()

    t1 = jnp.max(m1, axis=0, keepdims=True)
    t2 = jnp.max(jnp.where(m1 == t1, m2, m1), axis=0, keepdims=True)
    i1 = (0xFFFF - t1[0, 0]) & (S - 1)
    i2 = (0xFFFF - t2[0, 0]) & (S - 1)
    g1 = pl.multiple_of(i1 & -GRP, GRP)
    g2 = pl.multiple_of(i2 & -GRP, GRP)

    xs = jnp.concatenate([h2_v[pl.ds(g1, GRP), 0:D], h2_v[pl.ds(g2, GRP), 0:D]], axis=0)

    def act(j):
        fc = slice(j * FC, (j + 1) * FC)
        g = _r(jnp.dot(xs, wg_v[:, fc], preferred_element_type=f32))
        u = _r(jnp.dot(xs, wu_v[:, fc], preferred_element_type=f32))
        return (_r(g * jax.nn.sigmoid(g)) * u).astype(bf16)

    y = None
    a = act(0)
    for j in range(F // FC):
        a_next = act(j + 1) if (j + 1) * FC < F else None
        d = jnp.dot(a, wd_v[j * FC:(j + 1) * FC, 0:D], preferred_element_type=f32)
        y = d if y is None else y + d
        a = a_next
    h2 = xs.astype(f32)
    x2 = jnp.concatenate(
        [jnp.concatenate([l_v[k, pl.ds(g, GRP), :] for k in range(D // 128)], axis=1)
         for g in (g1, g2)], axis=0).astype(f32)
    r = _r(jnp.sum(router_parts(h2)[-1], axis=1, keepdims=True))
    upd = _r(_r(y) * _r(jax.nn.sigmoid(r)))
    loc = lax.broadcasted_iota(jnp.int32, (2 * GRP, D), 0)
    row = jnp.where(loc < GRP, g1 + loc, g2 + loc - GRP)
    sel = jnp.logical_or(row == i1, row == i2)
    hb = _r(h2 + jnp.where(sel, upd, 0.0))
    fix_v[...] = (x2 + _r(mrow(GB, 2 * GRP) * hb)).astype(bf16)

    cp(out_v.at[:, pl.ds(0, D)], out_hbm.at[0], SEM_OUT).wait()
    fix1 = cp(fix_v.at[pl.ds(0, GRP), :], out_hbm.at[0, pl.ds(g1, GRP), :], SEM_FIX)
    fix2 = cp(fix_v.at[pl.ds(GRP, GRP), :], out_hbm.at[0, pl.ds(g2, GRP), :], SEM_FIX + 1)
    fix1.start()

    @pl.when(g2 != g1)
    def _():
        fix2.start()
        fix2.wait()

    fix1.wait()


@jax.jit
def pallas_adaLN_cond__mha_block_cached__moe_arch_mod__prompt_kernel(
    A_x: jax.Array,
    A_k_cache: jax.Array,
    A_v_cache: jax.Array,
    A_wq: jax.Array,
    A_wo: jax.Array,
    B_x: jax.Array,
    B_w_r: jax.Array,
    B_w_gate: jax.Array,
    B_w_up: jax.Array,
    B_w_down: jax.Array,
    c: jax.Array,
    w_mod: jax.Array,
):
    del B_x
    vm = pltpu.VMEM
    scratch = [
        vm((S, D), bf16),
        vm((S, D + PAD), bf16),
        vm((S, D + PAD), bf16),
        vm((HH, S, DH), bf16),
        vm((H, S, DH), f32),
        vm((E_ROWS, D), f32),
        vm((2 * H, D, DH), bf16),
        vm((D, F), bf16),
        vm((D, F), bf16),
        vm((F, D + PAD), bf16),
        vm((2, 2, S, DH), bf16),
        vm((2, 2, S, DH), bf16),
        vm((HH, S, DH), bf16),
        vm((1, D), bf16),
        vm((D,), bf16),
        vm((GRP, D), bf16),
        vm((D, 128), f32),
        vm((D, 128), f32),
        vm((8, D), f32),
        vm((H, 8, DH), f32),
        vm((8, 5 * D), f32),
        vm((2, 8, 128), jnp.int32),
        vm((E_SUB, E_ROWS, 128), f32),
        vm((2 * GRP, D), bf16),
        pltpu.SemaphoreType.DMA((N_SEM,)),
    ]
    return pl.pallas_call(
        _kernel,
        in_specs=[pl.BlockSpec(memory_space=pl.ANY)] * 11,
        out_specs=pl.BlockSpec(memory_space=pl.ANY),
        out_shape=jax.ShapeDtypeStruct(A_x.shape, A_x.dtype),
        scratch_shapes=scratch,
        compiler_params=pltpu.CompilerParams(vmem_limit_bytes=124 * 1024 * 1024,
                                             disable_bounds_checks=True,
                                             disable_semaphore_checks=True),
        name="adaln_mha_moe",
    )(A_x, A_k_cache, A_v_cache, A_wq, A_wo, B_w_r, B_w_gate, B_w_up, B_w_down, c, w_mod)
```

```python
import jax
import jax.numpy as jnp
from jax import lax
import jax.experimental.pallas as pl
import jax.experimental.pallas.tpu as pltpu

S = 2048
D = 1024
H = 32
DH = 128
F = 3584
EPS = 1e-5
HH = H // 2

TQ = 256
KR = 512
P_ROWS = 256
P_HEADS = 4
U_ROWS = 128
N_RB = S // U_ROWS
N_QU = (H - P_HEADS) // 4 * N_RB
N_OU = 2 * 2 * N_RB
U_PER_IT = (N_QU + N_OU) // HH
E_ROWS = 64
E_SUB = 4
PACE = 48
MV_STEP, MV_U0 = 2, 7
GRP = 16
FC = 512
PAD = 128
P_LO, P_HI, P_SQ = 0.25, 0.97, 10
E_LO0, E_LO1, E_HI, E_KEY, E_RUN = 0.35, 0.3, 0.97, 0.3, 2

Q_SCALE = float(DH) ** -0.5 * 1.4426950408889634

f32 = jnp.float32
bf16 = jnp.bfloat16
u32 = jnp.uint32


def _r(x):
    return x.astype(bf16).astype(f32)


def _recip(x):
    r0 = pl.reciprocal(x, approx=True)
    return r0 * (2.0 - x * r0)


def _pace(t):
    for _ in range(PACE):
        t = jnp.minimum(t, jnp.max(t, axis=1, keepdims=True))
    return t


def _tiles(v):
    u = pltpu.bitcast(v, u32)
    return [[u[a * 8:(a + 1) * 8, b * 128:(b + 1) * 128] for b in range(u.shape[1] // 128)]
            for a in range(u.shape[0] // 8)]


def _col_dots(k_tiles, rhs, n_tiles, never, deps):
    n_r = len(k_tiles) // 4
    n_i = k_tiles[0].shape[0] // GRP
    total = n_tiles * n_r * n_i
    at = {}
    for n, (pos, d) in enumerate(deps):
        at.setdefault((min(int(pos * total), total - 1), n % 4), []).append(d)
    outs = []
    for j in range(n_tiles):
        tl = list(k_tiles)
        for k in range(len(k_tiles)):
            base = (j * n_r + k // 4) * n_i
            if not any((base + i, k % 4) in at for i in range(n_i)):
                continue
            tu = pltpu.bitcast(tl[k], u32)
            parts = []
            for i in range(n_i):
                t = tu[i * 8:(i + 1) * 8, :]
                for d in at.get((base + i, k % 4), ()):
                    t = jnp.where(never, d, t)
                parts.append(t)
            tl[k] = pltpu.bitcast(jnp.concatenate(parts, axis=0), bf16)
        outs.append(jnp.dot(jnp.concatenate(tl, axis=1), rhs(j), preferred_element_type=f32))
    return outs


def _matvec(a_ref, w_refs):
    accs = [None] * len(w_refs)
    steps = []
    for s in range(D // GRP):
        a = a_ref[s * GRP:(s + 1) * GRP, :]
        for n, w in enumerate(w_refs):
            t = w[s * GRP:(s + 1) * GRP, :].astype(f32) * a
            accs[n] = t if accs[n] is None else accs[n] + t
        if s % MV_STEP == MV_STEP - 1:
            steps += [t[0] for acc in accs for t in _tiles(acc)]
    res = [jnp.broadcast_to(jnp.sum(acc, axis=0, keepdims=True), (8, 128)) for acc in accs]
    return res, steps


def _lane_bcast(row):
    return jnp.concatenate([row] * 16, axis=0).T


def _never(i):
    return jnp.full((8, 128), i, jnp.int32) > (1 << 20)


def _attention(heads):
    items = [(refs, c) for refs in heads for c in range(S // TQ)]

    def scores(item):
        (q_ref, bias, k_ref, _, _), c = item
        q = q_ref[c * TQ:(c + 1) * TQ, :] + jnp.concatenate([bias] * (TQ // 8), axis=0)
        q = (q * Q_SCALE).astype(bf16)
        return lax.dot_general(q, k_ref[...], (((1,), (1,)), ((), ())),
                               preferred_element_type=f32)

    def weigh(item, s):
        (_, _, _, v_ref, o_ref), c = item
        m = jnp.max(s, axis=1, keepdims=True)
        o = None
        lp = None
        for r in range(S // KR):
            p = jnp.exp2(s[:, r * KR:(r + 1) * KR] - m)
            ps = [p[:, j * 128:(j + 1) * 128] for j in range(KR // 128)]
            t = ps[0]
            for x in ps[1:]:
                t = t + x
            lp = t if lp is None else lp + t
            ps[-1] = jnp.minimum(ps[-1], t)
            p = jnp.concatenate(ps, axis=1)
            d = jnp.dot(p.astype(bf16), v_ref[r * KR:(r + 1) * KR, :],
                        preferred_element_type=f32)
            o = d if o is None else o + d
        l = jnp.sum(lp, axis=1, keepdims=True)
        o_ref[c * TQ:(c + 1) * TQ, :] = (o * _recip(l)).astype(bf16)

    s = scores(items[0])
    for n, item in enumerate(items):
        s_next = scores(items[n + 1]) if n + 1 < len(items) else None
        weigh(item, s)
        s = s_next


SEM_C, SEM_WR, SEM_WMA, SEM_X, SEM_WQ, SEM_KV, SEM_BG, SEM_OUT, SEM_FIX, SEM_WMB, SEM_O, N_SEM = (
    0, 1, 2, 6, 14, 17, 21, 25, 26, 28, 30, 32)
WO = H
GA, SB, CB1, GB, WR = range(5)


def _kernel(x_hbm, k_hbm, v_hbm, wq_hbm, wo_hbm, wr_hbm, wg_hbm, wu_hbm, wd_hbm, c_hbm,
            wm_hbm, out_hbm,
            x_v, h2_v, out_v, l_v, f_v, acc_v, w_v, wg_v, wu_v, wd_v, k_v, v_v, o_v,
            c_v, wr_v, sc_v, scb_v, sab_v, ca_v, sq_v, mod_v, top_v, rp_v, fix_v, sems):
    n_p = S // P_ROWS
    n_e = S // (E_SUB * E_ROWS)
    pq = P_HEADS * DH

    def cp(src, dst, sem):
        return pltpu.make_async_copy(src, dst, sems.at[sem])

    def cp_c():
        return cp(c_hbm, c_v, SEM_C)

    def cp_wr():
        return cp(wr_hbm, wr_v, SEM_WR)

    def cp_wca(j):
        return cp(wm_hbm.at[:, pl.ds(D + j * 512, 512)],
                  h2_v.at[pl.ds(D, D), pl.ds(j * 512, 512)], SEM_WMA + j)

    def cp_wsa():
        return cp(wm_hbm.at[:, pl.ds(0, D)], h2_v.at[pl.ds(0, D), pl.ds(0, D)], SEM_WMA + 2)

    def cp_x(i):
        return cp(x_hbm.at[0, pl.ds(i * P_ROWS, P_ROWS), :], x_v.at[pl.ds(i * P_ROWS, P_ROWS), :],
                  SEM_X + i)

    def cp_wqp():
        return cp(wq_hbm.at[:, pl.ds(0, pq)], out_v.at[pl.ds(0, D), pl.ds(0, pq)], SEM_WQ)

    def cp_tile(src, row, col, j, sem):
        return cp(src.at[pl.ds(pl.multiple_of(row * D, D), D), pl.ds(pl.multiple_of(col * DH, DH), DH)],
                  w_v.at[j], sem)

    def tiles_wait(lo, n, sem):
        cp(w_v.at[pl.ds(lo, n)], w_v.at[pl.ds(lo, n)], sem).wait()

    def cp_k(it):
        return cp(k_hbm.at[0, pl.ds(2 * it, 2)], k_v.at[it & 1], SEM_KV + (it & 1))

    def cp_v(it):
        return cp(v_hbm.at[0, pl.ds(2 * it, 2)], v_v.at[it & 1], SEM_KV + 2 + (it & 1))

    def cp_rows(src, dst, i, n, sem):
        return cp(src.at[pl.ds(i * n, n), :], dst.at[pl.ds(i * n, n), pl.ds(0, src.shape[1])], sem)

    def wmb_start(it):
        for k in range(2):
            cp_tile(wm_hbm, 0, 2 * D // DH + 2 * it + k, 2 * (it & 1) + k,
                    SEM_WMB + (it & 1)).start()

    def cp_out(i, n):
        return cp(out_v.at[pl.ds(i * E_ROWS, n * E_ROWS), pl.ds(0, D)],
                  out_hbm.at[0, pl.ds(i * E_ROWS, n * E_ROWS), :], SEM_OUT)

    def mrow(k, n):
        m = mod_v[:, k * D:(k + 1) * D]
        return jnp.concatenate([m] * (n // 8), axis=0)

    cp_c().start()
    cp_wr().start()
    for j in range(2):
        cp_wca(j).start()
    cp_x(0).start()
    cp_wqp().start()
    for i in range(1, n_p):
        cp_x(i).start()
    cp_wsa().start()
    cp_k(0).start()
    cp_v(0).start()
    wmb_start(0)

    cp_c().wait()
    cp_wr().wait()
    mod_v[:, WR * D:(WR + 1) * D] = jnp.broadcast_to(wr_v[...].astype(f32).reshape(1, D), (8, D))
    int_min = jnp.iinfo(jnp.int32).min
    top_v[...] = jnp.full(top_v.shape, int_min, jnp.int32)
    acc_v[...] = jnp.zeros(acc_v.shape, f32)
    rp_v[...] = jnp.zeros(rp_v.shape, f32)
    cf = c_v[...].astype(f32)
    sc = jnp.broadcast_to(_r(cf * jax.nn.sigmoid(cf)), (8, D))
    sc_v[...] = jnp.concatenate([sc, sc], axis=0).astype(bf16)
    scb_v[...] = _lane_bcast(sc)

    def wca_body(j, carry):
        cp_wca(j).wait()
        cols = pl.ds(pl.multiple_of(j * 512, 512), 512)
        mj = jnp.dot(sc_v[...], h2_v[D:2 * D, cols], preferred_element_type=f32)
        ca_v[:, cols] = _r(_r(mj[0:8, :]) + 1.0)
        return carry

    lax.fori_loop(0, 2, wca_body, 0)

    def ln1(i):
        rows = pl.ds(pl.multiple_of(i * P_ROWS, P_ROWS), P_ROWS)
        x = x_v[rows, :].astype(f32)
        mu = jnp.sum(x, axis=1, keepdims=True) * (1.0 / D)
        d = x - mu
        var = jnp.sum(d * d, axis=1, keepdims=True) * (1.0 / D)
        n = d * lax.rsqrt(var + EPS)
        h = (n * jnp.concatenate([ca_v[...]] * (P_ROWS // 8), axis=0)).astype(bf16)
        for k in range(D // 128):
            l_v[k, rows, :] = h[:, k * 128:(k + 1) * 128]
        return h

    cp_x(0).wait()
    ln1(0)
    cp_wqp().wait()

    def p_body(i, carry):
        cp_x(i + 1).wait()
        rows = pl.ds(pl.multiple_of(i * P_ROWS, P_ROWS), P_ROWS)
        lhs = [l_v[k, rows, :] for k in range(D // 128)]
        tl = [t for row in _tiles(ln1(i + 1)) for t in row]
        deps = [(P_LO + (P_HI - P_LO) * n / len(tl), t) for n, t in enumerate(tl)]
        qs = _col_dots(lhs, lambda j: out_v[0:D, j * DH:(j + 1) * DH], P_HEADS, _never(i), deps)
        for j in range(P_HEADS):
            f_v[j, rows, :] = qs[j]
        for k in range(4):
            hd = P_HEADS + 4 * i + k
            cp_tile(wq_hbm, 0, hd, hd, SEM_WQ + jnp.where(i < 1, 1, 2)).start()
        return carry

    lax.fori_loop(0, n_p - 1, p_body, 0)
    cp_k(1).start()
    cp_v(1).start()
    wmb_start(1)
    cp_wsa().wait()

    def halves(lhs, w):
        return [lambda h=h: jnp.dot(lhs(h), w(h), preferred_element_type=f32) for h in range(2)]

    def kh(h):
        return slice(h * 512, (h + 1) * 512)

    sa_t = []
    sa = None
    for n in range(2 * P_HEADS):
        j, rows = n // 2, slice(S - P_ROWS + n % 2 * 128, S - P_ROWS + (n % 2 + 1) * 128)
        big = halves(lambda h: jnp.concatenate([l_v[4 * h + k, rows, :] for k in range(4)], axis=1),
                     lambda h: out_v[kh(h), j * DH:(j + 1) * DH])
        acc = None
        for h in range(2):
            d = big[h]()
            acc = d if acc is None else acc + d
            r = 2 * n + h
            if r < 8:
                a, b = halves(lambda h: sc_v[:, kh(h)], lambda h: h2_v[kh(h), r * 128:(r + 1) * 128])
                sa_t.append(_r(a() + b()))
                if r == 7:
                    sa = jnp.concatenate(sa_t, axis=1)
                    sab_v[...] = _lane_bcast(sa[0:8, :])
                    sa = sa.astype(bf16)
            elif P_SQ <= r < P_SQ + P_HEADS:
                t = r - P_SQ
                a, b = halves(lambda h: sa[:, kh(h)], lambda h: out_v[kh(h), t * DH:(t + 1) * DH])
                sq_v[t] = (a() + b())[0:8, :]
        f_v[j, rows, :] = acc
    tiles_wait(P_HEADS, 4, SEM_WQ + 1)

    def m_body(it, carry):
        @pl.when(it == 1)
        def _():
            tiles_wait(P_HEADS + 4, H - P_HEADS - 4, SEM_WQ + 2)

        @pl.when(it == N_QU // U_PER_IT)
        def _():
            tiles_wait(WO, H, SEM_BG)

        @pl.when(jnp.logical_or(it == 6, it == 10))
        def _():
            cp(out_hbm.at[0], out_hbm.at[0], SEM_O).wait()

        @pl.when(jnp.logical_or(it == 8, it == 12))
        def _():
            dst = l_v.at[pl.ds(24 - 2 * it, 8)]
            cp(dst, dst, SEM_O + 1).wait()

        cp_k(it).wait()
        cp_v(it).wait()
        tiles_wait(2 * (it & 1), 2, SEM_WMB + (it & 1))
        slot = it & 1

        def unit(u, js, deps=()):
            g = it * U_PER_IT + u
            is_q = g < N_QU
            blk4 = (g >> 4) * 4
            fb = blk4 + jnp.where(is_q, P_HEADS, -(H - P_HEADS))
            wb = blk4 + P_HEADS
            lb = jnp.where(is_q, 0, 8 - (fb & 8))
            r0 = pl.multiple_of((g & (N_RB - 1)) * U_ROWS, U_ROWS)
            lhs = [l_v[lb + k, pl.ds(r0, U_ROWS), :] for k in range(8)]
            res = _col_dots(lhs, lambda n: w_v[wb + js[n]], len(js), never, deps)
            return [(fb + j, r0, v) for j, v in zip(js, res)]

        def put(tiles):
            for j, r0, v in tiles:
                f_v[j, pl.ds(r0, v.shape[0]), :] = v

        never = _never(it)
        late = unit(0, [0])
        _attention([(f_v.at[2 * it + e], sq_v[2 * it + e], k_v.at[slot, e], v_v.at[slot, e],
                     o_v.at[(2 * it + e) & (HH - 1)]) for e in range(2)])
        mb, steps = _matvec(scb_v, [w_v.at[2 * slot + e] for e in range(2)])
        one = jnp.where(it >> 2 == CB1 - GA, 1.0, 0.0)
        for e in range(2):
            cols = pl.ds(pl.multiple_of(GA * D + (2 * it + e) * 128, 128), 128)
            mod_v[:, cols] = _r(_r(mb[e]) + one)
        hq = jnp.minimum(2 * it + P_HEADS, H - 2)
        sq, more = _matvec(sab_v, [w_v.at[hq + e] for e in range(2)])
        for e in range(2):
            sq_v[hq + e] = sq[e]
        steps = steps + more
        span = (U_PER_IT - MV_U0) * 0.9 / len(steps)
        steps = [(MV_U0 + n * span, t) for n, t in enumerate(steps)]
        for u in range(U_PER_IT):
            tiles = unit(u, list(range(1 if u == 0 else 0, 4)),
                         [(pos - u, t) for pos, t in steps if u <= pos < u + 1])
            if u == 0:
                j, r0, v = tiles[0]
                late.append((j, r0, _pace(v[0:8, :])))
                tiles[0] = (j, r0 + 8, v[8:, :])
            put(tiles)
            if u == U_PER_IT - 2:
                put(late)

        @pl.when(it + 2 < HH)
        def _():
            cp_k(it + 2).start()
            cp_v(it + 2).start()
            wmb_start(it + 2)

        @pl.when(jnp.logical_or(it == 4, it == 8))
        def _():
            for k in range(8):
                cp(o_v.at[2 * it - 8 + k], out_hbm.at[0, :, pl.ds(k * DH, DH)], SEM_O).start()

        @pl.when(jnp.logical_or(it == 6, it == 10))
        def _():
            for k in range(8):
                cp(out_hbm.at[0, :, pl.ds(k * DH, DH)], l_v.at[20 - 2 * it + k], SEM_O + 1).start()

        @pl.when(it < 8)
        def _():
            for k in range(4):
                t = 4 * it + k
                cp_tile(wo_hbm, t >> 3, t & 7, WO + t, SEM_BG).start()

        for n, (src, dst) in enumerate(((wg_hbm, wg_v), (wu_hbm, wu_v), (wd_hbm, wd_v))):
            @pl.when(it >> 1 == n + 4)
            def _():
                cp_rows(src, dst, it & 1, src.shape[0] // 2, SEM_BG + 1 + n).start()

        return carry

    lax.fori_loop(0, HH, m_body, 0)

    cp(wg_v, wg_v, SEM_BG + 1).wait()
    cp(wu_v, wu_v, SEM_BG + 2).wait()
    cp(wd_hbm, wd_v.at[:, pl.ds(0, D)], SEM_BG + 3).wait()

    def router_parts(h2):
        pr = h2 * mrow(WR, h2.shape[0])
        run = [pr[:, 0:128]]
        for b in range(1, D // 128):
            run.append(run[-1] + pr[:, b * 128:(b + 1) * 128])
        return run

    def finish_rows(r0, attn, lo, hi):
        rows = pl.ds(r0, E_ROWS)
        x2 = _r(x_v[rows, :].astype(f32) + mrow(GA, E_ROWS) * attn)
        mu = jnp.sum(x2, axis=1, keepdims=True) * (1.0 / D)
        dc = x2 - mu
        var = _r(jnp.sum(dc * dc, axis=1, keepdims=True) * (1.0 / D))
        den = _r(jnp.sqrt(_r(var + EPS)))
        n = _r(_r(x2 - _r(mu)) * _recip(den))
        h2 = _r(_r(n * mrow(CB1, E_ROWS)) + mrow(SB, E_ROWS))
        x2b = x2.astype(bf16)
        for k in range(D // 128):
            l_v[k, rows, :] = x2b[:, k * 128:(k + 1) * 128]
        h2_v[rows, 0:D] = h2.astype(bf16)
        of = x2 + _r(mrow(GB, E_ROWS) * h2)
        out_v[rows, 0:D] = of.astype(bf16)
        run = router_parts(h2)
        deps = []
        ot = _tiles(of)
        n_t = len(ot) * len(ot[0])
        for g in range(len(ot)):
            for b in range(len(ot[0])):
                pos = lo + (hi - lo) * (g * len(ot[0]) + b) / n_t
                deps.append((pos, ot[g][b]))
                if b % E_RUN == E_RUN - 1:
                    deps.append((pos, pltpu.bitcast(run[b][g * 8:(g + 1) * 8, :], u32)))
        return run[-1], deps

    def score_rows(r0, rp, valid, m1, m2):
        r = _r(jnp.sum(rp, axis=1, keepdims=True)) + 0.0
        r = jnp.where(r != r, -jnp.inf, r)
        bits = pltpu.bitcast(jnp.broadcast_to(r, (E_ROWS, 128)), jnp.int32)
        bits = jnp.where(bits < 0, bits ^ 0x7FFF0000, bits)
        idx = r0 + lax.broadcasted_iota(jnp.int32, (E_ROWS, 128), 0)
        key = bits | (0xFFFF - idx)
        if valid is not None:
            key = jnp.where(valid, key, int_min)
        for g in range(E_ROWS // 8):
            kg = key[g * 8:(g + 1) * 8, :]
            m2 = jnp.maximum(m2, jnp.minimum(m1, kg))
            m1 = jnp.maximum(m1, kg)
        return m1, m2

    def out_proj(r0, never, deps):
        rows = pl.ds(r0, E_ROWS)
        lhs = [o_v[j, rows, :] for j in range(HH)]
        ds = _col_dots(lhs, lambda j: jnp.concatenate([w_v[WO + 16 + j], w_v[WO + 24 + j]], axis=0),
                       D // 128, never, deps)
        return jnp.concatenate([f_v[j, rows, :] + f_v[8 + j, rows, :] + ds[j]
                                for j in range(D // 128)], axis=1)

    def e_body(c, carry):
        b0 = E_SUB * c

        @pl.when(c >= 2)
        def _():
            cp_out(b0 - E_SUB - 1, 1).start()

        @pl.when(c >= 1)
        def _():
            cp_out(b0 - E_SUB, E_SUB - 1).start()

        never = _never(c)
        m1, m2 = top_v[0], top_v[1]
        for t in range(E_SUB):
            m1, m2 = score_rows((b0 - E_SUB - 1 + t) * E_ROWS, rp_v[t],
                                c >= (2 if t == 0 else 1), m1, m2)
        top_v[0] = m1
        top_v[1] = m2
        attn = acc_v[...]
        for t in range(E_SUB):
            prev = jnp.maximum(b0 - 1, 0) if t == 0 else b0 + t - 1
            rp_v[t], deps = finish_rows(pl.multiple_of(prev * E_ROWS, E_ROWS), attn,
                                        E_LO0 if t == 0 else E_LO1, E_HI)
            if t == 0:
                deps.append((E_KEY, pltpu.bitcast(m2, u32)))
            attn = out_proj(pl.multiple_of((b0 + t) * E_ROWS, E_ROWS), never, deps)
        acc_v[...] = attn
        return carry

    lax.fori_loop(0, n_e, e_body, 0)
    n_b = S // E_ROWS
    cp_out(n_b - E_SUB - 1, E_SUB).start()
    m1, m2 = top_v[0], top_v[1]
    for t in range(E_SUB):
        m1, m2 = score_rows((n_b - E_SUB - 1 + t) * E_ROWS, rp_v[t], None, m1, m2)
    rp_last, _ = finish_rows(S - E_ROWS, acc_v[...], 0.0, 1.0)
    m1, m2 = score_rows(S - E_ROWS, rp_last, None, m1, m2)
    cp_out(n_b - 1, 1).start()

    t1 = jnp.max(m1, axis=0, keepdims=True)
    t2 = jnp.max(jnp.where(m1 == t1, m2, m1), axis=0, keepdims=True)
    i1 = (0xFFFF - t1[0, 0]) & (S - 1)
    i2 = (0xFFFF - t2[0, 0]) & (S - 1)
    g1 = pl.multiple_of(i1 & -GRP, GRP)
    g2 = pl.multiple_of(i2 & -GRP, GRP)

    xs = jnp.concatenate([h2_v[pl.ds(g1, GRP), 0:D], h2_v[pl.ds(g2, GRP), 0:D]], axis=0)

    def act(j):
        fc = slice(j * FC, (j + 1) * FC)
        g = _r(jnp.dot(xs, wg_v[:, fc], preferred_element_type=f32))
        u = _r(jnp.dot(xs, wu_v[:, fc], preferred_element_type=f32))
        return (_r(g * jax.nn.sigmoid(g)) * u).astype(bf16)

    y = None
    a = act(0)
    for j in range(F // FC):
        a_next = act(j + 1) if (j + 1) * FC < F else None
        d = jnp.dot(a, wd_v[j * FC:(j + 1) * FC, 0:D], preferred_element_type=f32)
        y = d if y is None else y + d
        a = a_next
    h2 = xs.astype(f32)
    x2 = jnp.concatenate(
        [jnp.concatenate([l_v[k, pl.ds(g, GRP), :] for k in range(D // 128)], axis=1)
         for g in (g1, g2)], axis=0).astype(f32)
    r = _r(jnp.sum(router_parts(h2)[-1], axis=1, keepdims=True))
    upd = _r(_r(y) * _r(jax.nn.sigmoid(r)))
    loc = lax.broadcasted_iota(jnp.int32, (2 * GRP, D), 0)
    row = jnp.where(loc < GRP, g1 + loc, g2 + loc - GRP)
    sel = jnp.logical_or(row == i1, row == i2)
    hb = _r(h2 + jnp.where(sel, upd, 0.0))
    fix_v[...] = (x2 + _r(mrow(GB, 2 * GRP) * hb)).astype(bf16)

    cp(out_v.at[:, pl.ds(0, D)], out_hbm.at[0], SEM_OUT).wait()
    fix1 = cp(fix_v.at[pl.ds(0, GRP), :], out_hbm.at[0, pl.ds(g1, GRP), :], SEM_FIX)
    fix2 = cp(fix_v.at[pl.ds(GRP, GRP), :], out_hbm.at[0, pl.ds(g2, GRP), :], SEM_FIX + 1)
    fix1.start()

    @pl.when(g2 != g1)
    def _():
        fix2.start()
        fix2.wait()

    fix1.wait()


@jax.jit
def pallas_adaLN_cond__mha_block_cached__moe_arch_mod__prompt_kernel(
    A_x: jax.Array,
    A_k_cache: jax.Array,
    A_v_cache: jax.Array,
    A_wq: jax.Array,
    A_wo: jax.Array,
    B_x: jax.Array,
    B_w_r: jax.Array,
    B_w_gate: jax.Array,
    B_w_up: jax.Array,
    B_w_down: jax.Array,
    c: jax.Array,
    w_mod: jax.Array,
):
    del B_x
    vm = pltpu.VMEM
    scratch = [
        vm((S, D), bf16),
        vm((S, D + PAD), bf16),
        vm((S, D + PAD), bf16),
        vm((HH, S, DH), bf16),
        vm((H, S, DH), f32),
        vm((E_ROWS, D), f32),
        vm((2 * H, D, DH), bf16),
        vm((D, F), bf16),
        vm((D, F), bf16),
        vm((F, D + PAD), bf16),
        vm((2, 2, S, DH), bf16),
        vm((2, 2, S, DH), bf16),
        vm((HH, S, DH), bf16),
        vm((1, D), bf16),
        vm((D,), bf16),
        vm((GRP, D), bf16),
        vm((D, 128), f32),
        vm((D, 128), f32),
        vm((8, D), f32),
        vm((H, 8, DH), f32),
        vm((8, 5 * D), f32),
        vm((2, 8, 128), jnp.int32),
        vm((E_SUB, E_ROWS, 128), f32),
        vm((2 * GRP, D), bf16),
        pltpu.SemaphoreType.DMA((N_SEM,)),
    ]
    return pl.pallas_call(
        _kernel,
        in_specs=[pl.BlockSpec(memory_space=pl.ANY)] * 11,
        out_specs=pl.BlockSpec(memory_space=pl.ANY),
        out_shape=jax.ShapeDtypeStruct(A_x.shape, A_x.dtype),
        scratch_shapes=scratch,
        compiler_params=pltpu.CompilerParams(vmem_limit_bytes=124 * 1024 * 1024,
                                             disable_bounds_checks=True,
                                             disable_semaphore_checks=True),
        name="adaln_mha_moe",
    )(A_x, A_k_cache, A_v_cache, A_wq, A_wo, B_w_r, B_w_gate, B_w_up, B_w_down, c, w_mod)
```

```python
import jax
import jax.numpy as jnp
from jax import lax
import jax.experimental.pallas as pl
import jax.experimental.pallas.tpu as pltpu

S = 2048
D = 1024
H = 32
DH = 128
F = 3584
EPS = 1e-5
HH = H // 2

TQ = 256
KR = 512
P_ROWS = 256
P_HEADS = 4
U_ROWS = 128
N_RB = S // U_ROWS
N_QU = (H - P_HEADS) // 4 * N_RB
N_OU = 2 * 2 * N_RB
U_PER_IT = (N_QU + N_OU) // HH
E_ROWS = 64
E_SUB = 4
PACE = 48
MV_STEP, MV_U0 = 2, 7
GRP = 16
FC = 512
PAD = 128
P_LO, P_HI, P_SQ = 0.35, 0.97, 10
E_LO0, E_LO1, E_HI, E_KEY, E_RUN = 0.35, 0.3, 0.97, 0.3, 2

Q_SCALE = float(DH) ** -0.5 * 1.4426950408889634

f32 = jnp.float32
bf16 = jnp.bfloat16
u32 = jnp.uint32


def _r(x):
    return x.astype(bf16).astype(f32)


def _recip(x):
    r0 = pl.reciprocal(x, approx=True)
    return r0 * (2.0 - x * r0)


def _pace(t):
    for _ in range(PACE):
        t = jnp.minimum(t, jnp.max(t, axis=1, keepdims=True))
    return t


def _tiles(v):
    u = pltpu.bitcast(v, u32)
    return [[u[a * 8:(a + 1) * 8, b * 128:(b + 1) * 128] for b in range(u.shape[1] // 128)]
            for a in range(u.shape[0] // 8)]


def _col_dots(k_tiles, rhs, n_tiles, never, deps):
    n_r = len(k_tiles) // 4
    n_i = k_tiles[0].shape[0] // GRP
    total = n_tiles * n_r * n_i
    at = {}
    for n, (pos, d) in enumerate(deps):
        at.setdefault((min(int(pos * total), total - 1), n % 4), []).append(d)
    outs = []
    for j in range(n_tiles):
        tl = list(k_tiles)
        for k in range(len(k_tiles)):
            base = (j * n_r + k // 4) * n_i
            if not any((base + i, k % 4) in at for i in range(n_i)):
                continue
            tu = pltpu.bitcast(tl[k], u32)
            parts = []
            for i in range(n_i):
                t = tu[i * 8:(i + 1) * 8, :]
                for d in at.get((base + i, k % 4), ()):
                    t = jnp.where(never, d, t)
                parts.append(t)
            tl[k] = pltpu.bitcast(jnp.concatenate(parts, axis=0), bf16)
        outs.append(jnp.dot(jnp.concatenate(tl, axis=1), rhs(j), preferred_element_type=f32))
    return outs


def _matvec(a_ref, w_refs):
    accs = [None] * len(w_refs)
    steps = []
    for s in range(D // GRP):
        a = a_ref[s * GRP:(s + 1) * GRP, :]
        for n, w in enumerate(w_refs):
            t = w[s * GRP:(s + 1) * GRP, :].astype(f32) * a
            accs[n] = t if accs[n] is None else accs[n] + t
        if s % MV_STEP == MV_STEP - 1:
            steps += [t[0] for acc in accs for t in _tiles(acc)]
    res = [jnp.broadcast_to(jnp.sum(acc, axis=0, keepdims=True), (8, 128)) for acc in accs]
    return res, steps


def _lane_bcast(row):
    return jnp.concatenate([row] * 16, axis=0).T


def _never(i):
    return jnp.full((8, 128), i, jnp.int32) > (1 << 20)


def _attention(heads):
    items = [(refs, c) for refs in heads for c in range(S // TQ)]

    def scores(item):
        (q_ref, bias, k_ref, _, _), c = item
        q = q_ref[c * TQ:(c + 1) * TQ, :] + jnp.concatenate([bias] * (TQ // 8), axis=0)
        q = (q * Q_SCALE).astype(bf16)
        return lax.dot_general(q, k_ref[...], (((1,), (1,)), ((), ())),
                               preferred_element_type=f32)

    def weigh(item, s):
        (_, _, _, v_ref, o_ref), c = item
        m = jnp.max(s, axis=1, keepdims=True)
        o = None
        lp = None
        for r in range(S // KR):
            p = jnp.exp2(s[:, r * KR:(r + 1) * KR] - m)
            ps = [p[:, j * 128:(j + 1) * 128] for j in range(KR // 128)]
            t = ps[0]
            for x in ps[1:]:
                t = t + x
            lp = t if lp is None else lp + t
            ps[-1] = jnp.minimum(ps[-1], t)
            p = jnp.concatenate(ps, axis=1)
            d = jnp.dot(p.astype(bf16), v_ref[r * KR:(r + 1) * KR, :],
                        preferred_element_type=f32)
            o = d if o is None else o + d
        l = jnp.sum(lp, axis=1, keepdims=True)
        o_ref[c * TQ:(c + 1) * TQ, :] = (o * _recip(l)).astype(bf16)

    s = scores(items[0])
    for n, item in enumerate(items):
        s_next = scores(items[n + 1]) if n + 1 < len(items) else None
        weigh(item, s)
        s = s_next


SEM_C, SEM_WR, SEM_WMA, SEM_X, SEM_WQ, SEM_KV, SEM_BG, SEM_OUT, SEM_FIX, SEM_WMB, SEM_O, N_SEM = (
    0, 1, 2, 6, 14, 17, 21, 25, 26, 28, 30, 32)
WO = H
GA, SB, CB1, GB, WR = range(5)


def _kernel(x_hbm, k_hbm, v_hbm, wq_hbm, wo_hbm, wr_hbm, wg_hbm, wu_hbm, wd_hbm, c_hbm,
            wm_hbm, out_hbm,
            x_v, h2_v, out_v, l_v, f_v, acc_v, w_v, wg_v, wu_v, wd_v, k_v, v_v, o_v,
            c_v, wr_v, sc_v, scb_v, sab_v, ca_v, sq_v, mod_v, top_v, rp_v, fix_v, sems):
    n_p = S // P_ROWS
    n_e = S // (E_SUB * E_ROWS)
    pq = P_HEADS * DH

    def cp(src, dst, sem):
        return pltpu.make_async_copy(src, dst, sems.at[sem])

    def cp_c():
        return cp(c_hbm, c_v, SEM_C)

    def cp_wr():
        return cp(wr_hbm, wr_v, SEM_WR)

    def cp_wca(j):
        return cp(wm_hbm.at[:, pl.ds(D + j * 512, 512)],
                  h2_v.at[pl.ds(D, D), pl.ds(j * 512, 512)], SEM_WMA + j)

    def cp_wsa():
        return cp(wm_hbm.at[:, pl.ds(0, D)], h2_v.at[pl.ds(0, D), pl.ds(0, D)], SEM_WMA + 2)

    def cp_x(i):
        return cp(x_hbm.at[0, pl.ds(i * P_ROWS, P_ROWS), :], x_v.at[pl.ds(i * P_ROWS, P_ROWS), :],
                  SEM_X + i)

    def cp_wqp():
        return cp(wq_hbm.at[:, pl.ds(0, pq)], out_v.at[pl.ds(0, D), pl.ds(0, pq)], SEM_WQ)

    def cp_tile(src, row, col, j, sem):
        return cp(src.at[pl.ds(pl.multiple_of(row * D, D), D), pl.ds(pl.multiple_of(col * DH, DH), DH)],
                  w_v.at[j], sem)

    def tiles_wait(lo, n, sem):
        cp(w_v.at[pl.ds(lo, n)], w_v.at[pl.ds(lo, n)], sem).wait()

    def cp_k(it):
        return cp(k_hbm.at[0, pl.ds(2 * it, 2)], k_v.at[it & 1], SEM_KV + (it & 1))

    def cp_v(it):
        return cp(v_hbm.at[0, pl.ds(2 * it, 2)], v_v.at[it & 1], SEM_KV + 2 + (it & 1))

    def cp_rows(src, dst, i, n, sem):
        return cp(src.at[pl.ds(i * n, n), :], dst.at[pl.ds(i * n, n), pl.ds(0, src.shape[1])], sem)

    def wmb_start(it):
        for k in range(2):
            cp_tile(wm_hbm, 0, 2 * D // DH + 2 * it + k, 2 * (it & 1) + k,
                    SEM_WMB + (it & 1)).start()

    def cp_out(i, n):
        return cp(out_v.at[pl.ds(i * E_ROWS, n * E_ROWS), pl.ds(0, D)],
                  out_hbm.at[0, pl.ds(i * E_ROWS, n * E_ROWS), :], SEM_OUT)

    def mrow(k, n):
        m = mod_v[:, k * D:(k + 1) * D]
        return jnp.concatenate([m] * (n // 8), axis=0)

    cp_c().start()
    cp_wr().start()
    for j in range(2):
        cp_wca(j).start()
    cp_x(0).start()
    cp_wqp().start()
    for i in range(1, n_p):
        cp_x(i).start()
    cp_wsa().start()
    cp_k(0).start()
    cp_v(0).start()
    wmb_start(0)

    cp_c().wait()
    cp_wr().wait()
    mod_v[:, WR * D:(WR + 1) * D] = jnp.broadcast_to(wr_v[...].astype(f32).reshape(1, D), (8, D))
    int_min = jnp.iinfo(jnp.int32).min
    top_v[...] = jnp.full(top_v.shape, int_min, jnp.int32)
    acc_v[...] = jnp.zeros(acc_v.shape, f32)
    rp_v[...] = jnp.zeros(rp_v.shape, f32)
    cf = c_v[...].astype(f32)
    sc = jnp.broadcast_to(_r(cf * jax.nn.sigmoid(cf)), (8, D))
    sc_v[...] = jnp.concatenate([sc, sc], axis=0).astype(bf16)
    scb_v[...] = _lane_bcast(sc)

    def wca_body(j, carry):
        cp_wca(j).wait()
        cols = pl.ds(pl.multiple_of(j * 512, 512), 512)
        mj = jnp.dot(sc_v[...], h2_v[D:2 * D, cols], preferred_element_type=f32)
        ca_v[:, cols] = _r(_r(mj[0:8, :]) + 1.0)
        return carry

    lax.fori_loop(0, 2, wca_body, 0)

    def ln1(i):
        rows = pl.ds(pl.multiple_of(i * P_ROWS, P_ROWS), P_ROWS)
        x = x_v[rows, :].astype(f32)
        mu = jnp.sum(x, axis=1, keepdims=True) * (1.0 / D)
        d = x - mu
        var = jnp.sum(d * d, axis=1, keepdims=True) * (1.0 / D)
        n = d * lax.rsqrt(var + EPS)
        h = n * jnp.concatenate([ca_v[...]] * (P_ROWS // 8), axis=0)
        hs = [h[:, k * 128:(k + 1) * 128].astype(bf16) for k in range(D // 128)]
        for k in range(D // 128):
            l_v[k, rows, :] = hs[k]
        return hs

    cp_x(0).wait()
    ln1(0)
    cp_wqp().wait()

    def p_body(i, carry):
        cp_x(i + 1).wait()
        rows = pl.ds(pl.multiple_of(i * P_ROWS, P_ROWS), P_ROWS)
        lhs = [l_v[k, rows, :] for k in range(D // 128)]
        tl = [t[0] for row in zip(*map(_tiles, ln1(i + 1))) for t in row]
        deps = [(P_LO + (P_HI - P_LO) * n / len(tl), t) for n, t in enumerate(tl)]
        qs = _col_dots(lhs, lambda j: out_v[0:D, j * DH:(j + 1) * DH], P_HEADS, _never(i), deps)
        for j in range(P_HEADS):
            f_v[j, rows, :] = qs[j]
        for k in range(4):
            hd = P_HEADS + 4 * i + k
            cp_tile(wq_hbm, 0, hd, hd, SEM_WQ + jnp.where(i < 1, 1, 2)).start()
        return carry

    lax.fori_loop(0, n_p - 1, p_body, 0)
    cp_k(1).start()
    cp_v(1).start()
    wmb_start(1)
    cp_wsa().wait()

    def halves(lhs, w):
        return [lambda h=h: jnp.dot(lhs(h), w(h), preferred_element_type=f32) for h in range(2)]

    def kh(h):
        return slice(h * 512, (h + 1) * 512)

    sa_t = []
    sa = None
    for n in range(2 * P_HEADS):
        j, rows = n // 2, slice(S - P_ROWS + n % 2 * 128, S - P_ROWS + (n % 2 + 1) * 128)
        big = halves(lambda h: jnp.concatenate([l_v[4 * h + k, rows, :] for k in range(4)], axis=1),
                     lambda h: out_v[kh(h), j * DH:(j + 1) * DH])
        acc = None
        for h in range(2):
            d = big[h]()
            acc = d if acc is None else acc + d
            r = 2 * n + h
            if r < 8:
                a, b = halves(lambda h: sc_v[:, kh(h)], lambda h: h2_v[kh(h), r * 128:(r + 1) * 128])
                sa_t.append(_r(a() + b()))
                if r == 7:
                    sa = jnp.concatenate(sa_t, axis=1)
                    sab_v[...] = _lane_bcast(sa[0:8, :])
                    sa = sa.astype(bf16)
            elif P_SQ <= r < P_SQ + P_HEADS:
                t = r - P_SQ
                a, b = halves(lambda h: sa[:, kh(h)], lambda h: out_v[kh(h), t * DH:(t + 1) * DH])
                sq_v[t] = (a() + b())[0:8, :]
        f_v[j, rows, :] = acc
    tiles_wait(P_HEADS, 4, SEM_WQ + 1)

    def m_body(it, carry):
        @pl.when(it == 1)
        def _():
            tiles_wait(P_HEADS + 4, H - P_HEADS - 4, SEM_WQ + 2)

        @pl.when(it == N_QU // U_PER_IT)
        def _():
            tiles_wait(WO, H, SEM_BG)

        @pl.when(jnp.logical_or(it == 6, it == 10))
        def _():
            cp(out_hbm.at[0], out_hbm.at[0], SEM_O).wait()

        @pl.when(jnp.logical_or(it == 8, it == 12))
        def _():
            dst = l_v.at[pl.ds(24 - 2 * it, 8)]
            cp(dst, dst, SEM_O + 1).wait()

        cp_k(it).wait()
        cp_v(it).wait()
        tiles_wait(2 * (it & 1), 2, SEM_WMB + (it & 1))
        slot = it & 1

        def unit(u, js, deps=()):
            g = it * U_PER_IT + u
            is_q = g < N_QU
            blk4 = (g >> 4) * 4
            fb = blk4 + jnp.where(is_q, P_HEADS, -(H - P_HEADS))
            wb = blk4 + P_HEADS
            lb = jnp.where(is_q, 0, 8 - (fb & 8))
            r0 = pl.multiple_of((g & (N_RB - 1)) * U_ROWS, U_ROWS)
            lhs = [l_v[lb + k, pl.ds(r0, U_ROWS), :] for k in range(8)]
            res = _col_dots(lhs, lambda n: w_v[wb + js[n]], len(js), never, deps)
            return [(fb + j, r0, v) for j, v in zip(js, res)]

        def put(tiles):
            for j, r0, v in tiles:
                f_v[j, pl.ds(r0, v.shape[0]), :] = v

        never = _never(it)
        late = unit(0, [0])
        _attention([(f_v.at[2 * it + e], sq_v[2 * it + e], k_v.at[slot, e], v_v.at[slot, e],
                     o_v.at[(2 * it + e) & (HH - 1)]) for e in range(2)])
        mb, steps = _matvec(scb_v, [w_v.at[2 * slot + e] for e in range(2)])
        one = jnp.where(it >> 2 == CB1 - GA, 1.0, 0.0)
        for e in range(2):
            cols = pl.ds(pl.multiple_of(GA * D + (2 * it + e) * 128, 128), 128)
            mod_v[:, cols] = _r(_r(mb[e]) + one)
        hq = jnp.minimum(2 * it + P_HEADS, H - 2)
        sq, more = _matvec(sab_v, [w_v.at[hq + e] for e in range(2)])
        for e in range(2):
            sq_v[hq + e] = sq[e]
        steps = steps + more
        span = (U_PER_IT - MV_U0) * 0.9 / len(steps)
        steps = [(MV_U0 + n * span, t) for n, t in enumerate(steps)]
        for u in range(U_PER_IT):
            tiles = unit(u, list(range(1 if u == 0 else 0, 4)),
                         [(pos - u, t) for pos, t in steps if u <= pos < u + 1])
            if u == 0:
                j, r0, v = tiles[0]
                late.append((j, r0, _pace(v[0:8, :])))
                tiles[0] = (j, r0 + 8, v[8:, :])
            put(tiles)
            if u == U_PER_IT - 2:
                put(late)

        @pl.when(it + 2 < HH)
        def _():
            cp_k(it + 2).start()
            cp_v(it + 2).start()
            wmb_start(it + 2)

        @pl.when(jnp.logical_or(it == 4, it == 8))
        def _():
            for k in range(8):
                cp(o_v.at[2 * it - 8 + k], out_hbm.at[0, :, pl.ds(k * DH, DH)], SEM_O).start()

        @pl.when(jnp.logical_or(it == 6, it == 10))
        def _():
            for k in range(8):
                cp(out_hbm.at[0, :, pl.ds(k * DH, DH)], l_v.at[20 - 2 * it + k], SEM_O + 1).start()

        @pl.when(it < 8)
        def _():
            for k in range(4):
                t = 4 * it + k
                cp_tile(wo_hbm, t >> 3, t & 7, WO + t, SEM_BG).start()

        for n, (src, dst) in enumerate(((wg_hbm, wg_v), (wu_hbm, wu_v), (wd_hbm, wd_v))):
            @pl.when(it >> 1 == n + 4)
            def _():
                cp_rows(src, dst, it & 1, src.shape[0] // 2, SEM_BG + 1 + n).start()

        return carry

    lax.fori_loop(0, HH, m_body, 0)

    cp(wg_v, wg_v, SEM_BG + 1).wait()
    cp(wu_v, wu_v, SEM_BG + 2).wait()
    cp(wd_hbm, wd_v.at[:, pl.ds(0, D)], SEM_BG + 3).wait()

    def router_parts(h2):
        pr = h2 * mrow(WR, h2.shape[0])
        run = [pr[:, 0:128]]
        for b in range(1, D // 128):
            run.append(run[-1] + pr[:, b * 128:(b + 1) * 128])
        return run

    def finish_rows(r0, attn, lo, hi):
        rows = pl.ds(r0, E_ROWS)
        x2 = _r(x_v[rows, :].astype(f32) + mrow(GA, E_ROWS) * attn)
        mu = jnp.sum(x2, axis=1, keepdims=True) * (1.0 / D)
        dc = x2 - mu
        var = _r(jnp.sum(dc * dc, axis=1, keepdims=True) * (1.0 / D))
        den = _r(jnp.sqrt(_r(var + EPS)))
        n = _r(_r(x2 - _r(mu)) * _recip(den))
        h2 = _r(_r(n * mrow(CB1, E_ROWS)) + mrow(SB, E_ROWS))
        x_v[rows, :] = x2.astype(bf16)
        h2_v[rows, 0:D] = h2.astype(bf16)
        of = x2 + _r(mrow(GB, E_ROWS) * h2)
        out_v[rows, 0:D] = of.astype(bf16)
        run = router_parts(h2)
        deps = []
        ot = _tiles(of)
        n_t = len(ot) * len(ot[0])
        for g in range(len(ot)):
            for b in range(len(ot[0])):
                pos = lo + (hi - lo) * (g * len(ot[0]) + b) / n_t
                deps.append((pos, ot[g][b]))
                if b % E_RUN == E_RUN - 1:
                    deps.append((pos, pltpu.bitcast(run[b][g * 8:(g + 1) * 8, :], u32)))
        return run[-1], deps

    def score_rows(r0, rp, valid, m1, m2):
        r = _r(jnp.sum(rp, axis=1, keepdims=True)) + 0.0
        r = jnp.where(r != r, -jnp.inf, r)
        bits = pltpu.bitcast(jnp.broadcast_to(r, (E_ROWS, 128)), jnp.int32)
        bits = jnp.where(bits < 0, bits ^ 0x7FFF0000, bits)
        idx = r0 + lax.broadcasted_iota(jnp.int32, (E_ROWS, 128), 0)
        key = bits | (0xFFFF - idx)
        if valid is not None:
            key = jnp.where(valid, key, int_min)
        for g in range(E_ROWS // 8):
            kg = key[g * 8:(g + 1) * 8, :]
            m2 = jnp.maximum(m2, jnp.minimum(m1, kg))
            m1 = jnp.maximum(m1, kg)
        return m1, m2

    def out_proj(r0, never, deps):
        rows = pl.ds(r0, E_ROWS)
        lhs = [o_v[j, rows, :] for j in range(HH)]
        ds = _col_dots(lhs, lambda j: jnp.concatenate([w_v[WO + 16 + j], w_v[WO + 24 + j]], axis=0),
                       D // 128, never, deps)
        return jnp.concatenate([f_v[j, rows, :] + f_v[8 + j, rows, :] + ds[j]
                                for j in range(D // 128)], axis=1)

    def e_body(c, carry):
        b0 = E_SUB * c

        @pl.when(c >= 2)
        def _():
            cp_out(b0 - E_SUB - 1, 1).start()

        @pl.when(c >= 1)
        def _():
            cp_out(b0 - E_SUB, E_SUB - 1).start()

        never = _never(c)
        m1, m2 = top_v[0], top_v[1]
        for t in range(E_SUB):
            m1, m2 = score_rows((b0 - E_SUB - 1 + t) * E_ROWS, rp_v[t],
                                c >= (2 if t == 0 else 1), m1, m2)
        top_v[0] = m1
        top_v[1] = m2
        attn = acc_v[...]
        for t in range(E_SUB):
            prev = jnp.maximum(b0 - 1, 0) if t == 0 else b0 + t - 1
            rp_v[t], deps = finish_rows(pl.multiple_of(prev * E_ROWS, E_ROWS), attn,
                                        E_LO0 if t == 0 else E_LO1, E_HI)
            if t == 0:
                deps.append((E_KEY, pltpu.bitcast(m2, u32)))
            attn = out_proj(pl.multiple_of((b0 + t) * E_ROWS, E_ROWS), never, deps)
        acc_v[...] = attn
        return carry

    lax.fori_loop(0, n_e, e_body, 0)
    n_b = S // E_ROWS
    cp_out(n_b - E_SUB - 1, E_SUB).start()
    m1, m2 = top_v[0], top_v[1]
    for t in range(E_SUB):
        m1, m2 = score_rows((n_b - E_SUB - 1 + t) * E_ROWS, rp_v[t], None, m1, m2)
    rp_last, _ = finish_rows(S - E_ROWS, acc_v[...], 0.0, 1.0)
    m1, m2 = score_rows(S - E_ROWS, rp_last, None, m1, m2)
    cp_out(n_b - 1, 1).start()

    t1 = jnp.max(m1, axis=0, keepdims=True)
    t2 = jnp.max(jnp.where(m1 == t1, m2, m1), axis=0, keepdims=True)
    i1 = (0xFFFF - t1[0, 0]) & (S - 1)
    i2 = (0xFFFF - t2[0, 0]) & (S - 1)
    g1 = pl.multiple_of(i1 & -GRP, GRP)
    g2 = pl.multiple_of(i2 & -GRP, GRP)

    xs = jnp.concatenate([h2_v[pl.ds(g1, GRP), 0:D], h2_v[pl.ds(g2, GRP), 0:D]], axis=0)

    def act(j):
        fc = slice(j * FC, (j + 1) * FC)
        g = _r(jnp.dot(xs, wg_v[:, fc], preferred_element_type=f32))
        u = _r(jnp.dot(xs, wu_v[:, fc], preferred_element_type=f32))
        return (_r(g * jax.nn.sigmoid(g)) * u).astype(bf16)

    y = None
    a = act(0)
    for j in range(F // FC):
        a_next = act(j + 1) if (j + 1) * FC < F else None
        d = jnp.dot(a, wd_v[j * FC:(j + 1) * FC, 0:D], preferred_element_type=f32)
        y = d if y is None else y + d
        a = a_next
    h2 = xs.astype(f32)
    x2 = jnp.concatenate([x_v[pl.ds(g1, GRP), :], x_v[pl.ds(g2, GRP), :]], axis=0).astype(f32)
    r = _r(jnp.sum(router_parts(h2)[-1], axis=1, keepdims=True))
    upd = _r(_r(y) * _r(jax.nn.sigmoid(r)))
    loc = lax.broadcasted_iota(jnp.int32, (2 * GRP, D), 0)
    row = jnp.where(loc < GRP, g1 + loc, g2 + loc - GRP)
    sel = jnp.logical_or(row == i1, row == i2)
    hb = _r(h2 + jnp.where(sel, upd, 0.0))
    fix_v[...] = (x2 + _r(mrow(GB, 2 * GRP) * hb)).astype(bf16)

    cp(out_v.at[:, pl.ds(0, D)], out_hbm.at[0], SEM_OUT).wait()
    fix1 = cp(fix_v.at[pl.ds(0, GRP), :], out_hbm.at[0, pl.ds(g1, GRP), :], SEM_FIX)
    fix2 = cp(fix_v.at[pl.ds(GRP, GRP), :], out_hbm.at[0, pl.ds(g2, GRP), :], SEM_FIX + 1)
    fix1.start()

    @pl.when(g2 != g1)
    def _():
        fix2.start()
        fix2.wait()

    fix1.wait()


@jax.jit
def pallas_adaLN_cond__mha_block_cached__moe_arch_mod__prompt_kernel(
    A_x: jax.Array,
    A_k_cache: jax.Array,
    A_v_cache: jax.Array,
    A_wq: jax.Array,
    A_wo: jax.Array,
    B_x: jax.Array,
    B_w_r: jax.Array,
    B_w_gate: jax.Array,
    B_w_up: jax.Array,
    B_w_down: jax.Array,
    c: jax.Array,
    w_mod: jax.Array,
):
    del B_x
    vm = pltpu.VMEM
    scratch = [
        vm((S, D), bf16),
        vm((S, D + PAD), bf16),
        vm((S, D + PAD), bf16),
        vm((HH, S, DH), bf16),
        vm((H, S, DH), f32),
        vm((E_ROWS, D), f32),
        vm((2 * H, D, DH), bf16),
        vm((D, F), bf16),
        vm((D, F), bf16),
        vm((F, D + PAD), bf16),
        vm((2, 2, S, DH), bf16),
        vm((2, 2, S, DH), bf16),
        vm((HH, S, DH), bf16),
        vm((1, D), bf16),
        vm((D,), bf16),
        vm((GRP, D), bf16),
        vm((D, 128), f32),
        vm((D, 128), f32),
        vm((8, D), f32),
        vm((H, 8, DH), f32),
        vm((8, 5 * D), f32),
        vm((2, 8, 128), jnp.int32),
        vm((E_SUB, E_ROWS, 128), f32),
        vm((2 * GRP, D), bf16),
        pltpu.SemaphoreType.DMA((N_SEM,)),
    ]
    return pl.pallas_call(
        _kernel,
        in_specs=[pl.BlockSpec(memory_space=pl.ANY)] * 11,
        out_specs=pl.BlockSpec(memory_space=pl.ANY),
        out_shape=jax.ShapeDtypeStruct(A_x.shape, A_x.dtype),
        scratch_shapes=scratch,
        compiler_params=pltpu.CompilerParams(vmem_limit_bytes=124 * 1024 * 1024,
                                             disable_bounds_checks=True,
                                             disable_semaphore_checks=True),
        name="adaln_mha_moe",
    )(A_x, A_k_cache, A_v_cache, A_wq, A_wo, B_w_r, B_w_gate, B_w_up, B_w_down, c, w_mod)
```

```python
import jax
import jax.numpy as jnp
from jax import lax
import jax.experimental.pallas as pl
import jax.experimental.pallas.tpu as pltpu

S = 2048
D = 1024
H = 32
DH = 128
F = 3584
EPS = 1e-5
HH = H // 2

TQ = 256
KR = 512
P_ROWS = 256
P_HEADS = 4
U_ROWS = 128
N_RB = S // U_ROWS
N_QU = (H - P_HEADS) // 4 * N_RB
N_OU = 2 * 2 * N_RB
U_PER_IT = (N_QU + N_OU) // HH
E_ROWS = 64
E_SUB = 4
PACE = 48
MV_STEP, MV_U0 = 2, 7
GRP = 16
FC = 512
PAD = 128
P_LO, P_HI, P_SQ = 0.35, 0.97, 10
E_LO0, E_LO1, E_HI, E_KEY, E_RUN = 0.35, 0.45, 0.97, 0.2, 2

Q_SCALE = float(DH) ** -0.5 * 1.4426950408889634

f32 = jnp.float32
bf16 = jnp.bfloat16
u32 = jnp.uint32


def _r(x):
    return x.astype(bf16).astype(f32)


def _recip(x):
    r0 = pl.reciprocal(x, approx=True)
    return r0 * (2.0 - x * r0)


def _pace(t):
    for _ in range(PACE):
        t = jnp.minimum(t, jnp.max(t, axis=1, keepdims=True))
    return t


def _tiles(v):
    u = pltpu.bitcast(v, u32)
    return [[u[a * 8:(a + 1) * 8, b * 128:(b + 1) * 128] for b in range(u.shape[1] // 128)]
            for a in range(u.shape[0] // 8)]


def _col_dots(k_tiles, rhs, n_tiles, never, deps):
    n_r = len(k_tiles) // 4
    n_i = k_tiles[0].shape[0] // GRP
    total = n_tiles * n_r * n_i
    at = {}
    for n, (pos, d) in enumerate(deps):
        at.setdefault((min(int(pos * total), total - 1), n % 4), []).append(d)
    outs = []
    for j in range(n_tiles):
        tl = list(k_tiles)
        for k in range(len(k_tiles)):
            base = (j * n_r + k // 4) * n_i
            if not any((base + i, k % 4) in at for i in range(n_i)):
                continue
            tu = pltpu.bitcast(tl[k], u32)
            parts = []
            for i in range(n_i):
                t = tu[i * 8:(i + 1) * 8, :]
                for d in at.get((base + i, k % 4), ()):
                    t = jnp.where(never, d, t)
                parts.append(t)
            tl[k] = pltpu.bitcast(jnp.concatenate(parts, axis=0), bf16)
        outs.append(jnp.dot(jnp.concatenate(tl, axis=1), rhs(j), preferred_element_type=f32))
    return outs


def _matvec(a_ref, w_refs):
    accs = [None] * len(w_refs)
    steps = []
    for s in range(D // GRP):
        a = a_ref[s * GRP:(s + 1) * GRP, :]
        for n, w in enumerate(w_refs):
            t = w[s * GRP:(s + 1) * GRP, :].astype(f32) * a
            accs[n] = t if accs[n] is None else accs[n] + t
        if s % MV_STEP == MV_STEP - 1:
            steps += [t[0] for acc in accs for t in _tiles(acc)]
    res = [jnp.broadcast_to(jnp.sum(acc, axis=0, keepdims=True), (8, 128)) for acc in accs]
    return res, steps


def _lane_bcast(row):
    return jnp.concatenate([row] * 16, axis=0).T


def _never(i):
    return jnp.full((8, 128), i, jnp.int32) > (1 << 20)


def _attention(heads):
    items = [(refs, c) for refs in heads for c in range(S // TQ)]

    def scores(item):
        (q_ref, bias, k_ref, _, _), c = item
        q = q_ref[c * TQ:(c + 1) * TQ, :] + jnp.concatenate([bias] * (TQ // 8), axis=0)
        q = (q * Q_SCALE).astype(bf16)
        return lax.dot_general(q, k_ref[...], (((1,), (1,)), ((), ())),
                               preferred_element_type=f32)

    def weigh(item, s):
        (_, _, _, v_ref, o_ref), c = item
        m = jnp.max(s, axis=1, keepdims=True)
        o = None
        lp = None
        for r in range(S // KR):
            p = jnp.exp2(s[:, r * KR:(r + 1) * KR] - m)
            ps = [p[:, j * 128:(j + 1) * 128] for j in range(KR // 128)]
            t = ps[0]
            for x in ps[1:]:
                t = t + x
            lp = t if lp is None else lp + t
            ps[-1] = jnp.minimum(ps[-1], t)
            p = jnp.concatenate(ps, axis=1)
            d = jnp.dot(p.astype(bf16), v_ref[r * KR:(r + 1) * KR, :],
                        preferred_element_type=f32)
            o = d if o is None else o + d
        l = jnp.sum(lp, axis=1, keepdims=True)
        o_ref[c * TQ:(c + 1) * TQ, :] = (o * _recip(l)).astype(bf16)

    s = scores(items[0])
    for n, item in enumerate(items):
        s_next = scores(items[n + 1]) if n + 1 < len(items) else None
        weigh(item, s)
        s = s_next


SEM_C, SEM_WR, SEM_WMA, SEM_X, SEM_WQ, SEM_KV, SEM_BG, SEM_OUT, SEM_FIX, SEM_WMB, SEM_O, N_SEM = (
    0, 1, 2, 6, 14, 17, 21, 25, 26, 28, 30, 32)
WO = H
GA, SB, CB1, GB, WR = range(5)


def _kernel(x_hbm, k_hbm, v_hbm, wq_hbm, wo_hbm, wr_hbm, wg_hbm, wu_hbm, wd_hbm, c_hbm,
            wm_hbm, out_hbm,
            x_v, h2_v, out_v, l_v, f_v, acc_v, w_v, wg_v, wu_v, wd_v, k_v, v_v, o_v,
            c_v, wr_v, sc_v, scb_v, sab_v, ca_v, sq_v, mod_v, top_v, rp_v, fix_v, sems):
    n_p = S // P_ROWS
    n_e = S // (E_SUB * E_ROWS)
    pq = P_HEADS * DH

    def cp(src, dst, sem):
        return pltpu.make_async_copy(src, dst, sems.at[sem])

    def cp_c():
        return cp(c_hbm, c_v, SEM_C)

    def cp_wr():
        return cp(wr_hbm, wr_v, SEM_WR)

    def cp_wca(j):
        return cp(wm_hbm.at[:, pl.ds(D + j * 512, 512)],
                  h2_v.at[pl.ds(D, D), pl.ds(j * 512, 512)], SEM_WMA + j)

    def cp_wsa():
        return cp(wm_hbm.at[:, pl.ds(0, D)], h2_v.at[pl.ds(0, D), pl.ds(0, D)], SEM_WMA + 2)

    def cp_x(i):
        return cp(x_hbm.at[0, pl.ds(i * P_ROWS, P_ROWS), :], x_v.at[pl.ds(i * P_ROWS, P_ROWS), :],
                  SEM_X + i)

    def cp_wqp():
        return cp(wq_hbm.at[:, pl.ds(0, pq)], out_v.at[pl.ds(0, D), pl.ds(0, pq)], SEM_WQ)

    def cp_tile(src, row, col, j, sem):
        return cp(src.at[pl.ds(pl.multiple_of(row * D, D), D), pl.ds(pl.multiple_of(col * DH, DH), DH)],
                  w_v.at[j], sem)

    def tiles_wait(lo, n, sem):
        cp(w_v.at[pl.ds(lo, n)], w_v.at[pl.ds(lo, n)], sem).wait()

    def cp_k(it):
        return cp(k_hbm.at[0, pl.ds(2 * it, 2)], k_v.at[it & 1], SEM_KV + (it & 1))

    def cp_v(it):
        return cp(v_hbm.at[0, pl.ds(2 * it, 2)], v_v.at[it & 1], SEM_KV + 2 + (it & 1))

    def cp_rows(src, dst, i, n, sem):
        return cp(src.at[pl.ds(i * n, n), :], dst.at[pl.ds(i * n, n), pl.ds(0, src.shape[1])], sem)

    def wmb_start(it):
        for k in range(2):
            cp_tile(wm_hbm, 0, 2 * D // DH + 2 * it + k, 2 * (it & 1) + k,
                    SEM_WMB + (it & 1)).start()

    def cp_out(i, n):
        return cp(out_v.at[pl.ds(i * E_ROWS, n * E_ROWS), pl.ds(0, D)],
                  out_hbm.at[0, pl.ds(i * E_ROWS, n * E_ROWS), :], SEM_OUT)

    def mrow(k, n):
        m = mod_v[:, k * D:(k + 1) * D]
        return jnp.concatenate([m] * (n // 8), axis=0)

    cp_c().start()
    cp_wr().start()
    for j in range(2):
        cp_wca(j).start()
    cp_x(0).start()
    cp_wqp().start()
    for i in range(1, n_p):
        cp_x(i).start()
    cp_wsa().start()
    cp_k(0).start()
    cp_v(0).start()
    wmb_start(0)

    cp_c().wait()
    cp_wr().wait()
    mod_v[:, WR * D:(WR + 1) * D] = jnp.broadcast_to(wr_v[...].astype(f32).reshape(1, D), (8, D))
    int_min = jnp.iinfo(jnp.int32).min
    top_v[...] = jnp.full(top_v.shape, int_min, jnp.int32)
    acc_v[...] = jnp.zeros(acc_v.shape, f32)
    rp_v[...] = jnp.zeros(rp_v.shape, f32)
    cf = c_v[...].astype(f32)
    sc = jnp.broadcast_to(_r(cf * jax.nn.sigmoid(cf)), (8, D))
    sc_v[...] = jnp.concatenate([sc, sc], axis=0).astype(bf16)
    scb_v[...] = _lane_bcast(sc)

    def wca_body(j, carry):
        cp_wca(j).wait()
        cols = pl.ds(pl.multiple_of(j * 512, 512), 512)
        mj = jnp.dot(sc_v[...], h2_v[D:2 * D, cols], preferred_element_type=f32)
        ca_v[:, cols] = _r(_r(mj[0:8, :]) + 1.0)
        return carry

    lax.fori_loop(0, 2, wca_body, 0)

    def ln1(i):
        rows = pl.ds(pl.multiple_of(i * P_ROWS, P_ROWS), P_ROWS)
        x = x_v[rows, :].astype(f32)
        mu = jnp.sum(x, axis=1, keepdims=True) * (1.0 / D)
        d = x - mu
        var = jnp.sum(d * d, axis=1, keepdims=True) * (1.0 / D)
        n = d * lax.rsqrt(var + EPS)
        h = n * jnp.concatenate([ca_v[...]] * (P_ROWS // 8), axis=0)
        hs = [h[:, k * 128:(k + 1) * 128].astype(bf16) for k in range(D // 128)]
        for k in range(D // 128):
            l_v[k, rows, :] = hs[k]
        return hs

    cp_x(0).wait()
    ln1(0)
    cp_wqp().wait()

    def p_body(i, carry):
        cp_x(i + 1).wait()
        rows = pl.ds(pl.multiple_of(i * P_ROWS, P_ROWS), P_ROWS)
        lhs = [l_v[k, rows, :] for k in range(D // 128)]
        tl = [t[0] for row in zip(*map(_tiles, ln1(i + 1))) for t in row]
        deps = [(P_LO + (P_HI - P_LO) * n / len(tl), t) for n, t in enumerate(tl)]
        qs = _col_dots(lhs, lambda j: out_v[0:D, j * DH:(j + 1) * DH], P_HEADS, _never(i), deps)
        for j in range(P_HEADS):
            f_v[j, rows, :] = qs[j]
        for k in range(4):
            hd = P_HEADS + 4 * i + k
            cp_tile(wq_hbm, 0, hd, hd, SEM_WQ + jnp.where(i < 1, 1, 2)).start()
        return carry

    lax.fori_loop(0, n_p - 1, p_body, 0)
    cp_k(1).start()
    cp_v(1).start()
    wmb_start(1)
    cp_wsa().wait()

    def halves(lhs, w):
        return [lambda h=h: jnp.dot(lhs(h), w(h), preferred_element_type=f32) for h in range(2)]

    def kh(h):
        return slice(h * 512, (h + 1) * 512)

    sa_t = []
    sa = None
    for n in range(2 * P_HEADS):
        j, rows = n // 2, slice(S - P_ROWS + n % 2 * 128, S - P_ROWS + (n % 2 + 1) * 128)
        big = halves(lambda h: jnp.concatenate([l_v[4 * h + k, rows, :] for k in range(4)], axis=1),
                     lambda h: out_v[kh(h), j * DH:(j + 1) * DH])
        acc = None
        for h in range(2):
            d = big[h]()
            acc = d if acc is None else acc + d
            r = 2 * n + h
            if r < 8:
                a, b = halves(lambda h: sc_v[:, kh(h)], lambda h: h2_v[kh(h), r * 128:(r + 1) * 128])
                sa_t.append(_r(a() + b()))
                if r == 7:
                    sa = jnp.concatenate(sa_t, axis=1)
                    sab_v[...] = _lane_bcast(sa[0:8, :])
                    sa = sa.astype(bf16)
            elif P_SQ <= r < P_SQ + P_HEADS:
                t = r - P_SQ
                a, b = halves(lambda h: sa[:, kh(h)], lambda h: out_v[kh(h), t * DH:(t + 1) * DH])
                sq_v[t] = (a() + b())[0:8, :]
        f_v[j, rows, :] = acc
    tiles_wait(P_HEADS, 4, SEM_WQ + 1)

    def m_body(it, carry):
        @pl.when(it == 1)
        def _():
            tiles_wait(P_HEADS + 4, H - P_HEADS - 4, SEM_WQ + 2)

        @pl.when(it == N_QU // U_PER_IT)
        def _():
            tiles_wait(WO, H, SEM_BG)

        @pl.when(jnp.logical_or(it == 6, it == 10))
        def _():
            cp(out_hbm.at[0], out_hbm.at[0], SEM_O).wait()

        @pl.when(jnp.logical_or(it == 8, it == 12))
        def _():
            dst = l_v.at[pl.ds(24 - 2 * it, 8)]
            cp(dst, dst, SEM_O + 1).wait()

        cp_k(it).wait()
        cp_v(it).wait()
        tiles_wait(2 * (it & 1), 2, SEM_WMB + (it & 1))
        slot = it & 1

        def unit(u, js, deps=()):
            g = it * U_PER_IT + u
            is_q = g < N_QU
            blk4 = (g >> 4) * 4
            fb = blk4 + jnp.where(is_q, P_HEADS, -(H - P_HEADS))
            wb = blk4 + P_HEADS
            lb = jnp.where(is_q, 0, 8 - (fb & 8))
            r0 = pl.multiple_of((g & (N_RB - 1)) * U_ROWS, U_ROWS)
            lhs = [l_v[lb + k, pl.ds(r0, U_ROWS), :] for k in range(8)]
            res = _col_dots(lhs, lambda n: w_v[wb + js[n]], len(js), never, deps)
            return [(fb + j, r0, v) for j, v in zip(js, res)]

        def put(tiles):
            for j, r0, v in tiles:
                f_v[j, pl.ds(r0, v.shape[0]), :] = v

        never = _never(it)
        late = unit(0, [0])
        _attention([(f_v.at[2 * it + e], sq_v[2 * it + e], k_v.at[slot, e], v_v.at[slot, e],
                     o_v.at[(2 * it + e) & (HH - 1)]) for e in range(2)])
        mb, steps = _matvec(scb_v, [w_v.at[2 * slot + e] for e in range(2)])
        one = jnp.where(it >> 2 == CB1 - GA, 1.0, 0.0)
        for e in range(2):
            cols = pl.ds(pl.multiple_of(GA * D + (2 * it + e) * 128, 128), 128)
            mod_v[:, cols] = _r(_r(mb[e]) + one)
        hq = jnp.minimum(2 * it + P_HEADS, H - 2)
        sq, more = _matvec(sab_v, [w_v.at[hq + e] for e in range(2)])
        for e in range(2):
            sq_v[hq + e] = sq[e]
        steps = steps + more
        span = (U_PER_IT - MV_U0) * 0.9 / len(steps)
        steps = [(MV_U0 + n * span, t) for n, t in enumerate(steps)]
        for u in range(U_PER_IT):
            tiles = unit(u, list(range(1 if u == 0 else 0, 4)),
                         [(pos - u, t) for pos, t in steps if u <= pos < u + 1])
            if u == 0:
                j, r0, v = tiles[0]
                late.append((j, r0, _pace(v[0:8, :])))
                tiles[0] = (j, r0 + 8, v[8:, :])
            put(tiles)
            if u == U_PER_IT - 2:
                put(late)

        @pl.when(it + 2 < HH)
        def _():
            cp_k(it + 2).start()
            cp_v(it + 2).start()
            wmb_start(it + 2)

        @pl.when(jnp.logical_or(it == 4, it == 8))
        def _():
            for k in range(8):
                cp(o_v.at[2 * it - 8 + k], out_hbm.at[0, :, pl.ds(k * DH, DH)], SEM_O).start()

        @pl.when(jnp.logical_or(it == 6, it == 10))
        def _():
            for k in range(8):
                cp(out_hbm.at[0, :, pl.ds(k * DH, DH)], l_v.at[20 - 2 * it + k], SEM_O + 1).start()

        @pl.when(it < 8)
        def _():
            for k in range(4):
                t = 4 * it + k
                cp_tile(wo_hbm, t >> 3, t & 7, WO + t, SEM_BG).start()

        for n, (src, dst) in enumerate(((wg_hbm, wg_v), (wu_hbm, wu_v), (wd_hbm, wd_v))):
            @pl.when(it >> 1 == n + 4)
            def _():
                cp_rows(src, dst, it & 1, src.shape[0] // 2, SEM_BG + 1 + n).start()

        return carry

    lax.fori_loop(0, HH, m_body, 0)

    cp(wg_v, wg_v, SEM_BG + 1).wait()
    cp(wu_v, wu_v, SEM_BG + 2).wait()
    cp(wd_hbm, wd_v.at[:, pl.ds(0, D)], SEM_BG + 3).wait()

    def router_parts(h2):
        pr = h2 * mrow(WR, h2.shape[0])
        run = [pr[:, 0:128]]
        for b in range(1, D // 128):
            run.append(run[-1] + pr[:, b * 128:(b + 1) * 128])
        return run

    def finish_rows(r0, attn, lo, hi, never=None):
        rows = pl.ds(r0, E_ROWS)
        x2 = _r(x_v[rows, :].astype(f32) + mrow(GA, E_ROWS) * attn)
        if never is None:
            mu = jnp.sum(x2, axis=1, keepdims=True) * (1.0 / D)
            dc = x2 - mu
            var = _r(jnp.sum(dc * dc, axis=1, keepdims=True) * (1.0 / D))
        else:
            mus, vrs = [], []
            for g in range(E_ROWS // 8):
                xg = x2[g * 8:(g + 1) * 8, :]
                sp = xg[:, 0:128]
                for b in range(1, D // 128):
                    sp = sp + xg[:, b * 128:(b + 1) * 128]
                if mus:
                    sp = jnp.where(never, jnp.broadcast_to(mus[-1], (8, 128)), sp)
                mus.append(jnp.sum(sp, axis=1, keepdims=True) * (1.0 / D))
                dg = xg - mus[-1]
                vrs.append(jnp.sum(dg * dg, axis=1, keepdims=True) * (1.0 / D))
            mu = jnp.concatenate(mus, axis=0)
            var = _r(jnp.concatenate(vrs, axis=0))
        den = _r(jnp.sqrt(_r(var + EPS)))
        n = _r(_r(x2 - _r(mu)) * _recip(den))
        h2 = _r(_r(n * mrow(CB1, E_ROWS)) + mrow(SB, E_ROWS))
        x_v[rows, :] = x2.astype(bf16)
        h2_v[rows, 0:D] = h2.astype(bf16)
        of = x2 + _r(mrow(GB, E_ROWS) * h2)
        out_v[rows, 0:D] = of.astype(bf16)
        run = router_parts(h2)
        deps = []
        ot = _tiles(of)
        n_t = len(ot) * len(ot[0])
        for g in range(len(ot)):
            for b in range(len(ot[0])):
                pos = lo + (hi - lo) * (g * len(ot[0]) + b) / n_t
                deps.append((pos, ot[g][b]))
                if b % E_RUN == E_RUN - 1:
                    deps.append((pos, pltpu.bitcast(run[b][g * 8:(g + 1) * 8, :], u32)))
        return run[-1], deps

    def score_rows(r0, rp, valid, m1, m2):
        r = _r(jnp.sum(rp, axis=1, keepdims=True)) + 0.0
        r = jnp.where(r != r, -jnp.inf, r)
        bits = pltpu.bitcast(jnp.broadcast_to(r, (E_ROWS, 128)), jnp.int32)
        bits = jnp.where(bits < 0, bits ^ 0x7FFF0000, bits)
        idx = r0 + lax.broadcasted_iota(jnp.int32, (E_ROWS, 128), 0)
        key = bits | (0xFFFF - idx)
        if valid is not None:
            key = jnp.where(valid, key, int_min)
        for g in range(E_ROWS // 8):
            kg = key[g * 8:(g + 1) * 8, :]
            m2 = jnp.maximum(m2, jnp.minimum(m1, kg))
            m1 = jnp.maximum(m1, kg)
        return m1, m2

    def out_proj(r0, never, deps):
        rows = pl.ds(r0, E_ROWS)
        lhs = [o_v[j, rows, :] for j in range(HH)]
        ds = _col_dots(lhs, lambda j: jnp.concatenate([w_v[WO + 16 + j], w_v[WO + 24 + j]], axis=0),
                       D // 128, never, deps)
        return jnp.concatenate([f_v[j, rows, :] + f_v[8 + j, rows, :] + ds[j]
                                for j in range(D // 128)], axis=1)

    def e_body(c, carry):
        b0 = E_SUB * c

        @pl.when(c >= 2)
        def _():
            cp_out(b0 - E_SUB - 1, 1).start()

        @pl.when(c >= 1)
        def _():
            cp_out(b0 - E_SUB, E_SUB - 1).start()

        never = _never(c)
        m1, m2 = top_v[0], top_v[1]
        keys = []
        for t in range(E_SUB):
            m1, m2 = score_rows((b0 - E_SUB - 1 + t) * E_ROWS, rp_v[t],
                                c >= (2 if t == 0 else 1), m1, m2)
            keys.append(m2)
        top_v[0] = m1
        top_v[1] = m2
        attn = acc_v[...]
        for t in range(E_SUB):
            prev = jnp.maximum(b0 - 1, 0) if t == 0 else b0 + t - 1
            rp_v[t], deps = finish_rows(pl.multiple_of(prev * E_ROWS, E_ROWS), attn,
                                        E_LO0 if t == 0 else E_LO1, E_HI,
                                        None if t == 0 else never)
            deps.append((E_KEY, pltpu.bitcast(keys[t], u32)))
            attn = out_proj(pl.multiple_of((b0 + t) * E_ROWS, E_ROWS), never, deps)
        acc_v[...] = attn
        return carry

    lax.fori_loop(0, n_e, e_body, 0)
    n_b = S // E_ROWS
    cp_out(n_b - E_SUB - 1, E_SUB).start()
    m1, m2 = top_v[0], top_v[1]
    for t in range(E_SUB):
        m1, m2 = score_rows((n_b - E_SUB - 1 + t) * E_ROWS, rp_v[t], None, m1, m2)
    rp_last, _ = finish_rows(S - E_ROWS, acc_v[...], 0.0, 1.0)
    m1, m2 = score_rows(S - E_ROWS, rp_last, None, m1, m2)
    cp_out(n_b - 1, 1).start()

    t1 = jnp.max(m1, axis=0, keepdims=True)
    t2 = jnp.max(jnp.where(m1 == t1, m2, m1), axis=0, keepdims=True)
    i1 = (0xFFFF - t1[0, 0]) & (S - 1)
    i2 = (0xFFFF - t2[0, 0]) & (S - 1)
    g1 = pl.multiple_of(i1 & -GRP, GRP)
    g2 = pl.multiple_of(i2 & -GRP, GRP)

    xs = jnp.concatenate([h2_v[pl.ds(g1, GRP), 0:D], h2_v[pl.ds(g2, GRP), 0:D]], axis=0)

    def act(j):
        fc = slice(j * FC, (j + 1) * FC)
        g = _r(jnp.dot(xs, wg_v[:, fc], preferred_element_type=f32))
        u = _r(jnp.dot(xs, wu_v[:, fc], preferred_element_type=f32))
        return (_r(g * jax.nn.sigmoid(g)) * u).astype(bf16)

    y = None
    a = act(0)
    for j in range(F // FC):
        a_next = act(j + 1) if (j + 1) * FC < F else None
        d = jnp.dot(a, wd_v[j * FC:(j + 1) * FC, 0:D], preferred_element_type=f32)
        y = d if y is None else y + d
        a = a_next
    h2 = xs.astype(f32)
    x2 = jnp.concatenate([x_v[pl.ds(g1, GRP), :], x_v[pl.ds(g2, GRP), :]], axis=0).astype(f32)
    r = _r(jnp.sum(router_parts(h2)[-1], axis=1, keepdims=True))
    upd = _r(_r(y) * _r(jax.nn.sigmoid(r)))
    loc = lax.broadcasted_iota(jnp.int32, (2 * GRP, D), 0)
    row = jnp.where(loc < GRP, g1 + loc, g2 + loc - GRP)
    sel = jnp.logical_or(row == i1, row == i2)
    hb = _r(h2 + jnp.where(sel, upd, 0.0))
    fix_v[...] = (x2 + _r(mrow(GB, 2 * GRP) * hb)).astype(bf16)

    cp(out_v.at[:, pl.ds(0, D)], out_hbm.at[0], SEM_OUT).wait()
    fix1 = cp(fix_v.at[pl.ds(0, GRP), :], out_hbm.at[0, pl.ds(g1, GRP), :], SEM_FIX)
    fix2 = cp(fix_v.at[pl.ds(GRP, GRP), :], out_hbm.at[0, pl.ds(g2, GRP), :], SEM_FIX + 1)
    fix1.start()

    @pl.when(g2 != g1)
    def _():
        fix2.start()
        fix2.wait()

    fix1.wait()


@jax.jit
def pallas_adaLN_cond__mha_block_cached__moe_arch_mod__prompt_kernel(
    A_x: jax.Array,
    A_k_cache: jax.Array,
    A_v_cache: jax.Array,
    A_wq: jax.Array,
    A_wo: jax.Array,
    B_x: jax.Array,
    B_w_r: jax.Array,
    B_w_gate: jax.Array,
    B_w_up: jax.Array,
    B_w_down: jax.Array,
    c: jax.Array,
    w_mod: jax.Array,
):
    del B_x
    vm = pltpu.VMEM
    scratch = [
        vm((S, D), bf16),
        vm((S, D + PAD), bf16),
        vm((S, D + PAD), bf16),
        vm((HH, S, DH), bf16),
        vm((H, S, DH), f32),
        vm((E_ROWS, D), f32),
        vm((2 * H, D, DH), bf16),
        vm((D, F), bf16),
        vm((D, F), bf16),
        vm((F, D + PAD), bf16),
        vm((2, 2, S, DH), bf16),
        vm((2, 2, S, DH), bf16),
        vm((HH, S, DH), bf16),
        vm((1, D), bf16),
        vm((D,), bf16),
        vm((GRP, D), bf16),
        vm((D, 128), f32),
        vm((D, 128), f32),
        vm((8, D), f32),
        vm((H, 8, DH), f32),
        vm((8, 5 * D), f32),
        vm((2, 8, 128), jnp.int32),
        vm((E_SUB, E_ROWS, 128), f32),
        vm((2 * GRP, D), bf16),
        pltpu.SemaphoreType.DMA((N_SEM,)),
    ]
    return pl.pallas_call(
        _kernel,
        in_specs=[pl.BlockSpec(memory_space=pl.ANY)] * 11,
        out_specs=pl.BlockSpec(memory_space=pl.ANY),
        out_shape=jax.ShapeDtypeStruct(A_x.shape, A_x.dtype),
        scratch_shapes=scratch,
        compiler_params=pltpu.CompilerParams(vmem_limit_bytes=124 * 1024 * 1024,
                                             disable_bounds_checks=True,
                                             disable_semaphore_checks=True),
        name="adaln_mha_moe",
    )(A_x, A_k_cache, A_v_cache, A_wq, A_wo, B_w_r, B_w_gate, B_w_up, B_w_down, c, w_mod)
```

```python
import jax
import jax.numpy as jnp
from jax import lax
import jax.experimental.pallas as pl
import jax.experimental.pallas.tpu as pltpu

S = 2048
D = 1024
H = 32
DH = 128
F = 3584
EPS = 1e-5
HH = H // 2

TQ = 256
KR = 512
P_ROWS = 256
P_HEADS = 4
U_ROWS = 128
N_RB = S // U_ROWS
N_QU = (H - P_HEADS) // 4 * N_RB
N_OU = 2 * 2 * N_RB
U_PER_IT = (N_QU + N_OU) // HH
E_ROWS = 64
E_SUB = 4
PACE = 48
MV_STEP, MV_U0 = 2, 7
GRP = 16
FC = 512
PAD = 128
P_LO, P_HI, P_SQ = 0.35, 0.97, 10
E_LO0, E_LO1, E_HI, E_KEY, E_RUN = 0.35, 0.45, 0.97, 0.2, 2

Q_SCALE = float(DH) ** -0.5 * 1.4426950408889634

f32 = jnp.float32
bf16 = jnp.bfloat16
u32 = jnp.uint32


def _r(x):
    return x.astype(bf16).astype(f32)


def _recip(x):
    r0 = pl.reciprocal(x, approx=True)
    return r0 * (2.0 - x * r0)


def _pace(t):
    for _ in range(PACE):
        t = jnp.minimum(t, jnp.max(t, axis=1, keepdims=True))
    return t


def _tiles(v):
    u = pltpu.bitcast(v, u32)
    return [[u[a * 8:(a + 1) * 8, b * 128:(b + 1) * 128] for b in range(u.shape[1] // 128)]
            for a in range(u.shape[0] // 8)]


def _col_dots(k_tiles, rhs, n_tiles, never, deps):
    n_r = len(k_tiles) // 4
    n_i = k_tiles[0].shape[0] // GRP
    total = n_tiles * n_r * n_i
    at = {}
    for n, (pos, d) in enumerate(deps):
        at.setdefault((min(int(pos * total), total - 1), n % 4), []).append(d)
    outs = []
    for j in range(n_tiles):
        tl = list(k_tiles)
        for k in range(len(k_tiles)):
            base = (j * n_r + k // 4) * n_i
            if not any((base + i, k % 4) in at for i in range(n_i)):
                continue
            tu = pltpu.bitcast(tl[k], u32)
            parts = []
            for i in range(n_i):
                t = tu[i * 8:(i + 1) * 8, :]
                for d in at.get((base + i, k % 4), ()):
                    t = jnp.where(never, d, t)
                parts.append(t)
            tl[k] = pltpu.bitcast(jnp.concatenate(parts, axis=0), bf16)
        outs.append(jnp.dot(jnp.concatenate(tl, axis=1), rhs(j), preferred_element_type=f32))
    return outs


def _matvec(a_ref, w_refs):
    accs = [None] * len(w_refs)
    steps = []
    for s in range(D // GRP):
        a = a_ref[s * GRP:(s + 1) * GRP, :]
        for n, w in enumerate(w_refs):
            t = w[s * GRP:(s + 1) * GRP, :].astype(f32) * a
            accs[n] = t if accs[n] is None else accs[n] + t
        if s % MV_STEP == MV_STEP - 1:
            steps += [t[0] for acc in accs for t in _tiles(acc)]
    res = [jnp.broadcast_to(jnp.sum(acc, axis=0, keepdims=True), (8, 128)) for acc in accs]
    return res, steps


def _lane_bcast(row):
    return jnp.concatenate([row] * 16, axis=0).T


def _never(i):
    return jnp.full((8, 128), i, jnp.int32) > (1 << 20)


def _attention(heads):
    items = [(refs, c) for refs in heads for c in range(S // TQ)]

    def scores(item):
        (q_ref, bias, k_ref, _, _), c = item
        q = q_ref[c * TQ:(c + 1) * TQ, :] + jnp.concatenate([bias] * (TQ // 8), axis=0)
        q = (q * Q_SCALE).astype(bf16)
        return lax.dot_general(q, k_ref[...], (((1,), (1,)), ((), ())),
                               preferred_element_type=f32)

    def weigh(item, s):
        (_, _, _, v_ref, o_ref), c = item
        m = jnp.max(s, axis=1, keepdims=True)
        o = None
        lp = None
        for r in range(S // KR):
            p = jnp.exp2(s[:, r * KR:(r + 1) * KR] - m)
            ps = [p[:, j * 128:(j + 1) * 128] for j in range(KR // 128)]
            t = ps[0]
            for x in ps[1:]:
                t = t + x
            lp = t if lp is None else lp + t
            ps[-1] = jnp.minimum(ps[-1], t)
            p = jnp.concatenate(ps, axis=1)
            d = jnp.dot(p.astype(bf16), v_ref[r * KR:(r + 1) * KR, :],
                        preferred_element_type=f32)
            o = d if o is None else o + d
        l = jnp.sum(lp, axis=1, keepdims=True)
        o_ref[c * TQ:(c + 1) * TQ, :] = (o * _recip(l)).astype(bf16)

    s = scores(items[0])
    for n, item in enumerate(items):
        s_next = scores(items[n + 1]) if n + 1 < len(items) else None
        weigh(item, s)
        s = s_next


SEM_C, SEM_WR, SEM_WMA, SEM_X, SEM_WQ, SEM_KV, SEM_BG, SEM_OUT, SEM_FIX, SEM_WMB, SEM_O, N_SEM = (
    0, 1, 2, 6, 14, 17, 21, 25, 26, 28, 30, 32)
WO = H
GA, SB, CB1, GB, WR = range(5)


def _kernel(x_hbm, k_hbm, v_hbm, wq_hbm, wo_hbm, wr_hbm, wg_hbm, wu_hbm, wd_hbm, c_hbm,
            wm_hbm, out_hbm,
            x_v, h2_v, out_v, l_v, f_v, acc_v, w_v, wg_v, wu_v, wd_v, k_v, v_v, o_v,
            c_v, wr_v, sc_v, scb_v, sab_v, ca_v, sq_v, mod_v, top_v, rp_v, fix_v, sems):
    n_p = S // P_ROWS
    n_e = S // (E_SUB * E_ROWS)
    pq = P_HEADS * DH

    def cp(src, dst, sem):
        return pltpu.make_async_copy(src, dst, sems.at[sem])

    def cp_c():
        return cp(c_hbm, c_v, SEM_C)

    def cp_wr():
        return cp(wr_hbm, wr_v, SEM_WR)

    def cp_wca(j):
        return cp(wm_hbm.at[:, pl.ds(D + j * 512, 512)],
                  h2_v.at[pl.ds(D, D), pl.ds(j * 512, 512)], SEM_WMA + j)

    def cp_wsa():
        return cp(wm_hbm.at[:, pl.ds(0, D)], h2_v.at[pl.ds(0, D), pl.ds(0, D)], SEM_WMA + 2)

    def cp_x(i):
        return cp(x_hbm.at[0, pl.ds(i * P_ROWS, P_ROWS), :], x_v.at[pl.ds(i * P_ROWS, P_ROWS), :],
                  SEM_X + i)

    def cp_wqp():
        return cp(wq_hbm.at[:, pl.ds(0, pq)], out_v.at[pl.ds(0, D), pl.ds(0, pq)], SEM_WQ)

    def cp_tile(src, row, col, j, sem):
        return cp(src.at[pl.ds(pl.multiple_of(row * D, D), D), pl.ds(pl.multiple_of(col * DH, DH), DH)],
                  w_v.at[j], sem)

    def tiles_wait(lo, n, sem):
        cp(w_v.at[pl.ds(lo, n)], w_v.at[pl.ds(lo, n)], sem).wait()

    def cp_k(it):
        return cp(k_hbm.at[0, pl.ds(2 * it, 2)], k_v.at[it & 1], SEM_KV + (it & 1))

    def cp_v(it):
        return cp(v_hbm.at[0, pl.ds(2 * it, 2)], v_v.at[it & 1], SEM_KV + 2 + (it & 1))

    def cp_rows(src, dst, i, n, sem):
        return cp(src.at[pl.ds(i * n, n), :], dst.at[pl.ds(i * n, n), pl.ds(0, src.shape[1])], sem)

    def wmb_start(it):
        for k in range(2):
            cp_tile(wm_hbm, 0, 2 * D // DH + 2 * it + k, 2 * (it & 1) + k,
                    SEM_WMB + (it & 1)).start()

    def cp_out(i, n):
        return cp(out_v.at[pl.ds(i * E_ROWS, n * E_ROWS), pl.ds(0, D)],
                  out_hbm.at[0, pl.ds(i * E_ROWS, n * E_ROWS), :], SEM_OUT)

    def mrow(k, n):
        m = mod_v[:, k * D:(k + 1) * D]
        return jnp.concatenate([m] * (n // 8), axis=0)

    cp_c().start()
    cp_wr().start()
    for j in range(2):
        cp_wca(j).start()
    cp_x(0).start()
    cp_wqp().start()
    for i in range(1, n_p):
        cp_x(i).start()
    cp_wsa().start()
    cp_k(0).start()
    cp_v(0).start()
    wmb_start(0)

    cp_c().wait()
    cp_wr().wait()
    mod_v[:, WR * D:(WR + 1) * D] = jnp.broadcast_to(wr_v[...].astype(f32).reshape(1, D), (8, D))
    int_min = jnp.iinfo(jnp.int32).min
    top_v[...] = jnp.full(top_v.shape, int_min, jnp.int32)
    acc_v[...] = jnp.zeros(acc_v.shape, f32)
    rp_v[...] = jnp.zeros(rp_v.shape, f32)
    cf = c_v[...].astype(f32)
    sc = jnp.broadcast_to(_r(cf * jax.nn.sigmoid(cf)), (8, D))
    sc_v[...] = jnp.concatenate([sc, sc], axis=0).astype(bf16)
    scb_v[...] = _lane_bcast(sc)

    def wca_body(j, carry):
        cp_wca(j).wait()
        cols = pl.ds(pl.multiple_of(j * 512, 512), 512)
        mj = jnp.dot(sc_v[...], h2_v[D:2 * D, cols], preferred_element_type=f32)
        ca_v[:, cols] = _r(_r(mj[0:8, :]) + 1.0)
        return carry

    lax.fori_loop(0, 2, wca_body, 0)

    def ln1(i):
        rows = pl.ds(pl.multiple_of(i * P_ROWS, P_ROWS), P_ROWS)
        x = x_v[rows, :].astype(f32)
        mu = jnp.sum(x, axis=1, keepdims=True) * (1.0 / D)
        d = x - mu
        var = jnp.sum(d * d, axis=1, keepdims=True) * (1.0 / D)
        n = d * lax.rsqrt(var + EPS)
        h = n * jnp.concatenate([ca_v[...]] * (P_ROWS // 8), axis=0)
        hs = [h[:, k * 128:(k + 1) * 128].astype(bf16) for k in range(D // 128)]
        for k in range(D // 128):
            l_v[k, rows, :] = hs[k]
        return hs

    cp_x(0).wait()
    ln1(0)
    cp_wqp().wait()

    def p_body(i, carry):
        cp_x(i + 1).wait()
        rows = pl.ds(pl.multiple_of(i * P_ROWS, P_ROWS), P_ROWS)
        lhs = [l_v[k, rows, :] for k in range(D // 128)]
        tl = [t[0] for row in zip(*map(_tiles, ln1(i + 1))) for t in row]
        deps = [(P_LO + (P_HI - P_LO) * n / len(tl), t) for n, t in enumerate(tl)]
        qs = _col_dots(lhs, lambda j: out_v[0:D, j * DH:(j + 1) * DH], P_HEADS, _never(i), deps)
        for j in range(P_HEADS):
            f_v[j, rows, :] = qs[j]
        for k in range(4):
            hd = P_HEADS + 4 * i + k
            cp_tile(wq_hbm, 0, hd, hd, SEM_WQ + jnp.where(i < 1, 1, 2)).start()
        return carry

    lax.fori_loop(0, n_p - 1, p_body, 0)
    cp_k(1).start()
    cp_v(1).start()
    wmb_start(1)
    cp_wsa().wait()

    def halves(lhs, w):
        return [lambda h=h: jnp.dot(lhs(h), w(h), preferred_element_type=f32) for h in range(2)]

    def kh(h):
        return slice(h * 512, (h + 1) * 512)

    sa_t = []
    sa = None
    for n in range(2 * P_HEADS):
        j, rows = n // 2, slice(S - P_ROWS + n % 2 * 128, S - P_ROWS + (n % 2 + 1) * 128)
        big = halves(lambda h: jnp.concatenate([l_v[4 * h + k, rows, :] for k in range(4)], axis=1),
                     lambda h: out_v[kh(h), j * DH:(j + 1) * DH])
        acc = None
        for h in range(2):
            d = big[h]()
            acc = d if acc is None else acc + d
            r = 2 * n + h
            if r < 8:
                a, b = halves(lambda h: sc_v[:, kh(h)], lambda h: h2_v[kh(h), r * 128:(r + 1) * 128])
                sa_t.append(_r(a() + b()))
                if r == 7:
                    sa = jnp.concatenate(sa_t, axis=1)
                    sab_v[...] = _lane_bcast(sa[0:8, :])
                    sa = sa.astype(bf16)
            elif P_SQ <= r < P_SQ + P_HEADS:
                t = r - P_SQ
                a, b = halves(lambda h: sa[:, kh(h)], lambda h: out_v[kh(h), t * DH:(t + 1) * DH])
                sq_v[t] = (a() + b())[0:8, :]
        f_v[j, rows, :] = acc
    tiles_wait(P_HEADS, 4, SEM_WQ + 1)

    def m_body(it, carry):
        @pl.when(it == 1)
        def _():
            tiles_wait(P_HEADS + 4, H - P_HEADS - 4, SEM_WQ + 2)

        @pl.when(it == N_QU // U_PER_IT)
        def _():
            tiles_wait(WO, H, SEM_BG)

        @pl.when(jnp.logical_or(it == 6, it == 10))
        def _():
            cp(out_hbm.at[0], out_hbm.at[0], SEM_O).wait()

        @pl.when(jnp.logical_or(it == 8, it == 12))
        def _():
            dst = l_v.at[pl.ds(24 - 2 * it, 8)]
            cp(dst, dst, SEM_O + 1).wait()

        cp_k(it).wait()
        cp_v(it).wait()
        tiles_wait(2 * (it & 1), 2, SEM_WMB + (it & 1))
        slot = it & 1

        def unit(u, js, deps=()):
            g = it * U_PER_IT + u
            is_q = g < N_QU
            blk4 = (g >> 4) * 4
            fb = blk4 + jnp.where(is_q, P_HEADS, -(H - P_HEADS))
            wb = blk4 + P_HEADS
            lb = jnp.where(is_q, 0, 8 - (fb & 8))
            r0 = pl.multiple_of((g & (N_RB - 1)) * U_ROWS, U_ROWS)
            lhs = [l_v[lb + k, pl.ds(r0, U_ROWS), :] for k in range(8)]
            res = _col_dots(lhs, lambda n: w_v[wb + js[n]], len(js), never, deps)
            return [(fb + j, r0, v) for j, v in zip(js, res)]

        def put(tiles):
            for j, r0, v in tiles:
                f_v[j, pl.ds(r0, v.shape[0]), :] = v

        never = _never(it)
        late = unit(0, [0])
        _attention([(f_v.at[2 * it + e], sq_v[2 * it + e], k_v.at[slot, e], v_v.at[slot, e],
                     o_v.at[(2 * it + e) & (HH - 1)]) for e in range(2)])
        mb, steps = _matvec(scb_v, [w_v.at[2 * slot + e] for e in range(2)])
        one = jnp.where(it >> 2 == CB1 - GA, 1.0, 0.0)
        for e in range(2):
            cols = pl.ds(pl.multiple_of(GA * D + (2 * it + e) * 128, 128), 128)
            mod_v[:, cols] = _r(_r(mb[e]) + one)
        hq = jnp.minimum(2 * it + P_HEADS, H - 2)
        sq, more = _matvec(sab_v, [w_v.at[hq + e] for e in range(2)])
        for e in range(2):
            sq_v[hq + e] = sq[e]
        steps = steps + more
        span = (U_PER_IT - MV_U0) * 0.9 / len(steps)
        steps = [(MV_U0 + n * span, t) for n, t in enumerate(steps)]
        for u in range(U_PER_IT):
            tiles = unit(u, list(range(1 if u == 0 else 0, 4)),
                         [(pos - u, t) for pos, t in steps if u <= pos < u + 1])
            if u == 0:
                j, r0, v = tiles[0]
                late.append((j, r0, _pace(v[0:8, :])))
                tiles[0] = (j, r0 + 8, v[8:, :])
            put(tiles)
            if u == U_PER_IT - 2:
                put(late)

        @pl.when(it + 2 < HH)
        def _():
            cp_k(it + 2).start()
            cp_v(it + 2).start()
            wmb_start(it + 2)

        @pl.when(jnp.logical_or(it == 4, it == 8))
        def _():
            for k in range(8):
                cp(o_v.at[2 * it - 8 + k], out_hbm.at[0, :, pl.ds(k * DH, DH)], SEM_O).start()

        @pl.when(jnp.logical_or(it == 6, it == 10))
        def _():
            for k in range(8):
                cp(out_hbm.at[0, :, pl.ds(k * DH, DH)], l_v.at[20 - 2 * it + k], SEM_O + 1).start()

        @pl.when(it < 8)
        def _():
            for k in range(4):
                t = 4 * it + k
                cp_tile(wo_hbm, t >> 3, t & 7, WO + t, SEM_BG).start()

        for n, (src, dst) in enumerate(((wg_hbm, wg_v), (wu_hbm, wu_v), (wd_hbm, wd_v))):
            @pl.when(it >> 1 == n + 4)
            def _():
                cp_rows(src, dst, it & 1, src.shape[0] // 2, SEM_BG + 1 + n).start()

        return carry

    lax.fori_loop(0, HH, m_body, 0)

    cp(wg_v, wg_v, SEM_BG + 1).wait()
    cp(wu_v, wu_v, SEM_BG + 2).wait()
    cp(wd_hbm, wd_v.at[:, pl.ds(0, D)], SEM_BG + 3).wait()

    def router_parts(h2):
        pr = h2 * mrow(WR, h2.shape[0])
        run = [pr[:, 0:128]]
        for b in range(1, D // 128):
            run.append(run[-1] + pr[:, b * 128:(b + 1) * 128])
        return run

    def finish_rows(r0, attn, lo, hi, never=None):
        rows = pl.ds(r0, E_ROWS)
        x2 = _r(x_v[rows, :].astype(f32) + mrow(GA, E_ROWS) * attn)
        if never is None:
            mu = jnp.sum(x2, axis=1, keepdims=True) * (1.0 / D)
            dc = x2 - mu
            var = _r(jnp.sum(dc * dc, axis=1, keepdims=True) * (1.0 / D))
        else:
            mus, vrs = [], []
            for g in range(E_ROWS // 8):
                xg = x2[g * 8:(g + 1) * 8, :]
                sp = xg[:, 0:128]
                for b in range(1, D // 128):
                    sp = sp + xg[:, b * 128:(b + 1) * 128]
                if mus:
                    sp = jnp.where(never, jnp.broadcast_to(mus[-1], (8, 128)), sp)
                mus.append(jnp.sum(sp, axis=1, keepdims=True) * (1.0 / D))
                dg = xg - mus[-1]
                vrs.append(jnp.sum(dg * dg, axis=1, keepdims=True) * (1.0 / D))
            mu = jnp.concatenate(mus, axis=0)
            var = _r(jnp.concatenate(vrs, axis=0))
        den = _r(jnp.sqrt(_r(var + EPS)))
        n = _r(_r(x2 - _r(mu)) * _recip(den))
        h2 = _r(_r(n * mrow(CB1, E_ROWS)) + mrow(SB, E_ROWS))
        x_v[rows, :] = x2.astype(bf16)
        h2_v[rows, 0:D] = h2.astype(bf16)
        of = x2 + _r(mrow(GB, E_ROWS) * h2)
        out_v[rows, 0:D] = of.astype(bf16)
        run = router_parts(h2)
        deps = []
        ot = _tiles(of)
        n_t = len(ot) * len(ot[0])
        for g in range(len(ot)):
            for b in range(len(ot[0])):
                pos = lo + (hi - lo) * (g * len(ot[0]) + b) / n_t
                deps.append((pos, ot[g][b]))
                if b % E_RUN == E_RUN - 1:
                    deps.append((pos, pltpu.bitcast(run[b][g * 8:(g + 1) * 8, :], u32)))
        return run[-1], deps

    def score_rows(r0, rp, valid, m1, m2):
        r = _r(jnp.sum(rp, axis=1, keepdims=True)) + 0.0
        r = jnp.where(r != r, -jnp.inf, r)
        bits = pltpu.bitcast(jnp.broadcast_to(r, (E_ROWS, 128)), jnp.int32)
        bits = jnp.where(bits < 0, bits ^ 0x7FFF0000, bits)
        idx = r0 + lax.broadcasted_iota(jnp.int32, (E_ROWS, 128), 0)
        key = bits | (0xFFFF - idx)
        if valid is not None:
            key = jnp.where(valid, key, int_min)
        for g in range(E_ROWS // 8):
            kg = key[g * 8:(g + 1) * 8, :]
            m2 = jnp.maximum(m2, jnp.minimum(m1, kg))
            m1 = jnp.maximum(m1, kg)
        return m1, m2

    def out_proj(r0, never, deps):
        rows = pl.ds(r0, E_ROWS)
        lhs = [o_v[j, rows, :] for j in range(HH)]
        ds = _col_dots(lhs, lambda j: jnp.concatenate([w_v[WO + 16 + j], w_v[WO + 24 + j]], axis=0),
                       D // 128, never, deps)
        return jnp.concatenate([f_v[j, rows, :] + f_v[8 + j, rows, :] + ds[j]
                                for j in range(D // 128)], axis=1)

    def e_body(c, carry):
        b0 = E_SUB * c

        @pl.when(c >= 2)
        def _():
            cp_out(b0 - E_SUB - 1, 1).start()

        @pl.when(c >= 1)
        def _():
            cp_out(b0 - E_SUB, E_SUB - 1).start()

        never = _never(c)
        m1, m2 = top_v[0], top_v[1]
        keys = []
        for t in range(E_SUB):
            m1, m2 = score_rows((b0 - E_SUB - 1 + t) * E_ROWS, rp_v[t],
                                c >= (2 if t == 0 else 1), m1, m2)
            keys.append(m2)
        top_v[0] = m1
        top_v[1] = m2
        attn = acc_v[...]
        for t in range(E_SUB):
            prev = jnp.maximum(b0 - 1, 0) if t == 0 else b0 + t - 1
            rp_v[t], deps = finish_rows(pl.multiple_of(prev * E_ROWS, E_ROWS), attn,
                                        E_LO0 if t == 0 else E_LO1, E_HI,
                                        None if t == 0 else never)
            deps.append((E_KEY, pltpu.bitcast(keys[t], u32)))
            attn = out_proj(pl.multiple_of((b0 + t) * E_ROWS, E_ROWS), never, deps)
        acc_v[...] = attn
        return carry

    lax.fori_loop(0, n_e, e_body, 0)
    n_b = S // E_ROWS
    cp_out(n_b - E_SUB - 1, E_SUB).start()
    m1, m2 = top_v[0], top_v[1]
    for t in range(E_SUB):
        m1, m2 = score_rows((n_b - E_SUB - 1 + t) * E_ROWS, rp_v[t], None, m1, m2)
    rp_last, _ = finish_rows(S - E_ROWS, acc_v[...], 0.0, 1.0)
    m1, m2 = score_rows(S - E_ROWS, rp_last, None, m1, m2)
    cp_out(n_b - 1, 1).start()

    t1 = jnp.max(m1, axis=0, keepdims=True)
    t2 = jnp.max(jnp.where(m1 == t1, m2, m1), axis=0, keepdims=True)
    i1 = (0xFFFF - t1[0, 0]) & (S - 1)
    i2 = (0xFFFF - t2[0, 0]) & (S - 1)
    g1 = pl.multiple_of(i1 & -GRP, GRP)
    g2 = pl.multiple_of(i2 & -GRP, GRP)

    xs = jnp.concatenate([h2_v[pl.ds(g1, GRP), 0:D], h2_v[pl.ds(g2, GRP), 0:D]], axis=0)

    def act(j):
        fc = slice(j * FC, (j + 1) * FC)
        g = _r(jnp.dot(xs, wg_v[:, fc], preferred_element_type=f32))
        u = _r(jnp.dot(xs, wu_v[:, fc], preferred_element_type=f32))
        return (_r(g * jax.nn.sigmoid(g)) * u).astype(bf16)

    y = None
    a = act(0)
    for j in range(F // FC):
        a_next = act(j + 1) if (j + 1) * FC < F else None
        d = jnp.dot(a, wd_v[j * FC:(j + 1) * FC, 0:D], preferred_element_type=f32)
        y = d if y is None else y + d
        a = a_next
    h2 = xs.astype(f32)
    x2 = jnp.concatenate([x_v[pl.ds(g1, GRP), :], x_v[pl.ds(g2, GRP), :]], axis=0).astype(f32)
    r = _r(jnp.sum(router_parts(h2)[-1], axis=1, keepdims=True))
    upd = _r(_r(y) * _r(jax.nn.sigmoid(r)))
    loc = lax.broadcasted_iota(jnp.int32, (2 * GRP, D), 0)
    row = jnp.where(loc < GRP, g1 + loc, g2 + loc - GRP)
    sel = jnp.logical_or(row == i1, row == i2)
    hb = _r(h2 + jnp.where(sel, upd, 0.0))
    fix_v[...] = (x2 + _r(mrow(GB, 2 * GRP) * hb)).astype(bf16)

    cp(out_v.at[:, pl.ds(0, D)], out_hbm.at[0], SEM_OUT).wait()
    fix1 = cp(fix_v.at[pl.ds(0, GRP), :], out_hbm.at[0, pl.ds(g1, GRP), :], SEM_FIX)
    fix2 = cp(fix_v.at[pl.ds(GRP, GRP), :], out_hbm.at[0, pl.ds(g2, GRP), :], SEM_FIX + 1)
    fix1.start()

    @pl.when(g2 != g1)
    def _():
        fix2.start()
        fix2.wait()

    fix1.wait()


@jax.jit
def pallas_adaLN_cond__mha_block_cached__moe_arch_mod__prompt_kernel(
    A_x: jax.Array,
    A_k_cache: jax.Array,
    A_v_cache: jax.Array,
    A_wq: jax.Array,
    A_wo: jax.Array,
    B_x: jax.Array,
    B_w_r: jax.Array,
    B_w_gate: jax.Array,
    B_w_up: jax.Array,
    B_w_down: jax.Array,
    c: jax.Array,
    w_mod: jax.Array,
):
    del B_x
    vm = pltpu.VMEM
    scratch = [
        vm((S, D), bf16),
        vm((S, D + PAD), bf16),
        vm((S, D + PAD), bf16),
        vm((HH, S, DH), bf16),
        vm((H, S, DH), f32),
        vm((E_ROWS, D), f32),
        vm((2 * H, D, DH), bf16),
        vm((D, F), bf16),
        vm((D, F), bf16),
        vm((F, D + PAD), bf16),
        vm((2, 2, S, DH), bf16),
        vm((2, 2, S, DH), bf16),
        vm((HH, S, DH), bf16),
        vm((1, D), bf16),
        vm((D,), bf16),
        vm((GRP, D), bf16),
        vm((D, 128), f32),
        vm((D, 128), f32),
        vm((8, D), f32),
        vm((H, 8, DH), f32),
        vm((8, 5 * D), f32),
        vm((2, 8, 128), jnp.int32),
        vm((E_SUB, E_ROWS, 128), f32),
        vm((2 * GRP, D), bf16),
        pltpu.SemaphoreType.DMA((N_SEM,)),
    ]
    def once(*refs):
        pl.when(pl.program_id(0) == 0)(lambda: _kernel(*refs))

    return pl.pallas_call(
        once,
        grid=(2,),
        in_specs=[pl.BlockSpec(memory_space=pl.ANY)] * 11,
        out_specs=pl.BlockSpec(memory_space=pl.ANY),
        out_shape=jax.ShapeDtypeStruct(A_x.shape, A_x.dtype),
        scratch_shapes=scratch,
        compiler_params=pltpu.CompilerParams(vmem_limit_bytes=124 * 1024 * 1024,
                                             disable_bounds_checks=True,
                                             disable_semaphore_checks=True),
        name="adaln_mha_moe",
    )(A_x, A_k_cache, A_v_cache, A_wq, A_wo, B_w_r, B_w_gate, B_w_up, B_w_down, c, w_mod)
```

```python
import jax
import jax.numpy as jnp
from jax import lax
import jax.experimental.pallas as pl
import jax.experimental.pallas.tpu as pltpu

S = 2048
D = 1024
H = 32
DH = 128
F = 3584
EPS = 1e-5
HH = H // 2

TQ = 256
KR = 512
P_ROWS = 256
P_HEADS = 4
U_ROWS = 128
N_RB = S // U_ROWS
N_QU = (H - P_HEADS) // 4 * N_RB
N_OU = 2 * 2 * N_RB
U_PER_IT = (N_QU + N_OU) // HH
E_ROWS = 64
E_SUB = 4
PACE = 48
MV_STEP, MV_U0 = 2, 7
GRP = 16
FC = 512
PAD = 128
P0_N, P0_LO, P_LO, P_HI, P_SQ = 3, 0.9, 0.35, 0.97, 10
E_LO0, E_LO1, E_HI, E_KEY, E_RUN = 0.35, 0.45, 0.97, 0.2, 2

Q_SCALE = float(DH) ** -0.5 * 1.4426950408889634

f32 = jnp.float32
bf16 = jnp.bfloat16
u32 = jnp.uint32


def _r(x):
    return x.astype(bf16).astype(f32)


def _recip(x):
    r0 = pl.reciprocal(x, approx=True)
    return r0 * (2.0 - x * r0)


def _pace(t):
    for _ in range(PACE):
        t = jnp.minimum(t, jnp.max(t, axis=1, keepdims=True))
    return t


def _tiles(v):
    u = pltpu.bitcast(v, u32)
    return [[u[a * 8:(a + 1) * 8, b * 128:(b + 1) * 128] for b in range(u.shape[1] // 128)]
            for a in range(u.shape[0] // 8)]


def _col_dots(k_tiles, rhs, n_tiles, never, deps):
    n_r = len(k_tiles) // 4
    n_i = k_tiles[0].shape[0] // GRP
    total = n_tiles * n_r * n_i
    at = {}
    for n, (pos, d) in enumerate(deps):
        at.setdefault((min(int(pos * total), total - 1), n % 4), []).append(d)
    outs = []
    for j in range(n_tiles):
        tl = list(k_tiles)
        for k in range(len(k_tiles)):
            base = (j * n_r + k // 4) * n_i
            if not any((base + i, k % 4) in at for i in range(n_i)):
                continue
            tu = pltpu.bitcast(tl[k], u32)
            parts = []
            for i in range(n_i):
                t = tu[i * 8:(i + 1) * 8, :]
                for d in at.get((base + i, k % 4), ()):
                    t = jnp.where(never, d, t)
                parts.append(t)
            tl[k] = pltpu.bitcast(jnp.concatenate(parts, axis=0), bf16)
        outs.append(jnp.dot(jnp.concatenate(tl, axis=1), rhs(j), preferred_element_type=f32))
    return outs


def _matvec(a_ref, w_refs):
    accs = [None] * len(w_refs)
    steps = []
    for s in range(D // GRP):
        a = a_ref[s * GRP:(s + 1) * GRP, :]
        for n, w in enumerate(w_refs):
            t = w[s * GRP:(s + 1) * GRP, :].astype(f32) * a
            accs[n] = t if accs[n] is None else accs[n] + t
        if s % MV_STEP == MV_STEP - 1:
            steps += [t[0] for acc in accs for t in _tiles(acc)]
    res = [jnp.broadcast_to(jnp.sum(acc, axis=0, keepdims=True), (8, 128)) for acc in accs]
    return res, steps


def _lane_bcast(row):
    return jnp.concatenate([row] * 16, axis=0).T


def _never(i):
    return jnp.full((8, 128), i, jnp.int32) > (1 << 20)


def _attention(heads):
    items = [(refs, c) for refs in heads for c in range(S // TQ)]

    def scores(item):
        (q_ref, bias, k_ref, _, _), c = item
        q = q_ref[c * TQ:(c + 1) * TQ, :] + jnp.concatenate([bias] * (TQ // 8), axis=0)
        q = (q * Q_SCALE).astype(bf16)
        return lax.dot_general(q, k_ref[...], (((1,), (1,)), ((), ())),
                               preferred_element_type=f32)

    def weigh(item, s):
        (_, _, _, v_ref, o_ref), c = item
        m = jnp.max(s, axis=1, keepdims=True)
        o = None
        lp = None
        for r in range(S // KR):
            p = jnp.exp2(s[:, r * KR:(r + 1) * KR] - m)
            ps = [p[:, j * 128:(j + 1) * 128] for j in range(KR // 128)]
            t = ps[0]
            for x in ps[1:]:
                t = t + x
            lp = t if lp is None else lp + t
            ps[-1] = jnp.minimum(ps[-1], t)
            p = jnp.concatenate(ps, axis=1)
            d = jnp.dot(p.astype(bf16), v_ref[r * KR:(r + 1) * KR, :],
                        preferred_element_type=f32)
            o = d if o is None else o + d
        l = jnp.sum(lp, axis=1, keepdims=True)
        o_ref[c * TQ:(c + 1) * TQ, :] = (o * _recip(l)).astype(bf16)

    s = scores(items[0])
    for n, item in enumerate(items):
        s_next = scores(items[n + 1]) if n + 1 < len(items) else None
        weigh(item, s)
        s = s_next


SEM_C, SEM_WR, SEM_WMA, SEM_X, SEM_WQ, SEM_KV, SEM_BG, SEM_OUT, SEM_FIX, SEM_WMB, SEM_O, N_SEM = (
    0, 1, 2, 6, 14, 17, 21, 25, 26, 28, 30, 32)
WO = H
GA, SB, CB1, GB, WR, SPARE = range(6)
MB_LAST = 11


def _kernel(x_hbm, k_hbm, v_hbm, wq_hbm, wo_hbm, wr_hbm, wg_hbm, wu_hbm, wd_hbm, c_hbm,
            wm_hbm, out_hbm,
            x_v, h2_v, out_v, l_v, f_v, acc_v, w_v, wmb_v, wg_v, wu_v, wd_v, k_v, v_v, o_v,
            c_v, wr_v, sc_v, scb_v, sab_v, ca_v, sq_v, mod_v, top_v, rp_v, fix_v, sems):
    n_p = S // P_ROWS
    n_e = S // (E_SUB * E_ROWS)
    pq = P_HEADS * DH

    def cp(src, dst, sem):
        return pltpu.make_async_copy(src, dst, sems.at[sem])

    def cp_c():
        return cp(c_hbm, c_v, SEM_C)

    def cp_wr():
        return cp(wr_hbm, wr_v, SEM_WR)

    def cp_wca(j):
        return cp(wm_hbm.at[:, pl.ds(D + j * 512, 512)],
                  h2_v.at[pl.ds(D, D), pl.ds(j * 512, 512)], SEM_WMA + j)

    def cp_wsa():
        return cp(wm_hbm.at[:, pl.ds(0, D)], h2_v.at[pl.ds(0, D), pl.ds(0, D)], SEM_WMA + 2)

    def cp_x(i):
        return cp(x_hbm.at[0, pl.ds(i * P_ROWS, P_ROWS), :], x_v.at[pl.ds(i * P_ROWS, P_ROWS), :],
                  SEM_X + i)

    def cp_wqp(j):
        cols = (pl.ds(0, P0_N * DH), pl.ds(P0_N * DH, pq - P0_N * DH))[j]
        return cp(wq_hbm.at[:, cols], out_v.at[pl.ds(0, D), cols], (SEM_WQ, SEM_WMA + 3)[j])

    def cp_tile(src, row, col, j, sem):
        return cp(src.at[pl.ds(pl.multiple_of(row * D, D), D), pl.ds(pl.multiple_of(col * DH, DH), DH)],
                  w_v.at[j], sem)

    def tiles_wait(lo, n, sem):
        cp(w_v.at[pl.ds(lo, n)], w_v.at[pl.ds(lo, n)], sem).wait()

    def cp_k(it):
        return cp(k_hbm.at[0, pl.ds(2 * it, 2)], k_v.at[it & 1], SEM_KV + (it & 1))

    def cp_v(it):
        return cp(v_hbm.at[0, pl.ds(2 * it, 2)], v_v.at[it & 1], SEM_KV + 2 + (it & 1))

    def cp_rows(src, dst, i, n, sem):
        return cp(src.at[pl.ds(i * n, n), :], dst.at[pl.ds(i * n, n), pl.ds(0, src.shape[1])], sem)

    def wmb_tile(it, k):
        return jnp.minimum(3 * (it - 1) + k, 4 * D // DH - 1)

    def wmb_start(it):
        for k in range(3):
            cols = pl.ds(pl.multiple_of(2 * D + wmb_tile(it, k) * DH, DH), DH)
            cp(wm_hbm.at[:, cols], wmb_v.at[it & 1, k], SEM_WMB + (it & 1)).start()

    def cp_out(i, n):
        return cp(out_v.at[pl.ds(i * E_ROWS, n * E_ROWS), pl.ds(0, D)],
                  out_hbm.at[0, pl.ds(i * E_ROWS, n * E_ROWS), :], SEM_OUT)

    def mrow(k, n):
        m = mod_v[:, k * D:(k + 1) * D]
        return jnp.concatenate([m] * (n // 8), axis=0)

    cp_c().start()
    cp_wr().start()
    for j in range(2):
        cp_wca(j).start()
    cp_x(0).start()
    cp_wqp(0).start()
    cp_wqp(1).start()
    for i in range(1, n_p):
        cp_x(i).start()
    cp_wsa().start()
    cp_k(0).start()
    cp_v(0).start()

    cp_c().wait()
    cp_wr().wait()
    mod_v[:, WR * D:(WR + 1) * D] = jnp.broadcast_to(wr_v[...].astype(f32).reshape(1, D), (8, D))
    int_min = jnp.iinfo(jnp.int32).min
    top_v[...] = jnp.full(top_v.shape, int_min, jnp.int32)
    acc_v[...] = jnp.zeros(acc_v.shape, f32)
    rp_v[...] = jnp.zeros(rp_v.shape, f32)
    wmb_v[0] = jnp.zeros(wmb_v.shape[1:], bf16)
    cf = c_v[...].astype(f32)
    sc = jnp.broadcast_to(_r(cf * jax.nn.sigmoid(cf)), (8, D))
    sc_v[...] = jnp.concatenate([sc, sc], axis=0).astype(bf16)
    scb_v[...] = _lane_bcast(sc)

    def wca_body(j, carry):
        cp_wca(j).wait()
        cols = pl.ds(pl.multiple_of(j * 512, 512), 512)
        mj = jnp.dot(sc_v[...], h2_v[D:2 * D, cols], preferred_element_type=f32)
        ca_v[:, cols] = _r(_r(mj[0:8, :]) + 1.0)
        return carry

    lax.fori_loop(0, 2, wca_body, 0)

    def ln1(i):
        rows = pl.ds(pl.multiple_of(i * P_ROWS, P_ROWS), P_ROWS)
        x = x_v[rows, :].astype(f32)
        mu = jnp.sum(x, axis=1, keepdims=True) * (1.0 / D)
        d = x - mu
        var = jnp.sum(d * d, axis=1, keepdims=True) * (1.0 / D)
        n = d * lax.rsqrt(var + EPS)
        h = n * jnp.concatenate([ca_v[...]] * (P_ROWS // 8), axis=0)
        hs = [h[:, k * 128:(k + 1) * 128].astype(bf16) for k in range(D // 128)]
        for k in range(D // 128):
            l_v[k, rows, :] = hs[k]
        return hs

    cp_x(0).wait()
    ln1(0)

    def p_step(i, js, lo):
        rows = pl.ds(pl.multiple_of(i * P_ROWS, P_ROWS), P_ROWS)
        lhs = [l_v[k, rows, :] for k in range(D // 128)]
        deps = []
        if lo is not None:
            tl = [t[0] for row in zip(*map(_tiles, ln1(i + 1))) for t in row]
            deps = [(lo + (P_HI - lo) * n / len(tl), t) for n, t in enumerate(tl)]
        qs = _col_dots(lhs, lambda n: out_v[0:D, js[n] * DH:(js[n] + 1) * DH], len(js),
                       _never(i + pl.program_id(0)), deps)
        for j, q in zip(js, qs):
            f_v[j, rows, :] = q
        if lo is not None:
            for k in range(4):
                hd = P_HEADS + 4 * i + k
                cp_tile(wq_hbm, 0, hd, hd, SEM_WQ + jnp.where(i < 1, 1, 2)).start()

    cp_wqp(0).wait()
    p_step(0, list(range(P0_N)), None)
    cp_wqp(1).wait()
    cp_x(1).wait()
    p_step(0, list(range(P0_N, P_HEADS)), P0_LO)

    def p_body(i, carry):
        cp_x(i + 1).wait()
        p_step(i, list(range(P_HEADS)), P_LO)
        return carry

    lax.fori_loop(1, n_p - 1, p_body, 0)
    cp_k(1).start()
    cp_v(1).start()
    wmb_start(1)
    cp_wsa().wait()

    def halves(lhs, w):
        return [lambda h=h: jnp.dot(lhs(h), w(h), preferred_element_type=f32) for h in range(2)]

    def kh(h):
        return slice(h * 512, (h + 1) * 512)

    sa_t = []
    sa = None
    for n in range(2 * P_HEADS):
        j, rows = n // 2, slice(S - P_ROWS + n % 2 * 128, S - P_ROWS + (n % 2 + 1) * 128)
        big = halves(lambda h: jnp.concatenate([l_v[4 * h + k, rows, :] for k in range(4)], axis=1),
                     lambda h: out_v[kh(h), j * DH:(j + 1) * DH])
        acc = None
        for h in range(2):
            d = big[h]()
            acc = d if acc is None else acc + d
            r = 2 * n + h
            if r < 8:
                a, b = halves(lambda h: sc_v[:, kh(h)], lambda h: h2_v[kh(h), r * 128:(r + 1) * 128])
                sa_t.append(_r(a() + b()))
                if r == 7:
                    sa = jnp.concatenate(sa_t, axis=1)
                    sab_v[...] = _lane_bcast(sa[0:8, :])
                    sa = sa.astype(bf16)
            elif P_SQ <= r < P_SQ + P_HEADS:
                t = r - P_SQ
                a, b = halves(lambda h: sa[:, kh(h)], lambda h: out_v[kh(h), t * DH:(t + 1) * DH])
                sq_v[t] = (a() + b())[0:8, :]
        f_v[j, rows, :] = acc
    tiles_wait(P_HEADS, 4, SEM_WQ + 1)

    def m_body(it, carry):
        @pl.when(it == 1)
        def _():
            tiles_wait(P_HEADS + 4, H - P_HEADS - 4, SEM_WQ + 2)

        @pl.when(it == N_QU // U_PER_IT)
        def _():
            tiles_wait(WO, H, SEM_BG)

        @pl.when(jnp.logical_or(it == 6, it == 10))
        def _():
            cp(out_hbm.at[0], out_hbm.at[0], SEM_O).wait()

        @pl.when(jnp.logical_or(it == 8, it == 12))
        def _():
            dst = l_v.at[pl.ds(24 - 2 * it, 8)]
            cp(dst, dst, SEM_O + 1).wait()

        cp_k(it).wait()
        cp_v(it).wait()
        slot = it & 1
        live = jnp.logical_and(it >= 1, it <= MB_LAST)

        @pl.when(live)
        def _():
            cp(wmb_v.at[slot], wmb_v.at[slot], SEM_WMB + slot).wait()

        def unit(u, js, deps=()):
            g = it * U_PER_IT + u
            is_q = g < N_QU
            blk4 = (g >> 4) * 4
            fb = blk4 + jnp.where(is_q, P_HEADS, -(H - P_HEADS))
            wb = blk4 + P_HEADS
            lb = jnp.where(is_q, 0, 8 - (fb & 8))
            r0 = pl.multiple_of((g & (N_RB - 1)) * U_ROWS, U_ROWS)
            lhs = [l_v[lb + k, pl.ds(r0, U_ROWS), :] for k in range(8)]
            res = _col_dots(lhs, lambda n: w_v[wb + js[n]], len(js), never, deps)
            return [(fb + j, r0, v) for j, v in zip(js, res)]

        def put(tiles):
            for j, r0, v in tiles:
                f_v[j, pl.ds(r0, v.shape[0]), :] = v

        never = _never(it)
        late = unit(0, [0])
        _attention([(f_v.at[2 * it + e], sq_v[2 * it + e], k_v.at[slot, e], v_v.at[slot, e],
                     o_v.at[(2 * it + e) & (HH - 1)]) for e in range(2)])
        mb, steps = _matvec(scb_v, [wmb_v.at[slot, k] for k in range(3)])
        for k in range(3):
            t = jnp.where(live, wmb_tile(it, k), SPARE * D // DH)
            one = jnp.where(t >> 3 == CB1, 1.0, 0.0)
            mod_v[:, pl.ds(pl.multiple_of(t * DH, DH), DH)] = _r(_r(mb[k]) + one)
        hq = jnp.minimum(2 * it + P_HEADS, H - 2)
        sq, more = _matvec(sab_v, [w_v.at[hq + e] for e in range(2)])
        for e in range(2):
            sq_v[hq + e] = sq[e]
        steps = steps + more
        span = (U_PER_IT - MV_U0) * 0.9 / len(steps)
        steps = [(MV_U0 + n * span, t) for n, t in enumerate(steps)]
        for u in range(U_PER_IT):
            tiles = unit(u, list(range(1 if u == 0 else 0, 4)),
                         [(pos - u, t) for pos, t in steps if u <= pos < u + 1])
            if u == 0:
                j, r0, v = tiles[0]
                late.append((j, r0, _pace(v[0:8, :])))
                tiles[0] = (j, r0 + 8, v[8:, :])
            put(tiles)
            if u == U_PER_IT - 2:
                put(late)

        @pl.when(it + 2 < HH)
        def _():
            cp_k(it + 2).start()
            cp_v(it + 2).start()

        @pl.when(it + 2 <= MB_LAST)
        def _():
            wmb_start(it + 2)

        @pl.when(jnp.logical_or(it == 4, it == 8))
        def _():
            for k in range(8):
                cp(o_v.at[2 * it - 8 + k], out_hbm.at[0, :, pl.ds(k * DH, DH)], SEM_O).start()

        @pl.when(jnp.logical_or(it == 6, it == 10))
        def _():
            for k in range(8):
                cp(out_hbm.at[0, :, pl.ds(k * DH, DH)], l_v.at[20 - 2 * it + k], SEM_O + 1).start()

        @pl.when(it < 8)
        def _():
            for k in range(4):
                t = 4 * it + k
                cp_tile(wo_hbm, t >> 3, t & 7, WO + t, SEM_BG).start()

        for n, (src, dst) in enumerate(((wg_hbm, wg_v), (wu_hbm, wu_v), (wd_hbm, wd_v))):
            @pl.when(it >> 1 == n + 4)
            def _():
                cp_rows(src, dst, it & 1, src.shape[0] // 2, SEM_BG + 1 + n).start()

        return carry

    lax.fori_loop(0, HH, m_body, 0)

    cp(wg_v, wg_v, SEM_BG + 1).wait()
    cp(wu_v, wu_v, SEM_BG + 2).wait()
    cp(wd_hbm, wd_v.at[:, pl.ds(0, D)], SEM_BG + 3).wait()

    def router_parts(h2):
        pr = h2 * mrow(WR, h2.shape[0])
        run = [pr[:, 0:128]]
        for b in range(1, D // 128):
            run.append(run[-1] + pr[:, b * 128:(b + 1) * 128])
        return run

    def finish_rows(r0, attn, lo, hi, never=None):
        rows = pl.ds(r0, E_ROWS)
        x2 = _r(x_v[rows, :].astype(f32) + mrow(GA, E_ROWS) * attn)
        if never is None:
            mu = jnp.sum(x2, axis=1, keepdims=True) * (1.0 / D)
            dc = x2 - mu
            var = _r(jnp.sum(dc * dc, axis=1, keepdims=True) * (1.0 / D))
        else:
            mus, vrs = [], []
            for g in range(E_ROWS // 8):
                xg = x2[g * 8:(g + 1) * 8, :]
                sp = xg[:, 0:128]
                for b in range(1, D // 128):
                    sp = sp + xg[:, b * 128:(b + 1) * 128]
                if mus:
                    sp = jnp.where(never, jnp.broadcast_to(mus[-1], (8, 128)), sp)
                mus.append(jnp.sum(sp, axis=1, keepdims=True) * (1.0 / D))
                dg = xg - mus[-1]
                vrs.append(jnp.sum(dg * dg, axis=1, keepdims=True) * (1.0 / D))
            mu = jnp.concatenate(mus, axis=0)
            var = _r(jnp.concatenate(vrs, axis=0))
        den = _r(jnp.sqrt(_r(var + EPS)))
        n = _r(_r(x2 - _r(mu)) * _recip(den))
        h2 = _r(_r(n * mrow(CB1, E_ROWS)) + mrow(SB, E_ROWS))
        x_v[rows, :] = x2.astype(bf16)
        h2_v[rows, 0:D] = h2.astype(bf16)
        of = x2 + _r(mrow(GB, E_ROWS) * h2)
        out_v[rows, 0:D] = of.astype(bf16)
        run = router_parts(h2)
        deps = []
        ot = _tiles(of)
        n_t = len(ot) * len(ot[0])
        for g in range(len(ot)):
            for b in range(len(ot[0])):
                pos = lo + (hi - lo) * (g * len(ot[0]) + b) / n_t
                deps.append((pos, ot[g][b]))
                if b % E_RUN == E_RUN - 1:
                    deps.append((pos, pltpu.bitcast(run[b][g * 8:(g + 1) * 8, :], u32)))
        return run[-1], deps

    def score_rows(r0, rp, valid, m1, m2):
        r = _r(jnp.sum(rp, axis=1, keepdims=True)) + 0.0
        r = jnp.where(r != r, -jnp.inf, r)
        bits = pltpu.bitcast(jnp.broadcast_to(r, (E_ROWS, 128)), jnp.int32)
        bits = jnp.where(bits < 0, bits ^ 0x7FFF0000, bits)
        idx = r0 + lax.broadcasted_iota(jnp.int32, (E_ROWS, 128), 0)
        key = bits | (0xFFFF - idx)
        if valid is not None:
            key = jnp.where(valid, key, int_min)
        for g in range(E_ROWS // 8):
            kg = key[g * 8:(g + 1) * 8, :]
            m2 = jnp.maximum(m2, jnp.minimum(m1, kg))
            m1 = jnp.maximum(m1, kg)
        return m1, m2

    def out_proj(r0, never, deps):
        rows = pl.ds(r0, E_ROWS)
        lhs = [o_v[j, rows, :] for j in range(HH)]
        ds = _col_dots(lhs, lambda j: jnp.concatenate([w_v[WO + 16 + j], w_v[WO + 24 + j]], axis=0),
                       D // 128, never, deps)
        return jnp.concatenate([f_v[j, rows, :] + f_v[8 + j, rows, :] + ds[j]
                                for j in range(D // 128)], axis=1)

    def e_body(c, carry):
        b0 = E_SUB * c

        @pl.when(c >= 2)
        def _():
            cp_out(b0 - E_SUB - 1, 1).start()

        @pl.when(c >= 1)
        def _():
            cp_out(b0 - E_SUB, E_SUB - 1).start()

        never = _never(c)
        m1, m2 = top_v[0], top_v[1]
        keys = []
        for t in range(E_SUB):
            m1, m2 = score_rows((b0 - E_SUB - 1 + t) * E_ROWS, rp_v[t],
                                c >= (2 if t == 0 else 1), m1, m2)
            keys.append(m2)
        top_v[0] = m1
        top_v[1] = m2
        attn = acc_v[...]
        for t in range(E_SUB):
            prev = jnp.maximum(b0 - 1, 0) if t == 0 else b0 + t - 1
            rp_v[t], deps = finish_rows(pl.multiple_of(prev * E_ROWS, E_ROWS), attn,
                                        E_LO0 if t == 0 else E_LO1, E_HI,
                                        None if t == 0 else never)
            deps.append((E_KEY, pltpu.bitcast(keys[t], u32)))
            attn = out_proj(pl.multiple_of((b0 + t) * E_ROWS, E_ROWS), never, deps)
        acc_v[...] = attn
        return carry

    lax.fori_loop(0, n_e, e_body, 0)
    n_b = S // E_ROWS
    cp_out(n_b - E_SUB - 1, E_SUB).start()
    m1, m2 = top_v[0], top_v[1]
    for t in range(E_SUB):
        m1, m2 = score_rows((n_b - E_SUB - 1 + t) * E_ROWS, rp_v[t], None, m1, m2)
    rp_last, _ = finish_rows(S - E_ROWS, acc_v[...], 0.0, 1.0)
    m1, m2 = score_rows(S - E_ROWS, rp_last, None, m1, m2)
    cp_out(n_b - 1, 1).start()

    t1 = jnp.max(m1, axis=0, keepdims=True)
    t2 = jnp.max(jnp.where(m1 == t1, m2, m1), axis=0, keepdims=True)
    i1 = (0xFFFF - t1[0, 0]) & (S - 1)
    i2 = (0xFFFF - t2[0, 0]) & (S - 1)
    g1 = pl.multiple_of(i1 & -GRP, GRP)
    g2 = pl.multiple_of(i2 & -GRP, GRP)

    xs = jnp.concatenate([h2_v[pl.ds(g1, GRP), 0:D], h2_v[pl.ds(g2, GRP), 0:D]], axis=0)

    def act(j):
        fc = slice(j * FC, (j + 1) * FC)
        g = _r(jnp.dot(xs, wg_v[:, fc], preferred_element_type=f32))
        u = _r(jnp.dot(xs, wu_v[:, fc], preferred_element_type=f32))
        return (_r(g * jax.nn.sigmoid(g)) * u).astype(bf16)

    y = None
    a = act(0)
    for j in range(F // FC):
        a_next = act(j + 1) if (j + 1) * FC < F else None
        d = jnp.dot(a, wd_v[j * FC:(j + 1) * FC, 0:D], preferred_element_type=f32)
        y = d if y is None else y + d
        a = a_next
    h2 = xs.astype(f32)
    x2 = jnp.concatenate([x_v[pl.ds(g1, GRP), :], x_v[pl.ds(g2, GRP), :]], axis=0).astype(f32)
    r = _r(jnp.sum(router_parts(h2)[-1], axis=1, keepdims=True))
    upd = _r(_r(y) * _r(jax.nn.sigmoid(r)))
    loc = lax.broadcasted_iota(jnp.int32, (2 * GRP, D), 0)
    row = jnp.where(loc < GRP, g1 + loc, g2 + loc - GRP)
    sel = jnp.logical_or(row == i1, row == i2)
    hb = _r(h2 + jnp.where(sel, upd, 0.0))
    fix_v[...] = (x2 + _r(mrow(GB, 2 * GRP) * hb)).astype(bf16)

    cp(out_v.at[:, pl.ds(0, D)], out_hbm.at[0], SEM_OUT).wait()
    fix1 = cp(fix_v.at[pl.ds(0, GRP), :], out_hbm.at[0, pl.ds(g1, GRP), :], SEM_FIX)
    fix2 = cp(fix_v.at[pl.ds(GRP, GRP), :], out_hbm.at[0, pl.ds(g2, GRP), :], SEM_FIX + 1)
    fix1.start()

    @pl.when(g2 != g1)
    def _():
        fix2.start()
        fix2.wait()

    fix1.wait()


@jax.jit
def pallas_adaLN_cond__mha_block_cached__moe_arch_mod__prompt_kernel(
    A_x: jax.Array,
    A_k_cache: jax.Array,
    A_v_cache: jax.Array,
    A_wq: jax.Array,
    A_wo: jax.Array,
    B_x: jax.Array,
    B_w_r: jax.Array,
    B_w_gate: jax.Array,
    B_w_up: jax.Array,
    B_w_down: jax.Array,
    c: jax.Array,
    w_mod: jax.Array,
):
    del B_x
    vm = pltpu.VMEM
    scratch = [
        vm((S, D), bf16),
        vm((S, D + PAD), bf16),
        vm((S, D + PAD), bf16),
        vm((HH, S, DH), bf16),
        vm((H, S, DH), f32),
        vm((E_ROWS, D), f32),
        vm((2 * H, D, DH), bf16),
        vm((2, 3, D, DH), bf16),
        vm((D, F), bf16),
        vm((D, F), bf16),
        vm((F, D + PAD), bf16),
        vm((2, 2, S, DH), bf16),
        vm((2, 2, S, DH), bf16),
        vm((HH, S, DH), bf16),
        vm((1, D), bf16),
        vm((D,), bf16),
        vm((GRP, D), bf16),
        vm((D, 128), f32),
        vm((D, 128), f32),
        vm((8, D), f32),
        vm((H, 8, DH), f32),
        vm((8, 5 * D + DH), f32),
        vm((2, 8, 128), jnp.int32),
        vm((E_SUB, E_ROWS, 128), f32),
        vm((2 * GRP, D), bf16),
        pltpu.SemaphoreType.DMA((N_SEM,)),
    ]
    def once(*refs):
        pl.when(pl.program_id(0) == 0)(lambda: _kernel(*refs))

    return pl.pallas_call(
        once,
        grid=(2,),
        in_specs=[pl.BlockSpec(memory_space=pl.ANY)] * 11,
        out_specs=pl.BlockSpec(memory_space=pl.ANY),
        out_shape=jax.ShapeDtypeStruct(A_x.shape, A_x.dtype),
        scratch_shapes=scratch,
        compiler_params=pltpu.CompilerParams(vmem_limit_bytes=124 * 1024 * 1024,
                                             disable_bounds_checks=True,
                                             disable_semaphore_checks=True),
        name="adaln_mha_moe",
    )(A_x, A_k_cache, A_v_cache, A_wq, A_wo, B_w_r, B_w_gate, B_w_up, B_w_down, c, w_mod)
```

```python
import jax
import jax.numpy as jnp
from jax import lax
import jax.experimental.pallas as pl
import jax.experimental.pallas.tpu as pltpu

S = 2048
D = 1024
H = 32
DH = 128
F = 3584
EPS = 1e-5
HH = H // 2

TQ = 256
KR = 512
P_ROWS = 256
P_HEADS = 4
U_ROWS = 128
N_RB = S // U_ROWS
N_QU = (H - P_HEADS) // 4 * N_RB
N_OU = 2 * 2 * N_RB
U_PER_IT = (N_QU + N_OU) // HH
E_ROWS = 64
E_SUB = 4
PACE = 48
MV_STEP, MV_U0 = 2, 7
GRP = 16
FC = 512
PAD = 128
P0_N, P0_LO, P_LO, P_HI, P_SQ = 3, 0.9, 0.35, 0.97, 10
E_LO0, E_LO1, E_HI, E_KEY, E_RUN = 0.35, 0.45, 0.97, 0.2, 2

Q_SCALE = float(DH) ** -0.5 * 1.4426950408889634

f32 = jnp.float32
bf16 = jnp.bfloat16
u32 = jnp.uint32


def _r(x):
    return x.astype(bf16).astype(f32)


def _recip(x):
    r0 = pl.reciprocal(x, approx=True)
    return r0 * (2.0 - x * r0)


def _pace(t):
    for _ in range(PACE):
        t = jnp.minimum(t, jnp.max(t, axis=1, keepdims=True))
    return t


def _tiles(v):
    u = pltpu.bitcast(v, u32)
    return [[u[a * 8:(a + 1) * 8, b * 128:(b + 1) * 128] for b in range(u.shape[1] // 128)]
            for a in range(u.shape[0] // 8)]


def _col_dots(k_tiles, rhs, n_tiles, never, deps):
    n_r = len(k_tiles) // 4
    n_i = k_tiles[0].shape[0] // GRP
    total = n_tiles * n_r * n_i
    at = {}
    for n, (pos, d) in enumerate(deps):
        at.setdefault((min(int(pos * total), total - 1), n % 4), []).append(d)
    outs = []
    for j in range(n_tiles):
        tl = list(k_tiles)
        for k in range(len(k_tiles)):
            base = (j * n_r + k // 4) * n_i
            if not any((base + i, k % 4) in at for i in range(n_i)):
                continue
            tu = pltpu.bitcast(tl[k], u32)
            parts = []
            for i in range(n_i):
                t = tu[i * 8:(i + 1) * 8, :]
                for d in at.get((base + i, k % 4), ()):
                    t = jnp.where(never, d, t)
                parts.append(t)
            tl[k] = pltpu.bitcast(jnp.concatenate(parts, axis=0), bf16)
        outs.append(jnp.dot(jnp.concatenate(tl, axis=1), rhs(j), preferred_element_type=f32))
    return outs


def _matvec(a_ref, w_refs):
    accs = [None] * len(w_refs)
    steps = []
    for s in range(D // GRP):
        a = a_ref[s * GRP:(s + 1) * GRP, :]
        for n, w in enumerate(w_refs):
            t = w[s * GRP:(s + 1) * GRP, :].astype(f32) * a
            accs[n] = t if accs[n] is None else accs[n] + t
        if s % MV_STEP == MV_STEP - 1:
            steps += [t[0] for acc in accs for t in _tiles(acc)]
    res = [jnp.broadcast_to(jnp.sum(acc, axis=0, keepdims=True), (8, 128)) for acc in accs]
    return res, steps


def _lane_bcast(row):
    return jnp.concatenate([row] * 16, axis=0).T


def _never(i):
    return jnp.full((8, 128), i, jnp.int32) > (1 << 20)


def _attention(heads):
    items = [(refs, c) for refs in heads for c in range(S // TQ)]

    def scores(item):
        (q_ref, bias, k_ref, _, _), c = item
        q = q_ref[c * TQ:(c + 1) * TQ, :] + jnp.concatenate([bias] * (TQ // 8), axis=0)
        q = (q * Q_SCALE).astype(bf16)
        return lax.dot_general(q, k_ref[...], (((1,), (1,)), ((), ())),
                               preferred_element_type=f32)

    def weigh(item, s):
        (_, _, _, v_ref, o_ref), c = item
        m = jnp.max(s, axis=1, keepdims=True)
        o = None
        lp = None
        for r in range(S // KR):
            p = jnp.exp2(s[:, r * KR:(r + 1) * KR] - m)
            ps = [p[:, j * 128:(j + 1) * 128] for j in range(KR // 128)]
            t = ps[0]
            for x in ps[1:]:
                t = t + x
            lp = t if lp is None else lp + t
            ps[-1] = jnp.minimum(ps[-1], t)
            p = jnp.concatenate(ps, axis=1)
            d = jnp.dot(p.astype(bf16), v_ref[r * KR:(r + 1) * KR, :],
                        preferred_element_type=f32)
            o = d if o is None else o + d
        l = jnp.sum(lp, axis=1, keepdims=True)
        o_ref[c * TQ:(c + 1) * TQ, :] = (o * _recip(l)).astype(bf16)

    s = scores(items[0])
    for n, item in enumerate(items):
        s_next = scores(items[n + 1]) if n + 1 < len(items) else None
        weigh(item, s)
        s = s_next


SEM_C, SEM_WR, SEM_WMA, SEM_X, SEM_WQ, SEM_KV, SEM_BG, SEM_OUT, SEM_FIX, SEM_WMB, SEM_O, N_SEM = (
    0, 1, 2, 6, 14, 17, 21, 25, 26, 28, 30, 32)
WO = H
GA, SB, CB1, GB, WR, SPARE = range(6)
MB_LAST = 11


def _kernel(x_hbm, k_hbm, v_hbm, wq_hbm, wo_hbm, wr_hbm, wg_hbm, wu_hbm, wd_hbm, c_hbm,
            wm_hbm, out_hbm,
            x_v, h2_v, out_v, l_v, f_v, acc_v, w_v, wmb_v, wg_v, wu_v, wd_v, k_v, v_v, o_v,
            c_v, wr_v, sc_v, scb_v, sab_v, ca_v, sq_v, mod_v, top_v, rp_v, fix_v, sems):
    n_p = S // P_ROWS
    n_e = S // (E_SUB * E_ROWS)
    pq = P_HEADS * DH

    def cp(src, dst, sem):
        return pltpu.make_async_copy(src, dst, sems.at[sem])

    def cp_c():
        return cp(c_hbm, c_v, SEM_C)

    def cp_wr():
        return cp(wr_hbm, wr_v, SEM_WR)

    def cp_wca(j):
        return cp(wm_hbm.at[:, pl.ds(D + j * 512, 512)],
                  h2_v.at[pl.ds(D, D), pl.ds(j * 512, 512)], SEM_WMA + j)

    def cp_wsa():
        return cp(wm_hbm.at[:, pl.ds(0, D)], h2_v.at[pl.ds(0, D), pl.ds(0, D)], SEM_WMA + 2)

    def cp_x(i):
        return cp(x_hbm.at[0, pl.ds(i * P_ROWS, P_ROWS), :], x_v.at[pl.ds(i * P_ROWS, P_ROWS), :],
                  SEM_X + i)

    def cp_wqp(j):
        cols = (pl.ds(0, P0_N * DH), pl.ds(P0_N * DH, pq - P0_N * DH))[j]
        return cp(wq_hbm.at[:, cols], out_v.at[pl.ds(0, D), cols], (SEM_WQ, SEM_WMA + 3)[j])

    def cp_tile(src, row, col, j, sem):
        return cp(src.at[pl.ds(pl.multiple_of(row * D, D), D), pl.ds(pl.multiple_of(col * DH, DH), DH)],
                  w_v.at[j], sem)

    def tiles(lo, n, sem):
        return cp(w_v.at[pl.ds(lo, n)], w_v.at[pl.ds(lo, n)], sem)

    def cp_k(it):
        return cp(k_hbm.at[0, pl.ds(2 * it, 2)], k_v.at[it & 1], SEM_KV + (it & 1))

    def cp_v(it):
        return cp(v_hbm.at[0, pl.ds(2 * it, 2)], v_v.at[it & 1], SEM_KV + 2 + (it & 1))

    def cp_rows(src, dst, i, n, sem):
        return cp(src.at[pl.ds(i * n, n), :], dst.at[pl.ds(i * n, n), pl.ds(0, src.shape[1])], sem)

    def wmb_tile(it, k):
        return jnp.minimum(3 * (it - 1) + k, 4 * D // DH - 1)

    def wmb_start(it):
        for k in range(3):
            cols = pl.ds(pl.multiple_of(2 * D + wmb_tile(it, k) * DH, DH), DH)
            cp(wm_hbm.at[:, cols], wmb_v.at[it & 1, k], SEM_WMB + (it & 1)).start()

    def cp_out(i, n):
        return cp(out_v.at[pl.ds(i * E_ROWS, n * E_ROWS), pl.ds(0, D)],
                  out_hbm.at[0, pl.ds(i * E_ROWS, n * E_ROWS), :], SEM_OUT)

    def mrow(k, n):
        m = mod_v[:, k * D:(k + 1) * D]
        return jnp.concatenate([m] * (n // 8), axis=0)

    cp_c().start()
    cp_wr().start()
    for j in range(2):
        cp_wca(j).start()
    cp_x(0).start()
    cp_wqp(0).start()
    cp_wqp(1).start()
    for i in range(1, n_p):
        cp_x(i).start()
    cp_wsa().start()
    cp_k(0).start()
    cp_v(0).start()

    cp_c().wait()
    cp_wr().wait()
    mod_v[:, WR * D:(WR + 1) * D] = jnp.broadcast_to(wr_v[...].astype(f32).reshape(1, D), (8, D))
    int_min = jnp.iinfo(jnp.int32).min
    top_v[...] = jnp.full(top_v.shape, int_min, jnp.int32)
    acc_v[...] = jnp.zeros(acc_v.shape, f32)
    rp_v[...] = jnp.zeros(rp_v.shape, f32)
    wmb_v[0] = jnp.zeros(wmb_v.shape[1:], bf16)
    cf = c_v[...].astype(f32)
    sc = jnp.broadcast_to(_r(cf * jax.nn.sigmoid(cf)), (8, D))
    sc_v[...] = jnp.concatenate([sc, sc], axis=0).astype(bf16)
    scb_v[...] = _lane_bcast(sc)

    def wca_body(j, carry):
        cp_wca(j).wait()
        cols = pl.ds(pl.multiple_of(j * 512, 512), 512)
        mj = jnp.dot(sc_v[...], h2_v[D:2 * D, cols], preferred_element_type=f32)
        ca_v[:, cols] = _r(_r(mj[0:8, :]) + 1.0)
        return carry

    lax.fori_loop(0, 2, wca_body, 0)

    def ln1(i):
        rows = pl.ds(pl.multiple_of(i * P_ROWS, P_ROWS), P_ROWS)
        x = x_v[rows, :].astype(f32)
        mu = jnp.sum(x, axis=1, keepdims=True) * (1.0 / D)
        d = x - mu
        var = jnp.sum(d * d, axis=1, keepdims=True) * (1.0 / D)
        n = d * lax.rsqrt(var + EPS)
        h = n * jnp.concatenate([ca_v[...]] * (P_ROWS // 8), axis=0)
        hs = [h[:, k * 128:(k + 1) * 128].astype(bf16) for k in range(D // 128)]
        for k in range(D // 128):
            l_v[k, rows, :] = hs[k]
        return hs

    cp_x(0).wait()
    ln1(0)

    def p_step(i, js, lo):
        rows = pl.ds(pl.multiple_of(i * P_ROWS, P_ROWS), P_ROWS)
        lhs = [l_v[k, rows, :] for k in range(D // 128)]
        deps = []
        if lo is not None:
            tl = [t[0] for row in zip(*map(_tiles, ln1(i + 1))) for t in row]
            deps = [(lo + (P_HI - lo) * n / len(tl), t) for n, t in enumerate(tl)]
        qs = _col_dots(lhs, lambda n: out_v[0:D, js[n] * DH:(js[n] + 1) * DH], len(js),
                       _never(i + pl.program_id(0)), deps)
        for j, q in zip(js, qs):
            f_v[j, rows, :] = q
        if lo is not None:
            for k in range(4):
                hd = P_HEADS + 4 * i + k
                cp_tile(wq_hbm, 0, hd, hd, SEM_WQ + jnp.where(i < 1, 1, 2)).start()

    cp_wqp(0).wait()
    p_step(0, list(range(P0_N)), None)
    cp_wqp(1).wait()
    cp_x(1).wait()
    p_step(0, list(range(P0_N, P_HEADS)), P0_LO)

    def p_body(i, carry):
        cp_x(i + 1).wait()
        p_step(i, list(range(P_HEADS)), P_LO)
        return carry

    lax.fori_loop(1, n_p - 1, p_body, 0)
    cp_k(1).start()
    cp_v(1).start()
    wmb_start(1)
    cp_wsa().wait()

    def halves(lhs, w):
        return [lambda h=h: jnp.dot(lhs(h), w(h), preferred_element_type=f32) for h in range(2)]

    def kh(h):
        return slice(h * 512, (h + 1) * 512)

    sa_t = []
    sa = None
    for n in range(2 * P_HEADS):
        j, rows = n // 2, slice(S - P_ROWS + n % 2 * 128, S - P_ROWS + (n % 2 + 1) * 128)
        big = halves(lambda h: jnp.concatenate([l_v[4 * h + k, rows, :] for k in range(4)], axis=1),
                     lambda h: out_v[kh(h), j * DH:(j + 1) * DH])
        acc = None
        for h in range(2):
            d = big[h]()
            acc = d if acc is None else acc + d
            r = 2 * n + h
            if r < 8:
                a, b = halves(lambda h: sc_v[:, kh(h)], lambda h: h2_v[kh(h), r * 128:(r + 1) * 128])
                sa_t.append(_r(a() + b()))
                if r == 7:
                    sa = jnp.concatenate(sa_t, axis=1)
                    sab_v[...] = _lane_bcast(sa[0:8, :])
                    sa = sa.astype(bf16)
            elif P_SQ <= r < P_SQ + P_HEADS:
                t = r - P_SQ
                a, b = halves(lambda h: sa[:, kh(h)], lambda h: out_v[kh(h), t * DH:(t + 1) * DH])
                sq_v[t] = (a() + b())[0:8, :]
        f_v[j, rows, :] = acc
    tiles(P_HEADS, 4, SEM_WQ + 1).wait()

    def m_waits(it):
        back = l_v.at[pl.ds(jnp.where(it == 8, 8, 0), 8)]
        kv = jnp.minimum(it, HH - 1)
        waits = [
            (it < HH, cp_k(kv)),
            (it < HH, cp_v(kv)),
            (it <= MB_LAST, cp(wmb_v.at[it & 1], wmb_v.at[it & 1], SEM_WMB + (it & 1))),
            (it == 1, tiles(P_HEADS + 4, H - P_HEADS - 4, SEM_WQ + 2)),
            (it == N_QU // U_PER_IT, tiles(WO, H, SEM_BG)),
            (jnp.logical_or(it == 6, it == 10), cp(out_hbm.at[0], out_hbm.at[0], SEM_O)),
            (jnp.logical_or(it == 8, it == 12), cp(back, back, SEM_O + 1)),
        ]
        for cond, copy in waits:
            pl.when(cond)(copy.wait)

    def m_starts(it):
        @pl.when(it + 2 < HH)
        def _():
            cp_k(it + 2).start()
            cp_v(it + 2).start()

        @pl.when(it + 2 <= MB_LAST)
        def _():
            wmb_start(it + 2)

        @pl.when(jnp.logical_or(it == 4, it == 8))
        def _():
            for k in range(8):
                cp(o_v.at[2 * it - 8 + k], out_hbm.at[0, :, pl.ds(k * DH, DH)], SEM_O).start()

        @pl.when(jnp.logical_or(it == 6, it == 10))
        def _():
            for k in range(8):
                cp(out_hbm.at[0, :, pl.ds(k * DH, DH)], l_v.at[20 - 2 * it + k], SEM_O + 1).start()

        @pl.when(it < 8)
        def _():
            for k in range(4):
                t = 4 * it + k
                cp_tile(wo_hbm, t >> 3, t & 7, WO + t, SEM_BG).start()

        for n, (src, dst) in enumerate(((wg_hbm, wg_v), (wu_hbm, wu_v), (wd_hbm, wd_v))):
            @pl.when(it >> 1 == n + 4)
            def _():
                cp_rows(src, dst, it & 1, src.shape[0] // 2, SEM_BG + 1 + n).start()

    cp_k(0).wait()
    cp_v(0).wait()

    def m_body(it, carry):
        slot = it & 1
        live = jnp.logical_and(it >= 1, it <= MB_LAST)

        def unit(u, js, deps=()):
            g = it * U_PER_IT + u
            is_q = g < N_QU
            blk4 = (g >> 4) * 4
            fb = blk4 + jnp.where(is_q, P_HEADS, -(H - P_HEADS))
            wb = blk4 + P_HEADS
            lb = jnp.where(is_q, 0, 8 - (fb & 8))
            r0 = pl.multiple_of((g & (N_RB - 1)) * U_ROWS, U_ROWS)
            lhs = [l_v[lb + k, pl.ds(r0, U_ROWS), :] for k in range(8)]
            res = _col_dots(lhs, lambda n: w_v[wb + js[n]], len(js), never, deps)
            return [(fb + j, r0, v) for j, v in zip(js, res)]

        def put(res):
            for j, r0, v in res:
                f_v[j, pl.ds(r0, v.shape[0]), :] = v

        never = _never(it)
        late = unit(0, [0])
        _attention([(f_v.at[2 * it + e], sq_v[2 * it + e], k_v.at[slot, e], v_v.at[slot, e],
                     o_v.at[(2 * it + e) & (HH - 1)]) for e in range(2)])
        mb, steps = _matvec(scb_v, [wmb_v.at[slot, k] for k in range(3)])
        for k in range(3):
            t = jnp.where(live, wmb_tile(it, k), SPARE * D // DH)
            one = jnp.where(t >> 3 == CB1, 1.0, 0.0)
            mod_v[:, pl.ds(pl.multiple_of(t * DH, DH), DH)] = _r(_r(mb[k]) + one)
        hq = jnp.minimum(2 * it + P_HEADS, H - 2)
        sq, more = _matvec(sab_v, [w_v.at[hq + e] for e in range(2)])
        for e in range(2):
            sq_v[hq + e] = sq[e]
        steps = steps + more
        span = (U_PER_IT - MV_U0) * 0.9 / len(steps)
        steps = [(MV_U0 + n * span, t) for n, t in enumerate(steps)]
        for u in range(U_PER_IT):
            res = unit(u, list(range(1 if u == 0 else 0, 4)),
                       [(pos - u, t) for pos, t in steps if u <= pos < u + 1])
            if u == 0:
                j, r0, v = res[0]
                late.append((j, r0, _pace(v[0:8, :])))
                res[0] = (j, r0 + 8, v[8:, :])
            put(res)
            if u == U_PER_IT - 2:
                put(late)
        m_starts(it)
        m_waits(it + 1)
        return carry

    lax.fori_loop(0, HH, m_body, 0)

    cp(wg_v, wg_v, SEM_BG + 1).wait()
    cp(wu_v, wu_v, SEM_BG + 2).wait()
    cp(wd_hbm, wd_v.at[:, pl.ds(0, D)], SEM_BG + 3).wait()

    def router_parts(h2):
        pr = h2 * mrow(WR, h2.shape[0])
        run = [pr[:, 0:128]]
        for b in range(1, D // 128):
            run.append(run[-1] + pr[:, b * 128:(b + 1) * 128])
        return run

    def finish_rows(r0, attn, lo, hi, never=None):
        rows = pl.ds(r0, E_ROWS)
        x2 = _r(x_v[rows, :].astype(f32) + mrow(GA, E_ROWS) * attn)
        if never is None:
            mu = jnp.sum(x2, axis=1, keepdims=True) * (1.0 / D)
            dc = x2 - mu
            var = _r(jnp.sum(dc * dc, axis=1, keepdims=True) * (1.0 / D))
        else:
            mus, vrs = [], []
            for g in range(E_ROWS // 8):
                xg = x2[g * 8:(g + 1) * 8, :]
                sp = xg[:, 0:128]
                for b in range(1, D // 128):
                    sp = sp + xg[:, b * 128:(b + 1) * 128]
                if mus:
                    sp = jnp.where(never, jnp.broadcast_to(mus[-1], (8, 128)), sp)
                mus.append(jnp.sum(sp, axis=1, keepdims=True) * (1.0 / D))
                dg = xg - mus[-1]
                vrs.append(jnp.sum(dg * dg, axis=1, keepdims=True) * (1.0 / D))
            mu = jnp.concatenate(mus, axis=0)
            var = _r(jnp.concatenate(vrs, axis=0))
        den = _r(jnp.sqrt(_r(var + EPS)))
        n = _r(_r(x2 - _r(mu)) * _recip(den))
        h2 = _r(_r(n * mrow(CB1, E_ROWS)) + mrow(SB, E_ROWS))
        x_v[rows, :] = x2.astype(bf16)
        h2_v[rows, 0:D] = h2.astype(bf16)
        of = x2 + _r(mrow(GB, E_ROWS) * h2)
        out_v[rows, 0:D] = of.astype(bf16)
        run = router_parts(h2)
        deps = []
        ot = _tiles(of)
        n_t = len(ot) * len(ot[0])
        for g in range(len(ot)):
            for b in range(len(ot[0])):
                pos = lo + (hi - lo) * (g * len(ot[0]) + b) / n_t
                deps.append((pos, ot[g][b]))
                if b % E_RUN == E_RUN - 1:
                    deps.append((pos, pltpu.bitcast(run[b][g * 8:(g + 1) * 8, :], u32)))
        return run[-1], deps

    def score_rows(r0, rp, valid, m1, m2):
        r = _r(jnp.sum(rp, axis=1, keepdims=True)) + 0.0
        r = jnp.where(r != r, -jnp.inf, r)
        bits = pltpu.bitcast(jnp.broadcast_to(r, (E_ROWS, 128)), jnp.int32)
        bits = jnp.where(bits < 0, bits ^ 0x7FFF0000, bits)
        idx = r0 + lax.broadcasted_iota(jnp.int32, (E_ROWS, 128), 0)
        key = bits | (0xFFFF - idx)
        if valid is not None:
            key = jnp.where(valid, key, int_min)
        for g in range(E_ROWS // 8):
            kg = key[g * 8:(g + 1) * 8, :]
            m2 = jnp.maximum(m2, jnp.minimum(m1, kg))
            m1 = jnp.maximum(m1, kg)
        return m1, m2

    def out_proj(r0, never, deps):
        rows = pl.ds(r0, E_ROWS)
        lhs = [o_v[j, rows, :] for j in range(HH)]
        ds = _col_dots(lhs, lambda j: jnp.concatenate([w_v[WO + 16 + j], w_v[WO + 24 + j]], axis=0),
                       D // 128, never, deps)
        return jnp.concatenate([f_v[j, rows, :] + f_v[8 + j, rows, :] + ds[j]
                                for j in range(D // 128)], axis=1)

    def e_body(c, carry):
        b0 = E_SUB * c

        @pl.when(c >= 2)
        def _():
            cp_out(b0 - E_SUB - 1, 1).start()

        @pl.when(c >= 1)
        def _():
            cp_out(b0 - E_SUB, E_SUB - 1).start()

        never = _never(c)
        m1, m2 = top_v[0], top_v[1]
        keys = []
        for t in range(E_SUB):
            m1, m2 = score_rows((b0 - E_SUB - 1 + t) * E_ROWS, rp_v[t],
                                c >= (2 if t == 0 else 1), m1, m2)
            keys.append(m2)
        top_v[0] = m1
        top_v[1] = m2
        attn = acc_v[...]
        for t in range(E_SUB):
            prev = jnp.maximum(b0 - 1, 0) if t == 0 else b0 + t - 1
            rp_v[t], deps = finish_rows(pl.multiple_of(prev * E_ROWS, E_ROWS), attn,
                                        E_LO0 if t == 0 else E_LO1, E_HI,
                                        None if t == 0 else never)
            deps.append((E_KEY, pltpu.bitcast(keys[t], u32)))
            attn = out_proj(pl.multiple_of((b0 + t) * E_ROWS, E_ROWS), never, deps)
        acc_v[...] = attn
        return carry

    lax.fori_loop(0, n_e, e_body, 0)
    n_b = S // E_ROWS
    cp_out(n_b - E_SUB - 1, E_SUB).start()
    m1, m2 = top_v[0], top_v[1]
    for t in range(E_SUB):
        m1, m2 = score_rows((n_b - E_SUB - 1 + t) * E_ROWS, rp_v[t], None, m1, m2)
    rp_last, _ = finish_rows(S - E_ROWS, acc_v[...], 0.0, 1.0)
    m1, m2 = score_rows(S - E_ROWS, rp_last, None, m1, m2)
    cp_out(n_b - 1, 1).start()

    t1 = jnp.max(m1, axis=0, keepdims=True)
    t2 = jnp.max(jnp.where(m1 == t1, m2, m1), axis=0, keepdims=True)
    i1 = (0xFFFF - t1[0, 0]) & (S - 1)
    i2 = (0xFFFF - t2[0, 0]) & (S - 1)
    g1 = pl.multiple_of(i1 & -GRP, GRP)
    g2 = pl.multiple_of(i2 & -GRP, GRP)

    xs = jnp.concatenate([h2_v[pl.ds(g1, GRP), 0:D], h2_v[pl.ds(g2, GRP), 0:D]], axis=0)

    def act(j):
        fc = slice(j * FC, (j + 1) * FC)
        g = _r(jnp.dot(xs, wg_v[:, fc], preferred_element_type=f32))
        u = _r(jnp.dot(xs, wu_v[:, fc], preferred_element_type=f32))
        return (_r(g * jax.nn.sigmoid(g)) * u).astype(bf16)

    y = None
    a = act(0)
    for j in range(F // FC):
        a_next = act(j + 1) if (j + 1) * FC < F else None
        d = jnp.dot(a, wd_v[j * FC:(j + 1) * FC, 0:D], preferred_element_type=f32)
        y = d if y is None else y + d
        a = a_next
    h2 = xs.astype(f32)
    x2 = jnp.concatenate([x_v[pl.ds(g1, GRP), :], x_v[pl.ds(g2, GRP), :]], axis=0).astype(f32)
    r = _r(jnp.sum(router_parts(h2)[-1], axis=1, keepdims=True))
    upd = _r(_r(y) * _r(jax.nn.sigmoid(r)))
    loc = lax.broadcasted_iota(jnp.int32, (2 * GRP, D), 0)
    row = jnp.where(loc < GRP, g1 + loc, g2 + loc - GRP)
    sel = jnp.logical_or(row == i1, row == i2)
    hb = _r(h2 + jnp.where(sel, upd, 0.0))
    fix_v[...] = (x2 + _r(mrow(GB, 2 * GRP) * hb)).astype(bf16)

    cp(out_v.at[:, pl.ds(0, D)], out_hbm.at[0], SEM_OUT).wait()
    fix1 = cp(fix_v.at[pl.ds(0, GRP), :], out_hbm.at[0, pl.ds(g1, GRP), :], SEM_FIX)
    fix2 = cp(fix_v.at[pl.ds(GRP, GRP), :], out_hbm.at[0, pl.ds(g2, GRP), :], SEM_FIX + 1)
    fix1.start()

    @pl.when(g2 != g1)
    def _():
        fix2.start()
        fix2.wait()

    fix1.wait()


@jax.jit
def pallas_adaLN_cond__mha_block_cached__moe_arch_mod__prompt_kernel(
    A_x: jax.Array,
    A_k_cache: jax.Array,
    A_v_cache: jax.Array,
    A_wq: jax.Array,
    A_wo: jax.Array,
    B_x: jax.Array,
    B_w_r: jax.Array,
    B_w_gate: jax.Array,
    B_w_up: jax.Array,
    B_w_down: jax.Array,
    c: jax.Array,
    w_mod: jax.Array,
):
    del B_x
    vm = pltpu.VMEM
    scratch = [
        vm((S, D), bf16),
        vm((S, D + PAD), bf16),
        vm((S, D + PAD), bf16),
        vm((HH, S, DH), bf16),
        vm((H, S, DH), f32),
        vm((E_ROWS, D), f32),
        vm((2 * H, D, DH), bf16),
        vm((2, 3, D, DH), bf16),
        vm((D, F), bf16),
        vm((D, F), bf16),
        vm((F, D + PAD), bf16),
        vm((2, 2, S, DH), bf16),
        vm((2, 2, S, DH), bf16),
        vm((HH, S, DH), bf16),
        vm((1, D), bf16),
        vm((D,), bf16),
        vm((GRP, D), bf16),
        vm((D, 128), f32),
        vm((D, 128), f32),
        vm((8, D), f32),
        vm((H, 8, DH), f32),
        vm((8, 5 * D + DH), f32),
        vm((2, 8, 128), jnp.int32),
        vm((E_SUB, E_ROWS, 128), f32),
        vm((2 * GRP, D), bf16),
        pltpu.SemaphoreType.DMA((N_SEM,)),
    ]
    def once(*refs):
        pl.when(pl.program_id(0) == 0)(lambda: _kernel(*refs))

    return pl.pallas_call(
        once,
        grid=(2,),
        in_specs=[pl.BlockSpec(memory_space=pl.ANY)] * 11,
        out_specs=pl.BlockSpec(memory_space=pl.ANY),
        out_shape=jax.ShapeDtypeStruct(A_x.shape, A_x.dtype),
        scratch_shapes=scratch,
        compiler_params=pltpu.CompilerParams(vmem_limit_bytes=124 * 1024 * 1024,
                                             disable_bounds_checks=True,
                                             disable_semaphore_checks=True),
        name="adaln_mha_moe",
    )(A_x, A_k_cache, A_v_cache, A_wq, A_wo, B_w_r, B_w_gate, B_w_up, B_w_down, c, w_mod)
```

```python
import jax
import jax.numpy as jnp
from jax import lax
import jax.experimental.pallas as pl
import jax.experimental.pallas.tpu as pltpu

S = 2048
D = 1024
H = 32
DH = 128
F = 3584
EPS = 1.0013580322265625e-05
HH = H // 2

TQ = 256
KR = 512
P_ROWS = 256
P_HEADS = 4
U_ROWS = 128
N_RB = S // U_ROWS
N_QU = (H - P_HEADS) // 4 * N_RB
N_OU = 2 * 2 * N_RB
U_PER_IT = (N_QU + N_OU) // HH
E_ROWS = 64
E_SUB = 4
PACE = 48
MV_STEP, MV_U0 = 2, 7
GRP = 16
FC = 896
PAD = 128
P0_N, P0_LO, P_LO, P_HI, P_SQ = 3, 0.9, 0.35, 0.97, 10
E_LO0, E_LO1, E_HI, E_KEY, E_RUN = 0.35, 0.45, 0.97, 0.2, 2

Q_SCALE = float(DH) ** -0.5 * 1.4426950408889634

f32 = jnp.float32
bf16 = jnp.bfloat16
u32 = jnp.uint32


def _r(x):
    return x.astype(bf16).astype(f32)


def _recip(x):
    r0 = pl.reciprocal(x, approx=True)
    return r0 * (2.0 - x * r0)


def _sigmoid(x):
    t = _r(1.0 + _r(jnp.exp(-x)))
    return _r(jnp.where(t == jnp.inf, 0.0, _recip(t)))


def _pace(t):
    for _ in range(PACE):
        t = jnp.minimum(t, jnp.max(t, axis=1, keepdims=True))
    return t


def _tiles(v):
    u = pltpu.bitcast(v, u32)
    return [[u[a * 8:(a + 1) * 8, b * 128:(b + 1) * 128] for b in range(u.shape[1] // 128)]
            for a in range(u.shape[0] // 8)]


def _col_dots(k_tiles, rhs, n_tiles, never, deps):
    n_r = len(k_tiles) // 4
    n_i = k_tiles[0].shape[0] // GRP
    total = n_tiles * n_r * n_i
    at = {}
    for n, (pos, d) in enumerate(deps):
        at.setdefault((min(int(pos * total), total - 1), n % 4), []).append(d)
    outs = []
    for j in range(n_tiles):
        tl = list(k_tiles)
        for k in range(len(k_tiles)):
            base = (j * n_r + k // 4) * n_i
            if not any((base + i, k % 4) in at for i in range(n_i)):
                continue
            tu = pltpu.bitcast(tl[k], u32)
            parts = []
            for i in range(n_i):
                t = tu[i * 8:(i + 1) * 8, :]
                for d in at.get((base + i, k % 4), ()):
                    t = jnp.where(never, d, t)
                parts.append(t)
            tl[k] = pltpu.bitcast(jnp.concatenate(parts, axis=0), bf16)
        outs.append(jnp.dot(jnp.concatenate(tl, axis=1), rhs(j), preferred_element_type=f32))
    return outs


def _matvec(a_ref, w_refs):
    accs = [None] * len(w_refs)
    steps = []
    for s in range(D // GRP):
        a = a_ref[s * GRP:(s + 1) * GRP, :]
        for n, w in enumerate(w_refs):
            t = w[s * GRP:(s + 1) * GRP, :].astype(f32) * a
            accs[n] = t if accs[n] is None else accs[n] + t
        if s % MV_STEP == MV_STEP - 1:
            steps += [t[0] for acc in accs for t in _tiles(acc)]
    res = [jnp.broadcast_to(jnp.sum(acc, axis=0, keepdims=True), (8, 128)) for acc in accs]
    return res, steps


def _lane_bcast(row):
    return jnp.concatenate([row] * 16, axis=0).T


def _never(i):
    return jnp.full((8, 128), i, jnp.int32) > (1 << 20)


def _attention(heads):
    items = [(refs, c) for refs in heads for c in range(S // TQ)]

    def scores(item):
        (q_ref, bias, k_ref, _, _), c = item
        q = q_ref[c * TQ:(c + 1) * TQ, :] + jnp.concatenate([bias] * (TQ // 8), axis=0)
        q = (q * Q_SCALE).astype(bf16)
        return lax.dot_general(q, k_ref[...], (((1,), (1,)), ((), ())),
                               preferred_element_type=f32)

    def weigh(item, s):
        (_, _, _, v_ref, o_ref), c = item
        m = jnp.max(s, axis=1, keepdims=True)
        o = None
        lp = None
        for r in range(S // KR):
            p = jnp.exp2(s[:, r * KR:(r + 1) * KR] - m)
            ps = [p[:, j * 128:(j + 1) * 128] for j in range(KR // 128)]
            t = ps[0]
            for x in ps[1:]:
                t = t + x
            lp = t if lp is None else lp + t
            ps[-1] = jnp.minimum(ps[-1], t)
            p = jnp.concatenate(ps, axis=1)
            d = jnp.dot(p.astype(bf16), v_ref[r * KR:(r + 1) * KR, :],
                        preferred_element_type=f32)
            o = d if o is None else o + d
        l = jnp.sum(lp, axis=1, keepdims=True)
        o_ref[c * TQ:(c + 1) * TQ, :] = (o * _recip(l)).astype(bf16)

    s = scores(items[0])
    for n, item in enumerate(items):
        s_next = scores(items[n + 1]) if n + 1 < len(items) else None
        weigh(item, s)
        s = s_next


SEM_C, SEM_WR, SEM_WMA, SEM_X, SEM_WQ, SEM_KV, SEM_BG, SEM_OUT, SEM_FIX, SEM_WMB, SEM_O, N_SEM = (
    0, 1, 2, 6, 14, 17, 21, 25, 26, 28, 30, 32)
WO = H
GA, SB, CB1, GB, WR, SPARE = range(6)
MB_LAST = 11


def _kernel(x_hbm, k_hbm, v_hbm, wq_hbm, wo_hbm, wr_hbm, wg_hbm, wu_hbm, wd_hbm, c_hbm,
            wm_hbm, out_hbm,
            x_v, h2_v, out_v, l_v, f_v, acc_v, w_v, wmb_v, wg_v, wu_v, wd_v, k_v, v_v, o_v,
            c_v, wr_v, sc_v, scb_v, sab_v, ca_v, sq_v, mod_v, top_v, rp_v, fix_v, sems):
    n_p = S // P_ROWS
    n_e = S // (E_SUB * E_ROWS)
    pq = P_HEADS * DH

    def cp(src, dst, sem):
        return pltpu.make_async_copy(src, dst, sems.at[sem])

    def cp_c():
        return cp(c_hbm, c_v, SEM_C)

    def cp_wr():
        return cp(wr_hbm, wr_v, SEM_WR)

    def cp_wca(j):
        return cp(wm_hbm.at[:, pl.ds(D + j * 512, 512)],
                  h2_v.at[pl.ds(D, D), pl.ds(j * 512, 512)], SEM_WMA + j)

    def cp_wsa():
        return cp(wm_hbm.at[:, pl.ds(0, D)], h2_v.at[pl.ds(0, D), pl.ds(0, D)], SEM_WMA + 2)

    def cp_x(i):
        return cp(x_hbm.at[0, pl.ds(i * P_ROWS, P_ROWS), :], x_v.at[pl.ds(i * P_ROWS, P_ROWS), :],
                  SEM_X + i)

    def cp_wqp(j):
        cols = (pl.ds(0, P0_N * DH), pl.ds(P0_N * DH, pq - P0_N * DH))[j]
        return cp(wq_hbm.at[:, cols], out_v.at[pl.ds(0, D), cols], (SEM_WQ, SEM_WMA + 3)[j])

    def cp_tile(src, row, col, j, sem):
        return cp(src.at[pl.ds(pl.multiple_of(row * D, D), D), pl.ds(pl.multiple_of(col * DH, DH), DH)],
                  w_v.at[j], sem)

    def tiles(lo, n, sem):
        return cp(w_v.at[pl.ds(lo, n)], w_v.at[pl.ds(lo, n)], sem)

    def cp_k(it):
        return cp(k_hbm.at[0, pl.ds(2 * it, 2)], k_v.at[it & 1], SEM_KV + (it & 1))

    def cp_v(it):
        return cp(v_hbm.at[0, pl.ds(2 * it, 2)], v_v.at[it & 1], SEM_KV + 2 + (it & 1))

    def cp_rows(src, dst, i, n, sem):
        return cp(src.at[pl.ds(i * n, n), :], dst.at[pl.ds(i * n, n), pl.ds(0, src.shape[1])], sem)

    def wmb_tile(it, k):
        return jnp.minimum(3 * (it - 1) + k, 4 * D // DH - 1)

    def wmb_start(it):
        for k in range(3):
            cols = pl.ds(pl.multiple_of(2 * D + wmb_tile(it, k) * DH, DH), DH)
            cp(wm_hbm.at[:, cols], wmb_v.at[it & 1, k], SEM_WMB + (it & 1)).start()

    def cp_out(i, n):
        return cp(out_v.at[pl.ds(i * E_ROWS, n * E_ROWS), pl.ds(0, D)],
                  out_hbm.at[0, pl.ds(i * E_ROWS, n * E_ROWS), :], SEM_OUT)

    def mrow(k, n):
        m = mod_v[:, k * D:(k + 1) * D]
        return jnp.concatenate([m] * (n // 8), axis=0)

    cp_c().start()
    cp_wr().start()
    for j in range(2):
        cp_wca(j).start()
    cp_x(0).start()
    cp_wqp(0).start()
    cp_wqp(1).start()
    for i in range(1, n_p):
        cp_x(i).start()
    cp_wsa().start()
    cp_k(0).start()
    cp_v(0).start()

    cp_c().wait()
    cp_wr().wait()
    mod_v[:, WR * D:(WR + 1) * D] = jnp.broadcast_to(wr_v[...].astype(f32).reshape(1, D), (8, D))
    int_min = jnp.iinfo(jnp.int32).min
    top_v[...] = jnp.full(top_v.shape, int_min, jnp.int32)
    acc_v[...] = jnp.zeros(acc_v.shape, f32)
    rp_v[...] = jnp.zeros(rp_v.shape, f32)
    wmb_v[0] = jnp.zeros(wmb_v.shape[1:], bf16)
    cf = c_v[...].astype(f32)
    sc = jnp.broadcast_to(_r(cf * _sigmoid(cf)), (8, D))
    sc_v[...] = jnp.concatenate([sc, sc], axis=0).astype(bf16)
    scb_v[...] = _lane_bcast(sc)

    def wca_body(j, carry):
        cp_wca(j).wait()
        cols = pl.ds(pl.multiple_of(j * 512, 512), 512)
        mj = jnp.dot(sc_v[...], h2_v[D:2 * D, cols], preferred_element_type=f32)
        ca_v[:, cols] = _r(_r(mj[0:8, :]) + 1.0)
        return carry

    lax.fori_loop(0, 2, wca_body, 0)

    def ln1(i):
        rows = pl.ds(pl.multiple_of(i * P_ROWS, P_ROWS), P_ROWS)
        x = x_v[rows, :].astype(f32)
        mu = jnp.sum(x, axis=1, keepdims=True) * (1.0 / D)
        d = x - mu
        var = jnp.sum(d * d, axis=1, keepdims=True) * (1.0 / D)
        n = d * lax.rsqrt(var + EPS)
        h = n * jnp.concatenate([ca_v[...]] * (P_ROWS // 8), axis=0)
        hs = [h[:, k * 128:(k + 1) * 128].astype(bf16) for k in range(D // 128)]
        for k in range(D // 128):
            l_v[k, rows, :] = hs[k]
        return hs

    cp_x(0).wait()
    ln1(0)

    def p_step(i, js, lo):
        rows = pl.ds(pl.multiple_of(i * P_ROWS, P_ROWS), P_ROWS)
        lhs = [l_v[k, rows, :] for k in range(D // 128)]
        deps = []
        if lo is not None:
            tl = [t[0] for row in zip(*map(_tiles, ln1(i + 1))) for t in row]
            deps = [(lo + (P_HI - lo) * n / len(tl), t) for n, t in enumerate(tl)]
        qs = _col_dots(lhs, lambda n: out_v[0:D, js[n] * DH:(js[n] + 1) * DH], len(js),
                       _never(i + pl.program_id(0)), deps)
        for j, q in zip(js, qs):
            f_v[j, rows, :] = q
        if lo is not None:
            for k in range(4):
                hd = P_HEADS + 4 * i + k
                cp_tile(wq_hbm, 0, hd, hd, SEM_WQ + jnp.where(i < 1, 1, 2)).start()

    cp_wqp(0).wait()
    p_step(0, list(range(P0_N)), None)
    cp_wqp(1).wait()
    cp_x(1).wait()
    p_step(0, list(range(P0_N, P_HEADS)), P0_LO)

    def p_body(i, carry):
        cp_x(i + 1).wait()
        p_step(i, list(range(P_HEADS)), P_LO)
        return carry

    lax.fori_loop(1, n_p - 1, p_body, 0)
    cp_k(1).start()
    cp_v(1).start()
    wmb_start(1)
    cp_wsa().wait()

    def halves(lhs, w):
        return [lambda h=h: jnp.dot(lhs(h), w(h), preferred_element_type=f32) for h in range(2)]

    def kh(h):
        return slice(h * 512, (h + 1) * 512)

    sa_t = []
    sa = None
    for n in range(2 * P_HEADS):
        j, rows = n // 2, slice(S - P_ROWS + n % 2 * 128, S - P_ROWS + (n % 2 + 1) * 128)
        big = halves(lambda h: jnp.concatenate([l_v[4 * h + k, rows, :] for k in range(4)], axis=1),
                     lambda h: out_v[kh(h), j * DH:(j + 1) * DH])
        acc = None
        for h in range(2):
            d = big[h]()
            acc = d if acc is None else acc + d
            r = 2 * n + h
            if r < 8:
                a, b = halves(lambda h: sc_v[:, kh(h)], lambda h: h2_v[kh(h), r * 128:(r + 1) * 128])
                sa_t.append(_r(a() + b()))
                if r == 7:
                    sa = jnp.concatenate(sa_t, axis=1)
                    sab_v[...] = _lane_bcast(sa[0:8, :])
                    sa = sa.astype(bf16)
            elif P_SQ <= r < P_SQ + P_HEADS:
                t = r - P_SQ
                a, b = halves(lambda h: sa[:, kh(h)], lambda h: out_v[kh(h), t * DH:(t + 1) * DH])
                sq_v[t] = (a() + b())[0:8, :]
        f_v[j, rows, :] = acc
    tiles(P_HEADS, 4, SEM_WQ + 1).wait()

    def m_waits(it):
        back = l_v.at[pl.ds(jnp.where(it == 8, 8, 0), 8)]
        kv = jnp.minimum(it, HH - 1)
        waits = [
            (it < HH, cp_k(kv)),
            (it < HH, cp_v(kv)),
            (it <= MB_LAST, cp(wmb_v.at[it & 1], wmb_v.at[it & 1], SEM_WMB + (it & 1))),
            (it == 1, tiles(P_HEADS + 4, H - P_HEADS - 4, SEM_WQ + 2)),
            (it == N_QU // U_PER_IT, tiles(WO, H, SEM_BG)),
            (jnp.logical_or(it == 6, it == 10), cp(out_hbm.at[0], out_hbm.at[0], SEM_O)),
            (jnp.logical_or(it == 8, it == 12), cp(back, back, SEM_O + 1)),
        ]
        for cond, copy in waits:
            pl.when(cond)(copy.wait)

    def m_starts(it):
        @pl.when(it + 2 < HH)
        def _():
            cp_k(it + 2).start()
            cp_v(it + 2).start()

        @pl.when(it + 2 <= MB_LAST)
        def _():
            wmb_start(it + 2)

        @pl.when(jnp.logical_or(it == 4, it == 8))
        def _():
            for k in range(8):
                cp(o_v.at[2 * it - 8 + k], out_hbm.at[0, :, pl.ds(k * DH, DH)], SEM_O).start()

        @pl.when(jnp.logical_or(it == 6, it == 10))
        def _():
            for k in range(8):
                cp(out_hbm.at[0, :, pl.ds(k * DH, DH)], l_v.at[20 - 2 * it + k], SEM_O + 1).start()

        @pl.when(it < 8)
        def _():
            for k in range(4):
                t = 4 * it + k
                cp_tile(wo_hbm, t >> 3, t & 7, WO + t, SEM_BG).start()

        for n, (src, dst) in enumerate(((wg_hbm, wg_v), (wu_hbm, wu_v), (wd_hbm, wd_v))):
            @pl.when(it >> 1 == n + 4)
            def _():
                cp_rows(src, dst, it & 1, src.shape[0] // 2, SEM_BG + 1 + n).start()

    cp_k(0).wait()
    cp_v(0).wait()

    def m_body(it, carry):
        slot = it & 1
        live = jnp.logical_and(it >= 1, it <= MB_LAST)

        def unit(u, js, deps=()):
            g = it * U_PER_IT + u
            is_q = g < N_QU
            blk4 = (g >> 4) * 4
            fb = blk4 + jnp.where(is_q, P_HEADS, -(H - P_HEADS))
            wb = blk4 + P_HEADS
            lb = jnp.where(is_q, 0, 8 - (fb & 8))
            r0 = pl.multiple_of((g & (N_RB - 1)) * U_ROWS, U_ROWS)
            lhs = [l_v[lb + k, pl.ds(r0, U_ROWS), :] for k in range(8)]
            res = _col_dots(lhs, lambda n: w_v[wb + js[n]], len(js), never, deps)
            return [(fb + j, r0, v) for j, v in zip(js, res)]

        def put(res):
            for j, r0, v in res:
                f_v[j, pl.ds(r0, v.shape[0]), :] = v

        never = _never(it)
        late = unit(0, [0])
        _attention([(f_v.at[2 * it + e], sq_v[2 * it + e], k_v.at[slot, e], v_v.at[slot, e],
                     o_v.at[(2 * it + e) & (HH - 1)]) for e in range(2)])
        mb, steps = _matvec(scb_v, [wmb_v.at[slot, k] for k in range(3)])
        for k in range(3):
            t = jnp.where(live, wmb_tile(it, k), SPARE * D // DH)
            one = jnp.where(t >> 3 == CB1, 1.0, 0.0)
            mod_v[:, pl.ds(pl.multiple_of(t * DH, DH), DH)] = _r(_r(mb[k]) + one)
        hq = jnp.minimum(2 * it + P_HEADS, H - 2)
        sq, more = _matvec(sab_v, [w_v.at[hq + e] for e in range(2)])
        for e in range(2):
            sq_v[hq + e] = sq[e]
        steps = steps + more
        span = (U_PER_IT - MV_U0) * 0.9 / len(steps)
        steps = [(MV_U0 + n * span, t) for n, t in enumerate(steps)]
        for u in range(U_PER_IT):
            res = unit(u, list(range(1 if u == 0 else 0, 4)),
                       [(pos - u, t) for pos, t in steps if u <= pos < u + 1])
            if u == 0:
                j, r0, v = res[0]
                late.append((j, r0, _pace(v[0:8, :])))
                res[0] = (j, r0 + 8, v[8:, :])
            put(res)
            if u == U_PER_IT - 2:
                put(late)
        m_starts(it)
        m_waits(it + 1)
        return carry

    lax.fori_loop(0, HH, m_body, 0)

    cp(wg_v, wg_v, SEM_BG + 1).wait()
    cp(wu_v, wu_v, SEM_BG + 2).wait()
    cp(wd_hbm, wd_v.at[:, pl.ds(0, D)], SEM_BG + 3).wait()

    def router_parts(h2):
        pr = h2 * mrow(WR, h2.shape[0])
        run = [pr[:, 0:128]]
        for b in range(1, D // 128):
            run.append(run[-1] + pr[:, b * 128:(b + 1) * 128])
        return run

    def finish_rows(r0, attn, lo, hi, never=None):
        rows = pl.ds(r0, E_ROWS)
        x2 = _r(x_v[rows, :].astype(f32) + mrow(GA, E_ROWS) * attn)
        if never is None:
            mu = jnp.sum(x2, axis=1, keepdims=True) * (1.0 / D)
            dc = x2 - mu
            var = _r(jnp.sum(dc * dc, axis=1, keepdims=True) * (1.0 / D))
        else:
            mus, vrs = [], []
            for g in range(E_ROWS // 8):
                xg = x2[g * 8:(g + 1) * 8, :]
                sp = xg[:, 0:128]
                for b in range(1, D // 128):
                    sp = sp + xg[:, b * 128:(b + 1) * 128]
                if mus:
                    sp = jnp.where(never, jnp.broadcast_to(mus[-1], (8, 128)), sp)
                mus.append(jnp.sum(sp, axis=1, keepdims=True) * (1.0 / D))
                dg = xg - mus[-1]
                vrs.append(jnp.sum(dg * dg, axis=1, keepdims=True) * (1.0 / D))
            mu = jnp.concatenate(mus, axis=0)
            var = _r(jnp.concatenate(vrs, axis=0))
        den = _r(jnp.sqrt(_r(var + EPS)))
        n = _r(_r(x2 - _r(mu)) * _recip(den))
        h2 = _r(_r(n * mrow(CB1, E_ROWS)) + mrow(SB, E_ROWS))
        x_v[rows, :] = x2.astype(bf16)
        h2_v[rows, 0:D] = h2.astype(bf16)
        of = x2 + _r(mrow(GB, E_ROWS) * h2)
        out_v[rows, 0:D] = of.astype(bf16)
        run = router_parts(h2)
        deps = []
        ot = _tiles(of)
        n_t = len(ot) * len(ot[0])
        for g in range(len(ot)):
            for b in range(len(ot[0])):
                pos = lo + (hi - lo) * (g * len(ot[0]) + b) / n_t
                deps.append((pos, ot[g][b]))
                if b % E_RUN == E_RUN - 1:
                    deps.append((pos, pltpu.bitcast(run[b][g * 8:(g + 1) * 8, :], u32)))
        return run[-1], deps

    def score_rows(r0, rp, valid, m1, m2):
        r = _r(jnp.sum(rp, axis=1, keepdims=True)) + 0.0
        r = jnp.where(r != r, -jnp.inf, r)
        bits = pltpu.bitcast(jnp.broadcast_to(r, (E_ROWS, 128)), jnp.int32)
        bits = jnp.where(bits < 0, bits ^ 0x7FFF0000, bits)
        idx = r0 + lax.broadcasted_iota(jnp.int32, (E_ROWS, 128), 0)
        key = bits | (0xFFFF - idx)
        if valid is not None:
            key = jnp.where(valid, key, int_min)
        for g in range(E_ROWS // 8):
            kg = key[g * 8:(g + 1) * 8, :]
            m2 = jnp.maximum(m2, jnp.minimum(m1, kg))
            m1 = jnp.maximum(m1, kg)
        return m1, m2

    def out_proj(r0, never, deps):
        rows = pl.ds(r0, E_ROWS)
        lhs = [o_v[j, rows, :] for j in range(HH)]
        ds = _col_dots(lhs, lambda j: jnp.concatenate([w_v[WO + 16 + j], w_v[WO + 24 + j]], axis=0),
                       D // 128, never, deps)
        return jnp.concatenate([f_v[j, rows, :] + f_v[8 + j, rows, :] + ds[j]
                                for j in range(D // 128)], axis=1)

    def e_body(c, carry):
        b0 = E_SUB * c

        @pl.when(c >= 2)
        def _():
            cp_out(b0 - E_SUB - 1, 1).start()

        @pl.when(c >= 1)
        def _():
            cp_out(b0 - E_SUB, E_SUB - 1).start()

        never = _never(c)
        m1, m2 = top_v[0], top_v[1]
        keys = []
        for t in range(E_SUB):
            m1, m2 = score_rows((b0 - E_SUB - 1 + t) * E_ROWS, rp_v[t],
                                c >= (2 if t == 0 else 1), m1, m2)
            keys.append(m2)
        top_v[0] = m1
        top_v[1] = m2
        attn = acc_v[...]
        for t in range(E_SUB):
            prev = jnp.maximum(b0 - 1, 0) if t == 0 else b0 + t - 1
            rp_v[t], deps = finish_rows(pl.multiple_of(prev * E_ROWS, E_ROWS), attn,
                                        E_LO0 if t == 0 else E_LO1, E_HI,
                                        None if t == 0 else never)
            deps.append((E_KEY, pltpu.bitcast(keys[t], u32)))
            attn = out_proj(pl.multiple_of((b0 + t) * E_ROWS, E_ROWS), never, deps)
        acc_v[...] = attn
        return carry

    lax.fori_loop(0, n_e, e_body, 0)
    n_b = S // E_ROWS
    cp_out(n_b - E_SUB - 1, E_SUB).start()
    m1, m2 = top_v[0], top_v[1]
    for t in range(E_SUB):
        m1, m2 = score_rows((n_b - E_SUB - 1 + t) * E_ROWS, rp_v[t], None, m1, m2)
    rp_last, _ = finish_rows(S - E_ROWS, acc_v[...], 0.0, 1.0)
    m1, m2 = score_rows(S - E_ROWS, rp_last, None, m1, m2)
    cp_out(n_b - 1, 1).start()

    t1 = jnp.max(m1, axis=0, keepdims=True)
    t2 = jnp.max(jnp.where(m1 == t1, m2, m1), axis=0, keepdims=True)
    i1 = (0xFFFF - t1[0, 0]) & (S - 1)
    i2 = (0xFFFF - t2[0, 0]) & (S - 1)
    g1 = pl.multiple_of(i1 & -GRP, GRP)
    g2 = pl.multiple_of(i2 & -GRP, GRP)

    xs = jnp.concatenate([h2_v[pl.ds(g1, GRP), 0:D], h2_v[pl.ds(g2, GRP), 0:D]], axis=0)

    def act(j):
        fc = slice(j * FC, (j + 1) * FC)
        g = _r(jnp.dot(xs, wg_v[:, fc], preferred_element_type=f32))
        u = _r(jnp.dot(xs, wu_v[:, fc], preferred_element_type=f32))
        return (_r(g * _sigmoid(g)) * u).astype(bf16)

    y = None
    a = act(0)
    for j in range(F // FC):
        a_next = act(j + 1) if (j + 1) * FC < F else None
        d = jnp.dot(a, wd_v[j * FC:(j + 1) * FC, 0:D], preferred_element_type=f32)
        y = d if y is None else y + d
        a = a_next
    h2 = xs.astype(f32)
    x2 = jnp.concatenate([x_v[pl.ds(g1, GRP), :], x_v[pl.ds(g2, GRP), :]], axis=0).astype(f32)
    r = _r(jnp.sum(router_parts(h2)[-1], axis=1, keepdims=True))
    upd = _r(_r(y) * _sigmoid(r))
    loc = lax.broadcasted_iota(jnp.int32, (2 * GRP, D), 0)
    row = jnp.where(loc < GRP, g1 + loc, g2 + loc - GRP)
    sel = jnp.logical_or(row == i1, row == i2)
    hb = _r(h2 + jnp.where(sel, upd, 0.0))
    fix_v[...] = (x2 + _r(mrow(GB, 2 * GRP) * hb)).astype(bf16)

    cp(out_v.at[:, pl.ds(0, D)], out_hbm.at[0], SEM_OUT).wait()
    fix1 = cp(fix_v.at[pl.ds(0, GRP), :], out_hbm.at[0, pl.ds(g1, GRP), :], SEM_FIX)
    fix2 = cp(fix_v.at[pl.ds(GRP, GRP), :], out_hbm.at[0, pl.ds(g2, GRP), :], SEM_FIX + 1)
    fix1.start()

    @pl.when(g2 != g1)
    def _():
        fix2.start()
        fix2.wait()

    fix1.wait()


@jax.jit
def pallas_adaLN_cond__mha_block_cached__moe_arch_mod__prompt_kernel(
    A_x: jax.Array,
    A_k_cache: jax.Array,
    A_v_cache: jax.Array,
    A_wq: jax.Array,
    A_wo: jax.Array,
    B_x: jax.Array,
    B_w_r: jax.Array,
    B_w_gate: jax.Array,
    B_w_up: jax.Array,
    B_w_down: jax.Array,
    c: jax.Array,
    w_mod: jax.Array,
):
    del B_x
    vm = pltpu.VMEM
    scratch = [
        vm((S, D), bf16),
        vm((S, D + PAD), bf16),
        vm((S, D + PAD), bf16),
        vm((HH, S, DH), bf16),
        vm((H, S, DH), f32),
        vm((E_ROWS, D), f32),
        vm((2 * H, D, DH), bf16),
        vm((2, 3, D, DH), bf16),
        vm((D, F), bf16),
        vm((D, F), bf16),
        vm((F, D + PAD), bf16),
        vm((2, 2, S, DH), bf16),
        vm((2, 2, S, DH), bf16),
        vm((HH, S, DH), bf16),
        vm((1, D), bf16),
        vm((D,), bf16),
        vm((GRP, D), bf16),
        vm((D, 128), f32),
        vm((D, 128), f32),
        vm((8, D), f32),
        vm((H, 8, DH), f32),
        vm((8, 5 * D + DH), f32),
        vm((2, 8, 128), jnp.int32),
        vm((E_SUB, E_ROWS, 128), f32),
        vm((2 * GRP, D), bf16),
        pltpu.SemaphoreType.DMA((N_SEM,)),
    ]

    def once(*refs):
        pl.when(pl.program_id(0) == 0)(lambda: _kernel(*refs))

    return pl.pallas_call(
        once,
        grid=(2,),
        in_specs=[pl.BlockSpec(memory_space=pl.ANY)] * 11,
        out_specs=pl.BlockSpec(memory_space=pl.ANY),
        out_shape=jax.ShapeDtypeStruct(A_x.shape, A_x.dtype),
        scratch_shapes=scratch,
        compiler_params=pltpu.CompilerParams(vmem_limit_bytes=124 * 1024 * 1024,
                                             disable_bounds_checks=True,
                                             disable_semaphore_checks=True),
        name="adaln_mha_moe",
    )(A_x, A_k_cache, A_v_cache, A_wq, A_wo, B_w_r, B_w_gate, B_w_up, B_w_down, c, w_mod)
```
